```python
import os as _os
_os.environ.setdefault("JAX_PLATFORMS", "cpu")
import jax
import jax.numpy as jnp

def _softmax(x, axis=-1):
    return jax.nn.softmax(x, axis=axis)
def _gelu(x):
    return jax.nn.gelu(x, approximate=True)
def _silu(x):
    return jax.nn.silu(x)
def _sigmoid(x):
    return jax.nn.sigmoid(x)
def _layernorm(x, axis=-1, eps=1e-5):
    m = jnp.mean(x, axis=axis, keepdims=True)
    v = jnp.var(x, axis=axis, keepdims=True)
    return (x - m) / jnp.sqrt(v + eps)
def _scatter_add(tgt, idx, src, axis=0):
    return tgt.at[idx].add(src)
def _segment_sum(src, seg, n):
    return jax.ops.segment_sum(src, seg, n)
class _Rng:
    def __init__(self, key):
        self._k = key
    def _next(self):
        self._k, sub = jax.random.split(self._k)
        return sub
    def normal(self, shape):
        return jax.random.normal(self._next(), shape, dtype=jnp.bfloat16)
    def randint(self, lo, hi, shape):
        return jax.random.randint(self._next(), shape, lo, hi, dtype=jnp.int32)
    def uniform(self, shape, lo=0.0, hi=1.0):
        return jax.random.uniform(self._next(), shape, jnp.bfloat16, lo, hi)
    def permutation(self, n):
        return jax.random.permutation(self._next(), n)


kernel_name = 'concat_heads__sliding_block__sliding_block__prompt'

def setup_inputs():
    _rng = _Rng(jax.random.key(int.from_bytes(__import__("os").urandom(4), "little")))
    _w = (lambda a: (lambda t: t.astype(jnp.bfloat16) if jnp.issubdtype(t.dtype, jnp.floating) else t)(jnp.asarray(a)))
    def _A_setup():
        B, S, D = 1, 2048, 448
        return {
            "x": _w((lambda *s: _rng.normal(s) * 0.2)(B, S, D)),
            "wqkv": _w((lambda *s: _rng.normal(s) * 0.2)(D, 3 * D)),
            "wo": _w((lambda *s: _rng.normal(s) * 0.05)(D, D)),
        }
    _A_in = _A_setup()

    def _B_setup():
        B, S, D = 1, 2048, 448
        return {
            "x": _w((lambda *s: _rng.normal(s) * 0.2)(B, S, D)),
            "wqkv": _w((lambda *s: _rng.normal(s) * 0.2)(D, 3 * D)),
            "wo": _w((lambda *s: _rng.normal(s) * 0.05)(D, D)),
        }
    _B_in = _B_setup()

    return {
        "A_x": _A_in["x"],
        "A_wqkv": _A_in["wqkv"],
        "A_wo": _A_in["wo"],
        "B_x": _B_in["x"],
        "B_wqkv": _B_in["wqkv"],
        "B_wo": _B_in["wo"],
    }

def reference(A_x, A_wqkv, A_wo, B_x, B_wqkv, B_wo):
    def _A_ref(x, wqkv, wo):
        B, S, D = x.shape
        H = 16; Dh = D // H; W = 256
        qkv = (lambda x, *d: x.transpose(*d))((x @ wqkv).reshape(B, S, 3, H, Dh), 2, 0, 3, 1, 4)
        q, k, v = qkv[0], qkv[1], qkv[2]
        scores = jnp.einsum("bhqd,bhkd->bhqk", q, k) * (Dh ** -0.5)
        idx = jnp.arange(S)
        mask = (idx[:, None] - idx[None, :] >= 0) & (idx[:, None] - idx[None, :] < W)
        scores = jnp.where(mask[None, None], scores, -1e9)
        p = _softmax(scores, axis=-1)
        o = jnp.einsum("bhqk,bhkd->bhqd", p, v)
        return (lambda x, *d: x.transpose(*d))(o, 0, 2, 1, 3).reshape(B, S, D) @ wo

    def _B_ref(x, wqkv, wo):
        B, S, D = x.shape
        H = 16; Dh = D // H; W = 256
        qkv = (lambda x, *d: x.transpose(*d))((x @ wqkv).reshape(B, S, 3, H, Dh), 2, 0, 3, 1, 4)
        q, k, v = qkv[0], qkv[1], qkv[2]
        scores = jnp.einsum("bhqd,bhkd->bhqk", q, k) * (Dh ** -0.5)
        idx = jnp.arange(S)
        mask = (idx[:, None] - idx[None, :] >= 0) & (idx[:, None] - idx[None, :] < W)
        scores = jnp.where(mask[None, None], scores, -1e9)
        p = _softmax(scores, axis=-1)
        o = jnp.einsum("bhqk,bhkd->bhqd", p, v)
        return (lambda x, *d: x.transpose(*d))(o, 0, 2, 1, 3).reshape(B, S, D) @ wo

    a = _A_ref(A_x, A_wqkv, A_wo)
    b = _B_ref(B_x, B_wqkv, B_wo)
    return jnp.concatenate([a, b], axis=-1)
```

```python
import functools
import jax
import jax.numpy as jnp
from jax import lax
import jax.experimental.pallas as pl
import jax.experimental.pallas.tpu as pltpu

S, D, H, DH, WIN = 2048, 448, 16, 28, 256
T = 128
TQ = 256
NB = TQ // T
NT_ = S // T
GRP = 4 * DH
LOG2E = 1.4426950408889634
QSCALE = (DH ** -0.5) * LOG2E
NEG = -1e30
f32 = jnp.float32
bf16 = jnp.bfloat16
u32 = jnp.uint32
NSLOT = 3
SB = 32
KROWS = S // 2
POFF = 4 * KROWS
PROWS = 144
FIRST_TIE = 5


def _pk(x):
    return pltpu.bitcast(x.astype(bf16), u32)


def _ubf(x):
    return pltpu.bitcast(x, bf16)


def _cat(xs, axis=0):
    xs = [x for x in xs if x.shape[axis] > 0]
    return xs[0] if len(xs) == 1 else jnp.concatenate(xs, axis=axis)


def _kernel(xa_ref, wqa_ref, woa_ref, xb_ref, wqb_ref, wob_ref, o_ref,
            wT_ref, woT_ref, vT_ref, q_ref, oT_ref, z_ref, kp0_ref, kp1_ref, *s_refs):
    step = pl.program_id(0)
    kp_refs = (kp0_ref, kp1_ref)

    @pl.when(step == 0)
    def _():
        wT_ref[0] = pltpu.bitcast(wqa_ref[...].T, u32)
        wT_ref[1] = pltpu.bitcast(wqb_ref[...].T, u32)
        woT_ref[0] = pltpu.bitcast(woa_ref[...].T, u32)
        woT_ref[1] = pltpu.bitcast(wob_ref[...].T, u32)
        z_ref[0] = 0
        z_ref[1] = 0

    zw = pl.multiple_of(z_ref[0], 8)
    zr = pl.multiple_of(z_ref[1], 8)

    sub = lax.broadcasted_iota(jnp.int32, (8, T), 0)
    lane8 = lax.broadcasted_iota(jnp.int32, (8, T), 1)
    lo4 = sub < 4
    ones_hi = jnp.where(sub == 4, 1.0, 0.0).astype(f32)
    ones_lo = jnp.where(sub == 0, 1.0, 0.0).astype(f32)
    HD = D // 2

    def kbase(br, g):
        return (2 * br + g // 2) * KROWS

    def project(br, x_ref):
        x = x_ref[...]
        qT = jnp.dot(_ubf(wT_ref[br, 0:HD, :]), x, preferred_element_type=f32) * QSCALE
        for b in range(NB):
            for g in range(4):
                blk = qT[GRP * g:GRP * g + GRP, b * T:(b + 1) * T]
                h1 = pltpu.roll(blk[24:56], T - SB, 1)
                h2 = pltpu.roll(blk[56:88], T - 2 * SB, 1)
                h3 = pltpu.roll(blk[80:112], T - 3 * SB, 1)
                qg = jnp.concatenate([
                    blk[0:24], jnp.where(lo4, blk[24:32], h1[0:8]), h1[8:32],
                    h2[0:24], jnp.where(lo4, h2[24:32], h3[0:8]), h3[8:32]], axis=0)
                q_ref[br, b, g] = _pk(qg)
        kT = jnp.dot(_ubf(wT_ref[br, HD:2 * HD, :]), x, preferred_element_type=f32)
        zero16 = jnp.zeros((16, TQ), f32)
        for g in range(4):
            kg = jnp.concatenate([kT[GRP * g:GRP * g + GRP], zero16], axis=0).astype(bf16)
            kgt = pltpu.bitcast(kg.T, u32)
            ev = pltpu.unpack_elementwise(kgt, index=0, packed_dtype=bf16, unpacked_dtype=f32)
            od = pltpu.unpack_elementwise(kgt, index=1, packed_dtype=bf16, unpacked_dtype=f32)
            rows = []
            for v in range(TQ // 16):
                rows += [ev[8 * v:8 * v + 8], od[8 * v:8 * v + 8]]
            off = pl.multiple_of(kbase(br, g) + step * (TQ // 2), TQ // 2)
            kp_refs[g % 2][pl.ds(off, TQ // 2), :] = _pk(jnp.concatenate(rows, axis=0))
        vT = jnp.dot(_ubf(wT_ref[br, 2 * HD:3 * HD, :]), x, preferred_element_type=f32)
        for b in range(NB):
            parts = []
            for p in range(H // 2):
                blk = vT[56 * p:56 * p + 56, b * T:(b + 1) * T]
                mid = blk[24:32]
                parts += [blk[0:24], jnp.where(lo4, mid, ones_hi),
                          jnp.where(lo4, ones_lo, mid), blk[32:56]]
            vT_ref[br, step * NB + b] = _pk(jnp.concatenate(parts, axis=0))

    srow = lax.broadcasted_iota(jnp.int32, (SB, T), 0)
    skey = (srow & 16) + 2 * (srow & 7) + ((srow >> 3) & 1)
    tri = skey <= (lax.broadcasted_iota(jnp.int32, (SB, T), 1) & (SB - 1))
    ql = lane8 & (SB - 1)
    pmask = [jnp.where(16 * v + 2 * sub <= ql, jnp.uint32(0xFFFF), jnp.uint32(0))
             | jnp.where(16 * v + 2 * sub + 1 <= ql, jnp.uint32(0xFFFF0000), jnp.uint32(0))
             for v in range(2)]
    crow = lax.broadcasted_iota(jnp.int32, (56, T), 0)
    ccol = lax.broadcasted_iota(jnp.int32, (56, T), 1)
    hrow = ((crow >= 14).astype(jnp.int32) + (crow >= 28).astype(jnp.int32)
            + (crow >= 42).astype(jnp.int32))
    code = (hrow + (ccol >> 5)) & 3
    odd = (lane8 & SB) != 0
    hi = lane8 >= 2 * SB

    def nprev(u, c, first):
        return min(WIN, u[1] * T + SB * c) if first else WIN

    def sm_items(u, n, first, ms):
        s_ref = s_refs[n % NSLOT]
        p_ref = kp_refs[(u[2] + 1) % 2]
        items = []
        for c in range(4):
            npv = nprev(u, c, first)
            nv = (WIN if npv == WIN else npv + SB) // 16
            pb = POFF + c * PROWS

            def item(v, c=c, npv=npv, pb=pb):
                s = s_ref[pl.ds(zr + (c * WIN + 16 * v), 16), :]
                p = jnp.exp2(s - ms[c])
                pk = pltpu.pack_elementwise([p[0:8], p[8:16]], packed_dtype=bf16)
                if v >= 2:
                    r = 8 * v if npv == WIN else 8 * (v - 2)
                    p_ref[pl.ds(zw + (pb + r), 8), :] = pk
                elif npv == WIN:
                    p_ref[pl.ds(zw + (pb + 8 * v), 8), :] = pk & ~pmask[v]
                    p_ref[pl.ds(zw + (pb + 128 + 8 * v), 8), :] = pk & pmask[v]
                else:
                    p_ref[pl.ds(zw + (pb + npv // 2 + 8 * v), 8), :] = pk
            items += [functools.partial(item, v) for v in range(nv)]
        return items

    def qk(u, n, first, items):
        br, b, g = u
        s_ref = s_refs[n % NSLOT]
        k_ref = kp_refs[g % 2]
        base = pl.multiple_of(kbase(br, g) + (step * NB + b) * (T // 2), T // 2)
        offs = []
        for c in range(4):
            npv = nprev(u, c, first)
            offs.append([16 * c, 16 * c + 8] + [16 * c - npv // 2 + 8 * v for v in range(npv // 16)])
        rounds = max(len(o) for o in offs)
        t0 = min(FIRST_TIE, rounds - 1)
        done = 0
        ks = [[] for _ in range(4)]
        for v in range(rounds):
            if v >= t0:
                upto = (len(items) * (v - t0 + 1)) // (rounds - t0)
                for it in items[done:upto]:
                    it()
                done = upto
            for c in range(4):
                if v < len(offs[c]):
                    ks[c].append(k_ref[pl.ds(base + offs[c][v], 8), :])
        q = q_ref[br, b, g]
        ms = []
        for c in range(4):
            w = _ubf(jnp.concatenate(
                [jnp.where(code == c, q, jnp.uint32(0)), jnp.zeros((8, T), u32)], axis=0))
            s = jnp.dot(_ubf(_cat(ks[c])), w, preferred_element_type=f32)
            if nprev(u, c, first) == WIN:
                sm = jnp.concatenate([jnp.where(tri, s[0:SB], s[SB:2 * SB]), s[2 * SB:]], axis=0)
            else:
                sm = _cat([jnp.where(tri, s[0:SB], NEG), s[SB:]])
            s_ref[pl.ds(zw + c * WIN, sm.shape[0]), :] = sm
            ms.append(jnp.max(sm, axis=0, keepdims=True))
        return ms

    def pv(u, first):
        br, b, g = u
        i = step * NB + b
        p_ref = kp_refs[(g + 1) % 2]
        ntiles = min(3, b + 1) if first else 3
        zero = jnp.zeros((8, T), u32)
        acc = [None] * 4
        for t in range(ntiles):
            pj = [[] for _ in range(4)]
            for r in range(8):
                xs = []
                for c in range(4):
                    nv = (nprev(u, c, first) + SB) // 16
                    v = 8 * t + r - (8 * ntiles - (6 - 2 * c) - nv)
                    xs.append(p_ref[pl.ds(zr + (POFF + c * PROWS + 8 * v), 8), :]
                              if 0 <= v < nv else None)

                def sel(m, a, b_):
                    if a is None and b_ is None:
                        return None
                    return jnp.where(m, zero if a is None else a, zero if b_ is None else b_)
                ts = [sel(odd, xs[(j + 1) % 4], xs[j]) for j in range(4)]
                for j in range(4):
                    y = sel(hi, ts[(j + 2) % 4], ts[j])
                    pj[j].append(zero if y is None else y)
            for j in range(4):
                h = 4 * g + j
                vv = vT_ref[br, i - (ntiles - 1 - t), 16 * h:16 * h + 16, :]
                o = jnp.dot(_ubf(vv), _ubf(jnp.concatenate(pj[j], axis=0)),
                            preferred_element_type=f32)
                acc[j] = o if acc[j] is None else acc[j] + o
        outs = []
        for j in range(4):
            o = acc[j]
            l = o[28:29] if j % 2 == 0 else o[0:1]
            o = o * pl.reciprocal(l, approx=False)
            if j > 0:
                o = pltpu.roll(o, SB * j, 1)
            outs.append(o)
        a, bb, c, d = outs
        og = jnp.concatenate([
            a[0:24], jnp.where(lo4, a[24:32], bb[0:8]), bb[8:32],
            c[0:24], jnp.where(lo4, c[24:32], d[0:8]), d[8:32]], axis=0)
        oT_ref[br, b, 56 * g:56 * g + 56, :] = _pk(og)

    def body(first):
        project(0, xa_ref)
        project(1, xb_ref)
        units = [(br, b, g) for br in range(2) for b in range(NB) for g in range(4)]
        nu = len(units)
        ms = qk(units[0], 0, first, [])
        for n in range(nu):
            items = sm_items(units[n], n, first, ms)
            if n + 1 < nu:
                ms = qk(units[n + 1], n + 1, first, items)
            else:
                for it in items:
                    it()
            if n >= 1:
                pv(units[n - 1], first)
        pv(units[nu - 1], first)
        for b in range(NB):
            oa = jnp.dot(_ubf(woT_ref[0]), _ubf(oT_ref[0, b]), preferred_element_type=f32)
            ob = jnp.dot(_ubf(woT_ref[1]), _ubf(oT_ref[1, b]), preferred_element_type=f32)
            o_ref[b * T:(b + 1) * T, :] = jnp.concatenate([oa, ob], axis=0).astype(bf16).T

    @pl.when(step == 0)
    def _():
        body(True)

    @pl.when(step > 0)
    def _():
        body(False)


@jax.jit
def pallas_concat_heads__sliding_block__sliding_block__prompt_kernel(A_x, A_wqkv, A_wo, B_x, B_wqkv, B_wo):
    xspec = pl.BlockSpec((None, D, TQ), lambda i: (0, 0, i))
    wspec = pl.BlockSpec((D, 3 * D), lambda i: (0, 0))
    wospec = pl.BlockSpec((D, D), lambda i: (0, 0))
    return pl.pallas_call(
        _kernel,
        grid=(S // TQ,),
        in_specs=[xspec, wspec, wospec, xspec, wspec, wospec],
        out_specs=pl.BlockSpec((None, TQ, 2 * D), lambda i: (0, i, 0)),
        out_shape=jax.ShapeDtypeStruct((1, S, 2 * D), bf16),
        scratch_shapes=[
            pltpu.VMEM((2, 3 * D // 2, D), u32),
            pltpu.VMEM((2, D // 2, D), u32),
            pltpu.VMEM((2, NT_, 256, T), u32),
            pltpu.VMEM((2, NB, 4, 56, T), u32),
            pltpu.VMEM((2, NB, D // 2, T), u32),
            pltpu.SMEM((2,), jnp.int32),
            pltpu.VMEM((POFF + 4 * PROWS, T), u32),
            pltpu.VMEM((POFF + 4 * PROWS, T), u32),
        ] + [pltpu.VMEM((4 * WIN, T), f32)] * NSLOT,
        compiler_params=pltpu.CompilerParams(
            dimension_semantics=("arbitrary",),
            vmem_limit_bytes=64 * 1024 * 1024),
        name="swa",
    )(jnp.swapaxes(A_x, 1, 2), A_wqkv, A_wo, jnp.swapaxes(B_x, 1, 2), B_wqkv, B_wo)
```

```python
import functools
import os

import jax
import jax.numpy as jnp
from jax import lax
import jax.experimental.pallas as pl
import jax.experimental.pallas.tpu as pltpu

S, D, H, DH, WIN = 2048, 448, 16, 28, 256
T = 128
NT = S // T
U = int(os.environ.get("U", 4))
NSTEP = 2 + (NT - 4) // U
QSCALE = (DH ** -0.5) * 1.4426950408889634
NEG = -1e30
SB = 32
NR = D // 16
PROWS = 200
ZOFF = 4 * PROWS
MOFF = 4 * WIN
TIE0 = 12
NF = 8
HOPS = int(os.environ.get("HOPS", 1))
E = [int(v) for v in os.environ.get("E", "7,3,12,13,4").split(",")]
Q1T = int(os.environ.get("Q1T", 9))
DH2 = int(os.environ.get("DH2", 0))
XS = int(os.environ.get("XS", 1))

f32, bf16, u32 = jnp.float32, jnp.bfloat16, jnp.uint32


def _pk(x):
    return pltpu.bitcast(x.astype(bf16), u32)


def _ubf(x):
    return pltpu.bitcast(x, bf16)


def _cat(xs):
    xs = [x for x in xs if x.shape[0] > 0]
    return xs[0] if len(xs) == 1 else jnp.concatenate(xs, axis=0)


def _kernel(xa_hbm, wqa_hbm, woa_hbm, xb_hbm, wqb_hbm, wob_hbm, o_hbm,
            x_v, wq_v, wo_v, ob_v, wt_ref, k_ref, vT_ref, q_ref, oT_ref, oa_ref,
            s0_ref, s1_ref, s2_ref, s3_ref, p0_ref, p1_ref, p2_ref, p3_ref,
            qm_ref, cm_ref, tmp_ref, sems):
    step = pl.program_id(0)
    s_refs = (s0_ref, s1_ref, s2_ref, s3_ref)
    p_refs = (p0_ref, p1_ref, p2_ref, p3_ref)

    def w_cp(name):
        src, dst, k = {
            "waq": (wqa_hbm.at[:, 0:256], wq_v.at[0, :, 0:256], 0),
            "waq2": (wqa_hbm.at[:, 256:512], wq_v.at[0, :, 256:512], 1),
            "wak": (wqa_hbm.at[:, 512:896], wq_v.at[0, :, 512:896], 2),
            "wav": (wqa_hbm.at[:, 896:1344], wq_v.at[0, :, 896:1344], 3),
            "wb": (wqb_hbm, wq_v.at[1], 4),
            "woa": (woa_hbm, wo_v.at[0], 5),
            "wob": (wob_hbm, wo_v.at[1], 5),
        }[name]
        return pltpu.make_async_copy(src, dst, sems.at[k])

    xgroups = {
        "xa0": (0, 0, 2, 1), "xa02": (0, 2, 3, 2), "xb0": (1, 0, 2, 4),
        "xb1": (1, 2, 2 + U, 0), "xa1": (0, 3, 3 + U, 0),
        "xb2": (1, 2 + U, NT, 1 + 5 * XS), "xa2": (0, 3 + U, NT, 1 + 5 * XS),
    }

    def start(*names):
        for name in names:
            if name in xgroups:
                br, t0, t1, k = xgroups[name]
                for t in range(t0, t1):
                    pltpu.make_async_copy((xa_hbm, xb_hbm)[br].at[0, :, t * T:(t + 1) * T],
                                          x_v.at[br, t], sems.at[k]).start()
            else:
                w_cp(name).start()

    def wait(*names):
        for name in names:
            if name in xgroups:
                br, t0, t1, k = xgroups[name]
                pltpu.make_async_copy(x_v.at[br, t0:t1], x_v.at[br, t0:t1], sems.at[k]).wait()
            else:
                w_cp(name).wait()

    def out_cp(row0, nrows, c0=0, c1=2 * D):
        return pltpu.make_async_copy(ob_v.at[pl.ds(row0, nrows), c0:c1],
                                     o_hbm.at[0, pl.ds(row0, nrows), c0:c1], sems.at[2])

    @pl.when(step == 0)
    def _():
        start("waq", "xa0", "waq2", "xa02", "wak", "wav", "wb", "xb0", "woa", "wob")
        row = lax.broadcasted_iota(jnp.int32, (64, T), 0)
        col = lax.broadcasted_iota(jnp.int32, (64, T), 1)
        real = jnp.logical_or((row & 31) < 14, (row & 31) >= 18)
        code = ((row >> 4) + (col >> 5)) & 3
        for c in range(4):
            qm_ref[c] = jnp.where(jnp.logical_and(real, code == c),
                                  jnp.uint32(0xFFFFFFFF), jnp.uint32(0))
            qpos = (col + SB * c) & (T - 1)
            cm_ref[c] = (jnp.where(2 * row <= qpos, jnp.uint32(0xFFFF), jnp.uint32(0))
                         | jnp.where(2 * row + 1 <= qpos, jnp.uint32(0xFFFF0000), jnp.uint32(0)))
            p_refs[c][ZOFF:ZOFF + 8, :] = jnp.zeros((8, T), u32)
        vT_ref[1, 0, 128:256, :] = jnp.zeros((128, T), u32)

    zs = (pl.multiple_of((step >> 10) * 16, 16), pl.multiple_of((step >> 11) * 16, 16))
    zw, zr = zs

    lane8 = lax.broadcasted_iota(jnp.int32, (8, T), 1)
    tri = (lax.broadcasted_iota(jnp.int32, (SB, T), 0)
           <= (lax.broadcasted_iota(jnp.int32, (SB, T), 1) & (SB - 1)))
    odd = (lane8 & SB) != 0
    hi = lane8 >= 2 * SB
    zero8 = jnp.zeros((8, T), u32)

    def ties(items, nrounds, t0, t1):
        out = []
        done = 0
        for v in range(nrounds):
            zv = None
            if t0 <= v < t1:
                upto = (len(items) * (v - t0 + 1)) // (t1 - t0)
                if upto > done:
                    gs = sorted({it() for it in items[done:upto]})
                    done = upto
                    zv = functools.reduce(
                        jnp.bitwise_or, [p_refs[g][ZOFF:ZOFF + 8, :] for g in gs])
                    for h in range(HOPS):
                        tmp_ref[8 * h:8 * h + 8, :] = zv
                        zv = tmp_ref[8 * h:8 * h + 8, :]
            out.append(zv)
        return out

    def pad_heads(a, fill=None):
        parts = []
        for p in range(H // 2):
            b = a[56 * p:56 * p + 56]
            mid = b[24:32]
            if fill is None:
                parts += [b[0:32], b[24:56]]
            else:
                m = lax.broadcasted_iota(jnp.int32, mid.shape, 0) < 4
                parts += [b[0:24], jnp.where(m, mid, fill), jnp.where(m, fill, mid), b[32:56]]
        return jnp.concatenate(parts, axis=0)

    def roll_heads(a, back):
        parts = []
        for h in range(a.shape[0] // 16):
            j = h % 4
            b = a[16 * h:16 * h + 16]
            parts.append(b if j == 0 else pltpu.roll(b, SB * j if back else T - SB * j, 1))
        return jnp.concatenate(parts, axis=0)

    def moff(i, n):
        return i * n if isinstance(i, int) else pl.multiple_of(i * n, n)

    def prep_w(br, c0, c1):
        w = jnp.concatenate([wq_v[br, :, c0:c1], jnp.zeros((64, c1 - c0), bf16)], axis=0)
        wt_ref[br, c0 // 2:c1 // 2, :] = pltpu.bitcast(w.T, u32)

    def prep_wo(br):
        w = pad_heads(wo_v[br].astype(f32), 0.0).astype(bf16)
        wt_ref[br, 3 * D // 2:2 * D, :] = pltpu.bitcast(w.T, u32)

    def project(br, part, rhs, items, t0, mid):
        zv = ties(items, NR, t0, NR)
        rows = []
        for v in range(NR):
            r = 8 * (part * NR + v)
            w = wt_ref[br, r:r + 8, :]
            if zv[v] is not None:
                w = w | jnp.concatenate([zv[v]] * 4, axis=1)
            rows.append(w)
        y = jnp.dot(_ubf(jnp.concatenate(rows, axis=0)), rhs, preferred_element_type=f32)
        if mid:
            wait(*mid)
        return y

    def xtile(br, i):
        return jnp.concatenate([x_v[br, i], jnp.zeros((64, T), bf16)], axis=0)

    def proj_q(br, i, items=(), t0=TIE0, slot=None, mid=None):
        qT = project(br, 0, xtile(br, i), items, t0, mid) * QSCALE
        q_ref[br if slot is None else slot] = roll_heads(_pk(pad_heads(qT)), False)

    def proj_k(br, i, items=(), t0=TIE0):
        kT = pad_heads(project(br, 1, xtile(br, i), items, t0, None))
        for gp in range(2):
            kt = pltpu.bitcast(kT[2 * T * gp:2 * T * (gp + 1)].astype(bf16).T, u32)
            for gg in range(2):
                k_ref[br, 2 * gp + gg, pl.ds(moff(i, 64), 64), :] = kt[:, T * gg:T * (gg + 1)]

    def proj_v(br, i, items=(), t0=TIE0, mid=None):
        vT = project(br, 2, xtile(br, i), items, t0, mid)
        vT_ref[br, i + 1] = _pk(pad_heads(vT, 1.0))

    def proj_o(br, i, items=(), t0=TIE0, slot=None, aslot=0):
        o = project(br, 3, _ubf(oT_ref[br if slot is None else slot]), items, t0, None)
        row0 = moff(i, T)
        if br == 0:
            ob_v[pl.ds(row0, T), 0:384] = o[0:384].astype(bf16).T
            oa_ref[aslot] = o[384:448]
        else:
            ob_v[pl.ds(row0, T), 384:896] = jnp.concatenate(
                [oa_ref[aslot], o], axis=0).astype(bf16).T

    def ntiles(i):
        return min(3, i + 1) if isinstance(i, int) else 3

    def qk(br, i, g, items=(), t0=1, t1=18, zero_fill=False, slot=None, col=0,
           late=False, extra=None):
        s_ref, p_ref = s_refs[g], p_refs[g]
        nt = ntiles(i)
        late = late or nt < 3
        base = moff(i, 64)
        zv = ties(items, 18, t0, t1)
        if extra is not None:
            zv[17] = extra if zv[17] is None else zv[17] | extra
        q = q_ref[br if slot is None else slot, 64 * g:64 * g + 64, :]
        ms = [None] * 4
        for c in (range(4) if g % 2 == 0 else range(3, -1, -1)):
            npv = WIN if nt == 3 else i * T + SB * c
            offs = [16 * c, 16 * c + 8] + [16 * c - npv // 2 + 8 * v for v in range(npv // 16)]
            ks = []
            for v, off in enumerate(offs):
                kv = k_ref[br, g, pl.ds(base + off, 8), :]
                ks.append(kv if zv[v] is None else kv | zv[v])
            s = jnp.dot(_ubf(_cat(ks)), _ubf(q & qm_ref[c]), preferred_element_type=f32)
            if nt == 3:
                dg, rest = jnp.where(tri, s[0:SB], s[SB:2 * SB]), s[2 * SB:]
            else:
                dg, rest = jnp.where(tri, s[0:SB], NEG), s[SB:]
            nr = rest.shape[0] - SB * c
            s_ref[pl.ds(zw + (c * WIN + SB * c), SB), :] = dg
            if c > 0:
                s_ref[pl.ds(zw + c * WIN, SB * c), :] = rest[nr:]
            if nr > 0:
                s_ref[pl.ds(zw + (c * WIN + WIN - nr), nr), :] = rest[:nr]
            ms[c] = jnp.max(_cat([dg, rest]), axis=0, keepdims=True)
            if late:
                s_ref[pl.ds(zw + (MOFF + 8 * c), 8), :] = jnp.broadcast_to(ms[c], (8, T))

        def put(j, r, y):
            p_ref[pl.ds(zs[col] + (j * PROWS + 8 * r), 8), :] = y

        def sel(m, a, b):
            if a is None and b is None:
                return None
            return jnp.where(m, zero8 if a is None else a, zero8 if b is None else b)

        def item(rho):
            xs = []
            for c in range(4):
                if nt < 3 and rho < 8 and c < rho // 2:
                    xs.append(None)
                    continue
                s = s_ref[pl.ds(zr + (c * WIN + 16 * rho), 16), :]
                if late:
                    m = s_ref[pl.ds(zr + (MOFF + 8 * c), 8), :]
                    m = jnp.concatenate([m, m], axis=0)
                else:
                    m = ms[c]
                xs.append(_pk(jnp.exp2(s - m)))
            ts = [sel(odd, xs[(j + 1) % 4], xs[j]) for j in range(4)]
            for j in range(4):
                y = sel(hi, ts[(j + 2) % 4], ts[j])
                if rho >= 8 or nt == 1:
                    put(j, rho, y)
                elif nt == 3:
                    new = y & cm_ref[j, 8 * rho:8 * rho + 8, :]
                    put(j, rho + 16, new)
                    put(j, rho, y ^ new)
                else:
                    put(j, rho + 16, y)
                    if zero_fill:
                        put(j, rho, zero8)
            return g
        order = list(range(8, 16 if nt > 1 else 8)) + list(range(8))
        return [functools.partial(item, rho) for rho in order]

    def pv(br, i, g, items=(), slot=None, col=0):
        nt = ntiles(i)
        zv = ties(items, 6, 0, 6)
        acc = [None] * 4
        for t in range(3 - nt, 3):
            for j in range(4):
                h = 4 * g + j
                vv = vT_ref[br, i - 1 + t, 16 * h:16 * h + 16, :]
                vv = jnp.concatenate(
                    [vv[8 * e:8 * e + 8] if zv[2 * t + e] is None
                     else vv[8 * e:8 * e + 8] | zv[2 * t + e] for e in range(2)], axis=0)
                r = j * PROWS + (0 if nt == 1 else 64 * t)
                pj = p_refs[g][pl.ds(zs[1 - col] + r, 64), :]
                o = jnp.dot(_ubf(vv), _ubf(pj), preferred_element_type=f32)
                acc[j] = o if acc[j] is None else acc[j] + o
        og = jnp.concatenate(
            [acc[j] * pl.reciprocal(acc[j][28:29] if j % 2 == 0 else acc[j][0:1], approx=False)
             for j in range(4)], axis=0)
        oT_ref[br if slot is None else slot, 64 * g:64 * g + 64, :] = roll_heads(_pk(og), True)

    def half(br, i, nxt, fin, left, flush):
        ob = 1 - br
        for g in range(4):
            items = qk(br, i, g, left)
            n = len(items) if flush and g == 3 else NF
            items, left = items[:n], items[n:]
            if g > 1:
                pv(br, i, g - 2)
            else:
                pv(ob, fin, g + 2)
            if g == 2:
                proj_o(ob, fin, items)
            else:
                (proj_k, proj_q, None, proj_v)[g](ob, nxt, items)
        return left

    def period(i, left, flush):
        left = half(0, i, i, i - 1, left, False)
        return half(1, i, i + 1, i, left, flush)

    @pl.when(step == 0)
    def _():
        wait("waq")
        prep_w(0, 0, 256)
        if XS == 1:
            start("xb1", "xa1", "xb2", "xa2")
        wait("xa0", "waq2")
        prep_w(0, 256, 512)
        proj_q(0, 0, slot=2)
        proj_q(0, 1, slot=3, mid=("xa02", "wak"))
        if XS == 0:
            start("xb1", "xa1", "xb2", "xa2")
        prep_w(0, 512, 896)
        proj_q(0, 2)
        proj_k(0, 0)
        proj_k(0, 1)
        it = sum([qk(0, 0, g, slot=2, col=1) for g in range(4)], [])
        proj_k(0, 2, it, 4)
        it0 = qk(0, 1, 0, slot=3)
        it1 = qk(0, 1, 1, slot=3)
        wait("wav")
        prep_w(0, 896, 1344)
        it2 = qk(0, 1, 2, it0[:8], 1, 10, slot=3)
        it3 = qk(0, 1, 3, it0[8:], 1, 10, slot=3)
        proj_v(0, 0, it1, 1)
        proj_v(0, 1, it2, 1, mid=("wb", "xb0"))
        prep_w(1, 384, 896)
        prep_w(1, 0, 384)
        prep_w(1, 896, 1344)
        for g in range(4):
            pv(0, 0, g, slot=2, col=1)
        for g in range(3):
            pv(0, 1, g)
        proj_k(1, 0, it3, 1)
        proj_q(1, 0, slot=2)
        proj_k(1, 1)
        it = sum([qk(1, 0, g, slot=2, col=1) for g in range(4)], [])
        pv(0, 1, 3)
        proj_q(1, 1, it, 1)
        proj_v(1, 0, mid=("woa", "wob"))
        prep_wo(0)
        prep_wo(1)
        it0 = qk(1, 1, 0)
        it1 = qk(1, 1, 1)
        for g in range(4):
            pv(1, 0, g, slot=3, col=1)
        proj_v(1, 1, it0, 1)
        proj_o(0, 0, it1, 1, slot=2, aslot=1)
        proj_o(1, 0, slot=3, aslot=1)
        it0 = qk(1, 1, 2, zero_fill=True)
        it1 = qk(1, 1, 3, zero_fill=True)
        pv(1, 1, 0)
        pv(1, 1, 1)
        proj_o(0, 1, it0, 1)
        proj_v(0, 2, it1, 1)
        wait("xb1", "xa1")
        out_cp(0, T).start()

    @pl.when(jnp.logical_and(step > 0, step < NSTEP - 1))
    def _():
        left = ()
        i0 = 2 + (step - 1) * U
        for b in range(U):
            left = period(i0 + b, left, b == U - 1)
        out_cp(pl.multiple_of((i0 - 1) * T, T), U * T).start()

    @pl.when(step == 1)
    def _():
        wait("xb2", "xa2")

    @pl.when(step == NSTEP - 1)
    def _():
        i = NT - 1
        r0 = i * T
        left = period(i - 1, (), False)
        left = half(0, i, i, i - 1, left, False)
        out_cp((NT - 3) * T, 2 * T).start()
        def dma_tie(hops=0):
            ob_v[pl.ds(zw + r0, 16), 512:640] = jnp.zeros((16, T), bf16)
            z = pltpu.bitcast(ob_v[pl.ds(zr + r0, 16), 512:640], u32)
            for h in range(hops):
                tmp_ref[32 + 8 * h:40 + 8 * h, :] = z
                z = tmp_ref[32 + 8 * h:40 + 8 * h, :]
            return z
        zd = dma_tie()

        def o_part(g, extra=None):
            sets = ([4, 5, 6, 7, 8, 9, 10], [12, 13, 14, 15, 16, 17, 18],
                    [20, 21, 22, 23, 24, 25, 26], [0, 1, 2, 3, 11, 19, 27])
            w = wt_ref[1, 3 * D // 2:2 * D, T * g:T * (g + 1)]
            rhs = oT_ref[1, 64 * g:64 * g + 64, :]
            if extra is not None:
                rhs = jnp.concatenate([rhs[0:8] | extra, rhs[8:]], axis=0)
            rhs = _ubf(rhs)
            res = {}
            for rows in sets:
                lhs = jnp.concatenate([w[8 * v:8 * v + 8] for v in rows], axis=0)
                y = jnp.dot(_ubf(lhs), rhs, preferred_element_type=f32)
                for n, v in enumerate(rows):
                    res[v] = y[16 * n:16 * n + 16]
            return jnp.concatenate([res[v] for v in range(NR)], axis=0)

        it = qk(1, i, 0, left, late=True, extra=zd)
        pv(0, i, 2)
        it = it[E[0]:] + qk(1, i, 1, it[:E[0]], Q1T, late=True)
        pv(0, i, 3, it[:E[1]])
        it = it[E[1]:]
        it = it[E[2]:] + qk(1, i, 2, it[:E[2]], 0, late=True)
        it = it[E[3]:] + qk(1, i, 3, it[:E[3]], 0, late=True)
        proj_o(0, i, it[:len(it) - E[4]], 0)
        out_cp(r0, T, 0, 384).start()
        zd = dma_tie(DH2)
        pv(1, i, 0, it[len(it) - E[4]:])
        for g in range(1, 4):
            pv(1, i, g)
        o = o_part(0) + o_part(1) + o_part(2) + o_part(3, zd)
        ot = jnp.concatenate([oa_ref[0], o], axis=0).astype(bf16).T
        for a, b in ((0, 64), (64, 96), (96, 128)):
            ob_v[r0 + a:r0 + b, 384:896] = ot[a:b]
            out_cp(r0 + a, b - a, 384, 896).start()
        out_cp(0, S).wait()


@jax.jit
def pallas_concat_heads__sliding_block__sliding_block__prompt_kernel(A_x, A_wqkv, A_wo, B_x, B_wqkv, B_wo):
    anyspec = pl.BlockSpec(memory_space=pl.ANY)
    return pl.pallas_call(
        _kernel,
        grid=(NSTEP,),
        in_specs=[anyspec] * 6,
        out_specs=anyspec,
        out_shape=jax.ShapeDtypeStruct((1, S, 2 * D), bf16),
        scratch_shapes=[
            pltpu.VMEM((2, NT, D, T), bf16),
            pltpu.VMEM((2, D, 3 * D), bf16),
            pltpu.VMEM((2, D, D), bf16),
            pltpu.VMEM((S, 2 * D), bf16),
            pltpu.VMEM((2, 2 * D, 4 * T), u32),
            pltpu.VMEM((2, 4, S // 2, T), u32),
            pltpu.VMEM((2, NT + 1, 256, T), u32),
            pltpu.VMEM((4, 256, T), u32),
            pltpu.VMEM((4, 256, T), u32),
            pltpu.VMEM((2, 64, T), f32),
        ] + [pltpu.VMEM((MOFF + 32, T), f32)] * 4
        + [pltpu.VMEM((ZOFF + 32, T), u32)] * 4
        + [
            pltpu.VMEM((4, 64, T), u32),
            pltpu.VMEM((4, 64, T), u32),
            pltpu.VMEM((256, T), u32),
            pltpu.SemaphoreType.DMA((6 + XS,)),
        ],
        compiler_params=pltpu.CompilerParams(
            dimension_semantics=("arbitrary",),
            vmem_limit_bytes=64 * 1024 * 1024),
        name="swa",
    )(jnp.swapaxes(A_x, 1, 2), A_wqkv, A_wo, jnp.swapaxes(B_x, 1, 2), B_wqkv, B_wo)
```

```python
import functools

import jax
import jax.numpy as jnp
from jax import lax
import jax.experimental.pallas as pl
import jax.experimental.pallas.tpu as pltpu

S, D, H, DH, WIN = 2048, 448, 16, 28, 256
T = 128
NT = S // T
U = 4
NSTEP = 2 + (NT - 4) // U
QSCALE = (DH ** -0.5) * 1.4426950408889634
NEG = -1e30
SB = 32
NR = D // 16
ZP = 24
MS = 16
TIE0 = 12
NF = 8
HOPS = 2

f32, bf16, u32 = jnp.float32, jnp.bfloat16, jnp.uint32


def _pk(x):
    return pltpu.bitcast(x.astype(bf16), u32)


def _ubf(x):
    return pltpu.bitcast(x, bf16)


def _cat(xs):
    xs = [x for x in xs if x.shape[0] > 0]
    return xs[0] if len(xs) == 1 else jnp.concatenate(xs, axis=0)


def _kernel(xa_hbm, wqa_hbm, woa_hbm, xb_hbm, wqb_hbm, wob_hbm, o_hbm,
            x_v, wq_v, wo_v, ob_v, wt_ref, k_ref, vT_ref, q_ref, oT_ref, oa_ref,
            s0_ref, s1_ref, s2_ref, s3_ref, p0_ref, p1_ref, p2_ref, p3_ref,
            qm_ref, cm_ref, tmp_ref, sems):
    step = pl.program_id(0)
    s_refs = (s0_ref, s1_ref, s2_ref, s3_ref)
    p_refs = (p0_ref, p1_ref, p2_ref, p3_ref)

    def w_cp(name):
        src, dst, k = {
            "waq": (wqa_hbm.at[:, 0:256], wq_v.at[0, :, 0:256], 0),
            "waq2": (wqa_hbm.at[:, 256:512], wq_v.at[0, :, 256:512], 1),
            "wak": (wqa_hbm.at[:, 512:896], wq_v.at[0, :, 512:896], 2),
            "wav": (wqa_hbm.at[:, 896:1344], wq_v.at[0, :, 896:1344], 3),
            "wb": (wqb_hbm, wq_v.at[1], 4),
            "woa": (woa_hbm, wo_v.at[0], 5),
            "wob": (wob_hbm, wo_v.at[1], 5),
        }[name]
        return pltpu.make_async_copy(src, dst, sems.at[k])

    xgroups = {
        "xa0": (0, 0, 2, 7), "xa02": (0, 2, 3, 1), "xb0": (1, 0, 2, 4),
        "xb1": (1, 2, 2 + U, 0), "xa1": (0, 3, 3 + U, 0),
        "xb2": (1, 2 + U, NT, 6), "xa2": (0, 3 + U, NT, 6),
    }

    def start(*names):
        for name in names:
            if name in xgroups:
                br, t0, t1, k = xgroups[name]
                for t in range(t0, t1):
                    pltpu.make_async_copy((xa_hbm, xb_hbm)[br].at[0, :, t * T:(t + 1) * T],
                                          x_v.at[br, t], sems.at[k]).start()
            else:
                w_cp(name).start()

    def wait(*names):
        for name in names:
            if name in xgroups:
                br, t0, t1, k = xgroups[name]
                pltpu.make_async_copy(x_v.at[br, t0:t1], x_v.at[br, t0:t1], sems.at[k]).wait()
            else:
                w_cp(name).wait()

    def out_cp(row0, nrows, c0=0, c1=2 * D):
        return pltpu.make_async_copy(ob_v.at[pl.ds(row0, nrows), c0:c1],
                                     o_hbm.at[0, pl.ds(row0, nrows), c0:c1], sems.at[2])

    @pl.when(step == 0)
    def _():
        start("waq", "xa0", "waq2", "xa02", "wak", "wav", "wb", "xb0", "woa", "wob")
        row = lax.broadcasted_iota(jnp.int32, (64, T), 0)
        col = lax.broadcasted_iota(jnp.int32, (64, T), 1)
        real = jnp.logical_or((row & 31) < 14, (row & 31) >= 18)
        code = ((row >> 4) + (col >> 5)) & 3
        for c in range(4):
            qm_ref[c] = jnp.where(jnp.logical_and(real, code == c),
                                  jnp.uint32(0xFFFFFFFF), jnp.uint32(0))
            qpos = (col + SB * c) & (T - 1)
            cm = (jnp.where(2 * row <= qpos, jnp.uint32(0xFFFF), jnp.uint32(0))
                  | jnp.where(2 * row + 1 <= qpos, jnp.uint32(0xFFFF0000), jnp.uint32(0)))
            cm_ref[:, 8 * c:8 * c + 8, :] = cm.reshape(8, 8, T)
            p_refs[c][ZP] = jnp.zeros((32, T), u32)
        vT_ref[1, 0, 128:256, :] = jnp.zeros((128, T), u32)

    zs = (step >> 10, step >> 11)
    zw, zr = zs

    lane = lax.broadcasted_iota(jnp.int32, (SB, T), 1)
    tri = lax.broadcasted_iota(jnp.int32, (SB, T), 0) <= (lane & (SB - 1))
    odd = (lane & SB) != 0
    hi = lane >= 2 * SB
    zero8 = jnp.zeros((8, T), u32)

    def ties(items, nrounds, t0, t1):
        out = []
        done = 0
        for v in range(nrounds):
            zv = None
            if t0 <= v < t1:
                upto = (len(items) * (v - t0 + 1)) // (t1 - t0)
                if upto > done:
                    gs = sorted({it() for it in items[done:upto]})
                    done = upto
                    zv = functools.reduce(
                        jnp.bitwise_or, [p_refs[g][ZP, 0:8, :] for g in gs])
                    for h in range(HOPS):
                        tmp_ref[8 * h:8 * h + 8, :] = zv
                        zv = tmp_ref[8 * h:8 * h + 8, :]
            out.append(zv)
        return out

    def stack(zv):
        if all(z is None for z in zv):
            return None
        return jnp.concatenate([zero8 if z is None else z for z in zv], axis=0)

    def pad_heads(a, fill=None):
        parts = []
        for p in range(a.shape[0] // 56):
            b = a[56 * p:56 * p + 56]
            mid = b[24:32]
            if fill is None:
                parts += [b[0:32], b[24:56]]
            else:
                m = lax.broadcasted_iota(jnp.int32, mid.shape, 0) < 4
                parts += [b[0:24], jnp.where(m, mid, fill), jnp.where(m, fill, mid), b[32:56]]
        return jnp.concatenate(parts, axis=0)

    def roll_heads(a, back):
        parts = []
        for h in range(a.shape[0] // 16):
            j = h % 4
            b = a[16 * h:16 * h + 16]
            parts.append(b if j == 0 else pltpu.roll(b, SB * j if back else T - SB * j, 1))
        return jnp.concatenate(parts, axis=0)

    def moff(i, n):
        return i * n if isinstance(i, int) else pl.multiple_of(i * n, n)

    def prep_w(br, c0, c1):
        w = jnp.concatenate([wq_v[br, :, c0:c1], jnp.zeros((64, c1 - c0), bf16)], axis=0)
        wt_ref[br, c0 // 2:c1 // 2, :] = pltpu.bitcast(w.T, u32)

    def prep_wo(br):
        w = pad_heads(wo_v[br].astype(f32), 0.0).astype(bf16)
        wt_ref[br, 3 * D // 2:2 * D, :] = pltpu.bitcast(w.T, u32)

    def project(br, part, rhs, items, t0, mid):
        zv = stack(ties(items, NR, t0, NR))
        w = wt_ref[br, part * (D // 2):(part + 1) * (D // 2), :]
        if zv is not None:
            w = w | jnp.concatenate([zv] * 4, axis=1)
        y = jnp.dot(_ubf(w), rhs, preferred_element_type=f32)
        if mid:
            wait(*mid)
        return y

    def xtile(br, i):
        return jnp.concatenate([x_v[br, i], jnp.zeros((64, T), bf16)], axis=0)

    def proj_q(br, i, items=(), t0=TIE0, slot=None):
        qT = project(br, 0, xtile(br, i), items, t0, None) * QSCALE
        q_ref[br if slot is None else slot] = roll_heads(_pk(pad_heads(qT)), False)

    def proj_q_half(i, hf, slot, mid=None):
        y = jnp.dot(_ubf(wt_ref[0, 112 * hf:112 * hf + 112, :]), xtile(0, i),
                    preferred_element_type=f32)
        if mid:
            wait(*mid)
        q_ref[slot, T * hf:T * hf + T, :] = roll_heads(_pk(pad_heads(y * QSCALE)), False)

    def proj_k(br, i, items=(), t0=TIE0):
        kT = pad_heads(project(br, 1, xtile(br, i), items, t0, None))
        for gp in range(2):
            kt = pltpu.bitcast(kT[2 * T * gp:2 * T * (gp + 1)].astype(bf16).T, u32)
            for gg in range(2):
                k_ref[br, 2 * gp + gg, pl.ds(moff(i, 64), 64), :] = kt[:, T * gg:T * (gg + 1)]

    def proj_v(br, i, items=(), t0=TIE0, mid=None):
        vT = project(br, 2, xtile(br, i), items, t0, mid)
        vT_ref[br, i + 1] = _pk(pad_heads(vT, 1.0))

    def proj_o(br, i, items=(), t0=TIE0, slot=None, aslot=0):
        o = project(br, 3, _ubf(oT_ref[br if slot is None else slot]), items, t0, None)
        row0 = moff(i, T)
        if br == 0:
            ob_v[pl.ds(row0, T), 0:384] = o[0:384].astype(bf16).T
            oa_ref[aslot] = o[384:448]
        else:
            ob_v[pl.ds(row0, T), 384:896] = jnp.concatenate(
                [oa_ref[aslot], o], axis=0).astype(bf16).T

    def ntiles(i):
        return min(3, i + 1) if isinstance(i, int) else 3

    def qk(br, i, g, items=(), t0=1, t1=18, zero_fill=False, slot=None, col=0,
           late=False, extra=None):
        s_ref, p_ref = s_refs[g], p_refs[g]
        nt = ntiles(i)
        late = late or nt < 3
        zv = ties(items, 18, t0, t1)
        if extra is not None:
            zv[17] = extra if zv[17] is None else zv[17] | extra
        zv = stack(zv)
        q = q_ref[br if slot is None else slot, 64 * g:64 * g + 64, :]
        ms = [None] * 4
        for c in (range(4) if g % 2 == 0 else range(3, -1, -1)):
            n = min(WIN // 2, 64 * (nt - 1) + 16 * c)
            ks = k_ref[br, g, pl.ds(moff(i, 64) + (16 * c - n), n + 16), :]
            if n > 0:
                ks = jnp.concatenate([ks[n:], ks[:n]], axis=0)
            if zv is not None:
                ks = ks | (zv if nt == 3 else zv[:n + 16])
            s = jnp.dot(_ubf(ks), _ubf(q & qm_ref[c]), preferred_element_type=f32)
            if nt == 3:
                dg, rest = jnp.where(tri, s[0:SB], s[SB:2 * SB]), s[2 * SB:]
            else:
                dg, rest = jnp.where(tri, s[0:SB], NEG), s[SB:]
            nr = rest.shape[0] - SB * c
            cs = slice(16 * c, 16 * c + 16)
            s_ref[pl.ds(zw, 2 * c + 2), cs, :] = _cat([rest[nr:], dg]).reshape(2 * c + 2, 16, T)
            if nr > 0:
                s_ref[pl.ds(zw + (16 - nr // 16), nr // 16), cs, :] = (
                    rest[:nr].reshape(nr // 16, 16, T))
            ms[c] = jnp.broadcast_to(jnp.max(_cat([dg, rest]), axis=0, keepdims=True), (8, T))
            if late:
                s_ref[zw + MS, 8 * c:8 * c + 8, :] = ms[c]

        mall = None if late else jnp.concatenate([m for m in ms for _ in range(2)], axis=0)

        def item(rho):
            c0 = rho // 2 if nt < 3 and rho < 8 else 0
            if late:
                m = jnp.concatenate([s_ref[zr + MS, 8 * c0:32, :].reshape(4 - c0, 8, T)] * 2,
                                    axis=1).reshape(16 * (4 - c0), T)
            else:
                m = mall
            x = _pk(jnp.exp2(s_ref[zr + rho, 16 * c0:64, :] - m))
            if c0 > 0:
                x = jnp.concatenate([jnp.zeros((8 * c0, T), u32), x], axis=0)
            x = lax.select(odd, jnp.concatenate([x[8:], x[:8]], axis=0), x)
            y = lax.select(hi, jnp.concatenate([x[16:], x[:16]], axis=0), x)
            z = zs[col]
            if rho >= 8 or nt == 1:
                p_ref[z + rho] = y
            elif nt == 3:
                new = y & cm_ref[rho]
                p_ref[z + (rho + 16)] = new
                p_ref[z + rho] = y ^ new
            else:
                p_ref[z + (rho + 16)] = y
                if zero_fill:
                    p_ref[z + rho] = jnp.zeros((32, T), u32)
            return g
        order = list(range(8, 16 if nt > 1 else 8)) + list(range(8))
        return [functools.partial(item, rho) for rho in order]

    def pv(br, i, g, items=(), slot=None, col=0):
        nt = ntiles(i)
        zv = ties(items, 6, 0, 6)
        acc = [None] * 4
        for t in range(3 - nt, 3):
            vv = vT_ref[br, i - 1 + t, 64 * g:64 * g + 64, :]
            zt = stack(zv[2 * t:2 * t + 2] * 4)
            vv = _ubf(vv if zt is None else vv | zt)
            pp = p_refs[g][pl.ds(zs[1 - col] + (0 if nt == 1 else 8 * t), 8)]
            for j in range(4):
                pj = pp[:, 8 * j:8 * j + 8, :].reshape(64, T)
                o = jnp.dot(vv[32 * j:32 * j + 32], _ubf(pj), preferred_element_type=f32)
                acc[j] = o if acc[j] is None else acc[j] + o
        og = jnp.concatenate(
            [acc[j] * pl.reciprocal(acc[j][28:29] if j % 2 == 0 else acc[j][0:1], approx=False)
             for j in range(4)], axis=0)
        oT_ref[br if slot is None else slot, 64 * g:64 * g + 64, :] = roll_heads(_pk(og), True)

    def half(br, i, nxt, fin, left, flush):
        ob = 1 - br
        for g in range(4):
            items = qk(br, i, g, left)
            n = len(items) if flush and g == 3 else NF
            items, left = items[:n], items[n:]
            if g > 1:
                pv(br, i, g - 2)
            else:
                pv(ob, fin, g + 2)
            if g == 2:
                proj_o(ob, fin, items)
            else:
                (proj_k, proj_q, None, proj_v)[g](ob, nxt, items)
        return left

    def period(i, left, flush):
        left = half(0, i, i, i - 1, left, False)
        return half(1, i, i + 1, i, left, flush)

    @pl.when(step == 0)
    def _():
        wait("waq")
        prep_w(0, 0, 256)
        start("xb1", "xa1", "xb2", "xa2")
        wait("xa0")
        proj_q_half(0, 0, 2)
        proj_q_half(1, 0, 3, mid=("waq2", "xa02"))
        prep_w(0, 256, 512)
        proj_q_half(2, 0, 0)
        proj_q_half(0, 1, 2)
        proj_q_half(1, 1, 3, mid=("wak",))
        prep_w(0, 512, 896)
        proj_q_half(2, 1, 0)
        proj_k(0, 0)
        proj_k(0, 1)
        it = sum([qk(0, 0, g, slot=2, col=1) for g in range(4)], [])
        proj_k(0, 2, it, 4)
        it0 = qk(0, 1, 0, slot=3)
        it1 = qk(0, 1, 1, slot=3)
        wait("wav")
        prep_w(0, 896, 1344)
        it2 = qk(0, 1, 2, it0[:8], 1, 10, slot=3)
        it3 = qk(0, 1, 3, it0[8:], 1, 10, slot=3)
        proj_v(0, 0, it1, 1)
        proj_v(0, 1, it2, 1, mid=("wb", "xb0"))
        prep_w(1, 384, 896)
        prep_w(1, 0, 384)
        prep_w(1, 896, 1344)
        for g in range(4):
            pv(0, 0, g, slot=2, col=1)
        for g in range(3):
            pv(0, 1, g)
        proj_k(1, 0, it3, 1)
        proj_q(1, 0, slot=2)
        proj_k(1, 1)
        it = sum([qk(1, 0, g, slot=2, col=1) for g in range(4)], [])
        pv(0, 1, 3)
        proj_q(1, 1, it, 1)
        proj_v(1, 0, mid=("woa", "wob"))
        prep_wo(0)
        prep_wo(1)
        it0 = qk(1, 1, 0)
        it1 = qk(1, 1, 1)
        for g in range(4):
            pv(1, 0, g, slot=3, col=1)
        proj_v(1, 1, it0, 1)
        proj_o(0, 0, it1, 1, slot=2, aslot=1)
        proj_o(1, 0, slot=3, aslot=1)
        it0 = qk(1, 1, 2, zero_fill=True)
        it1 = qk(1, 1, 3, zero_fill=True)
        pv(1, 1, 0)
        pv(1, 1, 1)
        proj_o(0, 1, it0, 1)
        proj_v(0, 2, it1, 1)
        wait("xb1", "xa1")
        out_cp(0, T).start()

    @pl.when(jnp.logical_and(step > 0, step < NSTEP - 1))
    def _():
        left = ()
        i0 = 2 + (step - 1) * U
        for b in range(U):
            left = period(i0 + b, left, b == U - 1)
        out_cp(pl.multiple_of((i0 - 1) * T, T), U * T).start()

    @pl.when(step == 1)
    def _():
        wait("xb2", "xa2")

    @pl.when(step == NSTEP - 1)
    def _():
        i = NT - 1
        r0 = i * T
        left = period(i - 1, (), False)
        left = half(0, i, i, i - 1, left, False)
        out_cp((NT - 3) * T, 2 * T).start()

        def dma_tie():
            ob_v[pl.ds(moff(zw, 16) + r0, 16), 512:640] = jnp.zeros((16, T), bf16)
            return pltpu.bitcast(ob_v[pl.ds(moff(zr, 16) + r0, 16), 512:640], u32)

        def o_part(g, extra=None):
            sets = ([4, 5, 6, 7, 8, 9, 10], [12, 13, 14, 15, 16, 17, 18],
                    [20, 21, 22, 23, 24, 25, 26], [0, 1, 2, 3, 11, 19, 27])
            w = wt_ref[1, 3 * D // 2:2 * D, T * g:T * (g + 1)]
            rhs = oT_ref[1, 64 * g:64 * g + 64, :]
            if extra is not None:
                rhs = jnp.concatenate([rhs[0:8] | extra, rhs[8:]], axis=0)
            rhs = _ubf(rhs)
            res = {}
            for rows in sets:
                lhs = jnp.concatenate([w[8 * v:8 * v + 8] for v in rows], axis=0)
                y = jnp.dot(_ubf(lhs), rhs, preferred_element_type=f32)
                for n, v in enumerate(rows):
                    res[v] = y[16 * n:16 * n + 16]
            return jnp.concatenate([res[v] for v in range(NR)], axis=0)

        it = qk(1, i, 0, left, late=True, extra=dma_tie())
        pv(0, i, 2)
        it = it[7:] + qk(1, i, 1, it[:7], 9, late=True)
        pv(0, i, 3, it[:3])
        it = it[14:] + qk(1, i, 2, it[3:14], 0, late=True)
        it = it[12:] + qk(1, i, 3, it[:12], 0, late=True)
        proj_o(0, i, it[:-5], 0)
        out_cp(r0, T, 0, 384).start()
        zd = dma_tie()
        pv(1, i, 0, it[-5:])
        for g in range(1, 4):
            pv(1, i, g)
        o = o_part(0) + o_part(1) + o_part(2) + o_part(3, zd)
        ot = jnp.concatenate([oa_ref[0], o], axis=0).astype(bf16).T
        for a, b in ((0, 64), (64, 96), (96, 128)):
            ob_v[r0 + a:r0 + b, 384:896] = ot[a:b]
            out_cp(r0 + a, b - a, 384, 896).start()
        out_cp(0, S).wait()


@jax.jit
def pallas_concat_heads__sliding_block__sliding_block__prompt_kernel(A_x, A_wqkv, A_wo, B_x, B_wqkv, B_wo):
    anyspec = pl.BlockSpec(memory_space=pl.ANY)
    return pl.pallas_call(
        _kernel,
        grid=(NSTEP,),
        in_specs=[anyspec] * 6,
        out_specs=anyspec,
        out_shape=jax.ShapeDtypeStruct((1, S, 2 * D), bf16),
        scratch_shapes=[
            pltpu.VMEM((2, NT, D, T), bf16),
            pltpu.VMEM((2, D, 3 * D), bf16),
            pltpu.VMEM((2, D, D), bf16),
            pltpu.VMEM((S, 2 * D), bf16),
            pltpu.VMEM((2, 2 * D, 4 * T), u32),
            pltpu.VMEM((2, 4, S // 2, T), u32),
            pltpu.VMEM((2, NT + 1, 256, T), u32),
            pltpu.VMEM((4, 256, T), u32),
            pltpu.VMEM((4, 256, T), u32),
            pltpu.VMEM((2, 64, T), f32),
        ] + [pltpu.VMEM((MS + 1, 64, T), f32)] * 4
        + [pltpu.VMEM((ZP + 1, 32, T), u32)] * 4
        + [
            pltpu.VMEM((4, 64, T), u32),
            pltpu.VMEM((8, 32, T), u32),
            pltpu.VMEM((32, T), u32),
            pltpu.SemaphoreType.DMA((8,)),
        ],
        compiler_params=pltpu.CompilerParams(
            dimension_semantics=("arbitrary",),
            vmem_limit_bytes=64 * 1024 * 1024),
        name="swa",
    )(jnp.swapaxes(A_x, 1, 2), A_wqkv, A_wo, jnp.swapaxes(B_x, 1, 2), B_wqkv, B_wo)
```

```python
import functools

import jax
import jax.numpy as jnp
from jax import lax
import jax.experimental.pallas as pl
import jax.experimental.pallas.tpu as pltpu

S, D, H, DH, WIN = 2048, 448, 16, 28, 256
T = 128
NT = S // T
U = 4
NSTEP = 2 + (NT - 4) // U
QSCALE = (DH ** -0.5) * 1.4426950408889634
NEG = -1e30
SB = 32
NR = D // 16
ZP = 12
MS = 16
TIE0 = 12
NF = 9
HOPS = 2

f32, bf16, u32 = jnp.float32, jnp.bfloat16, jnp.uint32


def _pk(x):
    return pltpu.bitcast(x.astype(bf16), u32)


def _ubf(x):
    return pltpu.bitcast(x, bf16)


def _cat(xs):
    xs = [x for x in xs if x.shape[0] > 0]
    return xs[0] if len(xs) == 1 else jnp.concatenate(xs, axis=0)


def _kernel(xa_hbm, wqa_hbm, woa_hbm, xb_hbm, wqb_hbm, wob_hbm, o_hbm,
            x_v, wq_v, wo_v, ob_v, wt_ref, k_ref, vT_ref, q_ref, oT_ref, oa_ref,
            s0_ref, s1_ref, s2_ref, s3_ref, p0_ref, p1_ref, p2_ref, p3_ref,
            qm_ref, tmp_ref, sems):
    step = pl.program_id(0)
    s_refs = (s0_ref, s1_ref, s2_ref, s3_ref)
    p_refs = (p0_ref, p1_ref, p2_ref, p3_ref)

    def w_cp(name):
        src, dst, k = {
            "waq": (wqa_hbm.at[:, 0:256], wq_v.at[0, :, 0:256], 0),
            "waq2": (wqa_hbm.at[:, 256:512], wq_v.at[0, :, 256:512], 1),
            "wak": (wqa_hbm.at[:, 512:896], wq_v.at[0, :, 512:896], 2),
            "wav": (wqa_hbm.at[:, 896:1344], wq_v.at[0, :, 896:1344], 3),
            "wb": (wqb_hbm, wq_v.at[1], 4),
            "woa": (woa_hbm, wo_v.at[0], 5),
            "wob": (wob_hbm, wo_v.at[1], 5),
        }[name]
        return pltpu.make_async_copy(src, dst, sems.at[k])

    xgroups = {
        "xa0": (0, 0, 2, 7), "xa02": (0, 2, 3, 1), "xb0": (1, 0, 2, 4),
        "xb1": (1, 2, 2 + U, 0), "xa1": (0, 3, 3 + U, 0),
        "xb2": (1, 2 + U, NT, 6), "xa2": (0, 3 + U, NT, 6),
    }

    def start(*names):
        for name in names:
            if name in xgroups:
                br, t0, t1, k = xgroups[name]
                for t in range(t0, t1):
                    pltpu.make_async_copy((xa_hbm, xb_hbm)[br].at[0, :, t * T:(t + 1) * T],
                                          x_v.at[br, t], sems.at[k]).start()
            else:
                w_cp(name).start()

    def wait(*names):
        for name in names:
            if name in xgroups:
                br, t0, t1, k = xgroups[name]
                pltpu.make_async_copy(x_v.at[br, t0:t1], x_v.at[br, t0:t1], sems.at[k]).wait()
            else:
                w_cp(name).wait()

    def out_cp(row0, nrows, c0=0, c1=2 * D):
        return pltpu.make_async_copy(ob_v.at[pl.ds(row0, nrows), c0:c1],
                                     o_hbm.at[0, pl.ds(row0, nrows), c0:c1], sems.at[2])

    @pl.when(step == 0)
    def _():
        start("waq", "xa0", "waq2", "xa02", "wak", "wav", "wb", "xb0", "woa", "wob")
        row = lax.broadcasted_iota(jnp.int32, (64, T), 0)
        col = lax.broadcasted_iota(jnp.int32, (64, T), 1)
        real = jnp.logical_or((row & 31) < 14, (row & 31) >= 18)
        code = ((row >> 4) + (col >> 5)) & 3
        for c in range(4):
            qm_ref[c] = jnp.where(jnp.logical_and(real, code == c),
                                  jnp.uint32(0xFFFFFFFF), jnp.uint32(0))
            p_refs[c][ZP, 0] = jnp.zeros((16, 2 * T), bf16)
        vT_ref[1, 0, 128:256, :] = jnp.zeros((128, T), u32)

    zs = (step >> 10, step >> 11)
    zw, zr = zs

    lane = lax.broadcasted_iota(jnp.int32, (SB, T), 1)
    tri = lax.broadcasted_iota(jnp.int32, (SB, T), 0) <= (lane & (SB - 1))
    lane4 = lax.broadcasted_iota(jnp.int32, (4, 8, 2 * T), 2)
    odd = (lane4 & SB) != 0
    hi = (lane4 & (2 * SB)) != 0
    lane2 = lax.broadcasted_iota(jnp.int32, (1, 8, 2 * T), 2)
    key2 = lax.broadcasted_iota(jnp.int32, (1, 8, 2 * T), 1) + ((lane2 >> 7) << 4)
    tri2 = [key2 + 8 * e <= (lane2 & (SB - 1)) for e in range(2)]
    odd1 = (lane2 & SB) != 0
    hi1 = (lane2 & (2 * SB)) != 0
    zero2 = jnp.zeros((1, 8, 2 * T), bf16)
    zero8 = jnp.zeros((8, T), u32)

    def ties(items, nrounds, t0, t1):
        out = []
        done = 0
        for v in range(nrounds):
            zv = None
            if t0 <= v < t1:
                upto = (len(items) * (v - t0 + 1)) // (t1 - t0)
                if upto > done:
                    gs = sorted({it() for it in items[done:upto]})
                    done = upto
                    zv = functools.reduce(
                        jnp.bitwise_or, [pltpu.bitcast(p_refs[g][ZP, 0, :, 0:T], u32) for g in gs])
                    for h in range(HOPS):
                        tmp_ref[8 * h:8 * h + 8, :] = zv
                        zv = tmp_ref[8 * h:8 * h + 8, :]
            out.append(zv)
        return out

    def stack(zv):
        if all(z is None for z in zv):
            return None
        return jnp.concatenate([zero8 if z is None else z for z in zv], axis=0)

    def pad_heads(a, fill=None):
        parts = []
        for p in range(a.shape[0] // 56):
            b = a[56 * p:56 * p + 56]
            mid = b[24:32]
            if fill is None:
                parts += [b[0:32], b[24:56]]
            else:
                m = lax.broadcasted_iota(jnp.int32, mid.shape, 0) < 4
                parts += [b[0:24], jnp.where(m, mid, fill), jnp.where(m, fill, mid), b[32:56]]
        return jnp.concatenate(parts, axis=0)

    def roll_heads(a, back):
        parts = []
        for h in range(a.shape[0] // 16):
            j = h % 4
            b = a[16 * h:16 * h + 16]
            parts.append(b if j == 0 else pltpu.roll(b, SB * j if back else T - SB * j, 1))
        return jnp.concatenate(parts, axis=0)

    def moff(i, n):
        return i * n if isinstance(i, int) else pl.multiple_of(i * n, n)

    def prep_w(br, c0, c1):
        w = jnp.concatenate([wq_v[br, :, c0:c1], jnp.zeros((64, c1 - c0), bf16)], axis=0)
        wt_ref[br, c0 // 2:c1 // 2, :] = pltpu.bitcast(w.T, u32)

    def prep_wo(br):
        w = pad_heads(wo_v[br].astype(f32), 0.0).astype(bf16)
        wt_ref[br, 3 * D // 2:2 * D, :] = pltpu.bitcast(w.T, u32)

    def project(br, part, rhs, items, t0, mid):
        zv = stack(ties(items, NR, t0, NR))
        w = wt_ref[br, part * (D // 2):(part + 1) * (D // 2), :]
        if zv is not None:
            w = w | jnp.concatenate([zv] * 4, axis=1)
        y = jnp.dot(_ubf(w), rhs, preferred_element_type=f32)
        if mid:
            wait(*mid)
        return y

    def xtile(br, i):
        return jnp.concatenate([x_v[br, i], jnp.zeros((64, T), bf16)], axis=0)

    def proj_q(br, i, items=(), t0=TIE0, slot=None):
        qT = project(br, 0, xtile(br, i), items, t0, None) * QSCALE
        q_ref[br if slot is None else slot] = roll_heads(_pk(pad_heads(qT)), False)

    def proj_q_half(i, hf, slot, mid=None):
        y = jnp.dot(_ubf(wt_ref[0, 112 * hf:112 * hf + 112, :]), xtile(0, i),
                    preferred_element_type=f32)
        if mid:
            wait(*mid)
        q_ref[slot, T * hf:T * hf + T, :] = roll_heads(_pk(pad_heads(y * QSCALE)), False)

    def proj_k(br, i, items=(), t0=TIE0):
        kT = pad_heads(project(br, 1, xtile(br, i), items, t0, None))
        for gp in range(2):
            kt = pltpu.bitcast(kT[2 * T * gp:2 * T * (gp + 1)].astype(bf16).T, u32)
            for gg in range(2):
                k_ref[br, 2 * gp + gg, pl.ds(moff(i, 64), 64), :] = kt[:, T * gg:T * (gg + 1)]

    def proj_v(br, i, items=(), t0=TIE0, mid=None):
        vT = project(br, 2, xtile(br, i), items, t0, mid)
        vT_ref[br, i + 1] = _pk(pad_heads(vT, 1.0))

    def proj_o(br, i, items=(), t0=TIE0, slot=None, aslot=0):
        o = project(br, 3, _ubf(oT_ref[br if slot is None else slot]), items, t0, None)
        row0 = moff(i, T)
        if br == 0:
            ob_v[pl.ds(row0, T), 0:384] = o[0:384].astype(bf16).T
            oa_ref[aslot] = o[384:448]
        else:
            ob_v[pl.ds(row0, T), 384:896] = jnp.concatenate(
                [oa_ref[aslot], o], axis=0).astype(bf16).T

    def ntiles(i):
        return min(3, i + 1) if isinstance(i, int) else 3

    def qk(br, i, g, items=(), t0=1, t1=18, zero_fill=False, slot=None, col=0,
           late=False, extra=None):
        s_ref, p_ref = s_refs[g], p_refs[g]
        nt = ntiles(i)
        late = late or nt < 3
        zv = ties(items, 18, t0, t1)
        if extra is not None:
            zv[17] = extra if zv[17] is None else zv[17] | extra
        zv = stack(zv)
        q = q_ref[br if slot is None else slot, 64 * g:64 * g + 64, :]
        ms = [None] * 4
        for c in (range(4) if g % 2 == 0 else range(3, -1, -1)):
            n = min(WIN // 2, 64 * (nt - 1) + 16 * c)
            ks = k_ref[br, g, pl.ds(moff(i, 64) + (16 * c - n), n + 16), :]
            if n > 0:
                ks = jnp.concatenate([ks[n:], ks[:n]], axis=0)
            if zv is not None:
                ks = ks | (zv if nt == 3 else zv[:n + 16])
            s = jnp.dot(_ubf(ks), _ubf(q & qm_ref[c]), preferred_element_type=f32)
            if nt == 3:
                dg, rest = jnp.where(tri, s[0:SB], s[SB:2 * SB]), s[2 * SB:]
            else:
                dg, rest = jnp.where(tri, s[0:SB], NEG), s[SB:]
            nr = rest.shape[0] - SB * c

            def put_s(b0, rows):
                nb = rows.shape[0] // SB
                blk = rows.reshape(nb, 4, 8, T)
                blk = jnp.concatenate([blk[:, 0:2], blk[:, 2:4]], axis=3)
                s_ref[pl.ds(zw + 2 * b0, 2 * nb), c] = blk.reshape(2 * nb, 8, 2 * T)
            put_s(0, _cat([rest[nr:], dg]))
            if nr > 0:
                put_s(8 - nr // SB, rest[:nr])
            ms[c] = jnp.broadcast_to(jnp.max(_cat([dg, rest]), axis=0, keepdims=True), (8, T))
            if late:
                s_ref[zw + MS, c, :, 0:T] = ms[c]

        mall = None if late else jnp.stack(ms)

        def sel(m, a, b):
            if a is None and b is None:
                return None
            return lax.select(m, zero2 if a is None else a, zero2 if b is None else b)

        def put_p(b, e, x):
            if isinstance(x, list):
                x = [sel(odd1, x[(j + 1) % 4], x[j]) for j in range(4)]
                x = jnp.concatenate(
                    [sel(hi1, x[(j + 2) % 4], x[j]) for j in range(4)], axis=0)
            else:
                x = lax.select(odd, jnp.concatenate([x[1:], x[:1]], axis=0), x)
                x = lax.select(hi, jnp.concatenate([x[2:], x[:2]], axis=0), x)
            p_ref[zs[col] + b, :, 8 * e:8 * e + 8, :] = x

        def item(rho):
            b, e = rho // 2, rho % 2
            c0 = b if nt < 3 and rho < 8 else 0
            m = s_ref[zr + MS, c0:4, :, 0:T] if late else mall
            x = jnp.exp2(s_ref[zr + rho, c0:4] - jnp.concatenate([m, m], axis=2)).astype(bf16)
            if rho < 8:
                x = [None] * c0 + [x[c:c + 1] for c in range(4 - c0)]
            if rho >= 8 or nt == 1:
                put_p(b, e, x)
            elif nt == 3:
                put_p(b + 8, e, [None] * b + [sel(tri2[e], x[b], None)] + x[b + 1:])
                put_p(b, e, x[:b] + [sel(tri2[e], None, x[b])] + [None] * (3 - b))
            else:
                put_p(b + 8, e, x)
                if zero_fill:
                    p_ref[zs[col] + b, :, 8 * e:8 * e + 8, :] = jnp.zeros((4, 8, 2 * T), bf16)
            return g
        order = list(range(8, 16 if nt > 1 else 8)) + list(range(8))
        return [functools.partial(item, rho) for rho in order]

    def pv(br, i, g, items=(), slot=None, col=0):
        nt = ntiles(i)
        zv = ties(items, 6, 0, 6)
        acc = [None] * 4
        for t in range(3 - nt, 3):
            vv = vT_ref[br, i - 1 + t, 64 * g:64 * g + 64, :]
            zt = stack(zv[2 * t:2 * t + 2] * 4)
            vv = _ubf(vv if zt is None else vv | zt)
            bs = pl.ds(zs[1 - col] + (0 if nt == 1 else 4 * t), 4)
            for j in range(4):
                pj = jnp.concatenate([p_refs[g][bs, j, :, 0:T], p_refs[g][bs, j, :, T:2 * T]],
                                     axis=1).reshape(T, T)
                o = jnp.dot(vv[32 * j:32 * j + 32], pj, preferred_element_type=f32)
                acc[j] = o if acc[j] is None else acc[j] + o
        og = jnp.concatenate(
            [acc[j] * pl.reciprocal(acc[j][28:29] if j % 2 == 0 else acc[j][0:1], approx=False)
             for j in range(4)], axis=0)
        oT_ref[br if slot is None else slot, 64 * g:64 * g + 64, :] = roll_heads(_pk(og), True)

    def half(br, i, nxt, fin, left, flush):
        ob = 1 - br
        for g in range(4):
            items = qk(br, i, g, left)
            n = len(items) if flush and g == 3 else NF
            items, left = items[:n], items[n:]
            if g > 1:
                pv(br, i, g - 2)
            else:
                pv(ob, fin, g + 2)
            if g == 2:
                proj_o(ob, fin, items)
            else:
                (proj_k, proj_q, None, proj_v)[g](ob, nxt, items)
        return left

    def period(i, left, flush):
        left = half(0, i, i, i - 1, left, False)
        return half(1, i, i + 1, i, left, flush)

    @pl.when(step == 0)
    def _():
        wait("waq")
        prep_w(0, 0, 256)
        start("xb1", "xa1", "xb2", "xa2")
        wait("xa0")
        proj_q_half(0, 0, 2)
        proj_q_half(1, 0, 3, mid=("waq2", "xa02"))
        prep_w(0, 256, 512)
        proj_q_half(2, 0, 0)
        proj_q_half(0, 1, 2)
        proj_q_half(1, 1, 3, mid=("wak",))
        prep_w(0, 512, 896)
        proj_q_half(2, 1, 0)
        proj_k(0, 0)
        proj_k(0, 1)
        it = sum([qk(0, 0, g, slot=2, col=1) for g in range(4)], [])
        proj_k(0, 2, it, 4)
        it0 = qk(0, 1, 0, slot=3)
        it1 = qk(0, 1, 1, slot=3)
        wait("wav")
        prep_w(0, 896, 1344)
        it2 = qk(0, 1, 2, it0[:8], 1, 10, slot=3)
        it3 = qk(0, 1, 3, it0[8:], 1, 10, slot=3)
        proj_v(0, 0, it1, 1)
        proj_v(0, 1, it2, 1, mid=("wb", "xb0"))
        prep_w(1, 384, 896)
        prep_w(1, 0, 384)
        prep_w(1, 896, 1344)
        for g in range(4):
            pv(0, 0, g, slot=2, col=1)
        for g in range(3):
            pv(0, 1, g)
        proj_k(1, 0, it3, 11)
        proj_q(1, 0, slot=2)
        proj_k(1, 1)
        it = sum([qk(1, 0, g, slot=2, col=1) for g in range(4)], [])
        pv(0, 1, 3)
        proj_q(1, 1, it, 2)
        proj_v(1, 0, mid=("woa", "wob"))
        prep_wo(0)
        prep_wo(1)
        it0 = qk(1, 1, 0)
        it1 = qk(1, 1, 1)
        for g in range(4):
            pv(1, 0, g, slot=3, col=1)
        proj_v(1, 1, it0, 11)
        proj_o(0, 0, it1, 1, slot=2, aslot=1)
        proj_o(1, 0, slot=3, aslot=1)
        it0 = qk(1, 1, 2, zero_fill=True)
        it1 = qk(1, 1, 3, zero_fill=True)
        pv(1, 1, 0)
        pv(1, 1, 1)
        proj_o(0, 1, it0, 11)
        proj_v(0, 2, it1, 1)
        wait("xb1", "xa1")
        out_cp(0, T).start()

    @pl.when(jnp.logical_and(step > 0, step < NSTEP - 1))
    def _():
        left = ()
        i0 = 2 + (step - 1) * U
        for b in range(U):
            left = period(i0 + b, left, b == U - 1)
        out_cp(pl.multiple_of((i0 - 1) * T, T), U * T).start()

    @pl.when(step == 1)
    def _():
        wait("xb2", "xa2")

    @pl.when(step == NSTEP - 1)
    def _():
        i = NT - 1
        r0 = i * T
        left = period(i - 1, (), False)
        left = half(0, i, i, i - 1, left, False)
        out_cp((NT - 3) * T, 2 * T).start()

        def dma_tie():
            ob_v[pl.ds(moff(zw, 16) + r0, 16), 512:640] = jnp.zeros((16, T), bf16)
            return pltpu.bitcast(ob_v[pl.ds(moff(zr, 16) + r0, 16), 512:640], u32)

        def o_part(g):
            sets = ([4, 5, 6, 7, 8, 9, 10], [12, 13, 14, 15, 16, 17, 18],
                    [20, 21, 22, 23, 24, 25, 26], [0, 1, 2, 3, 11, 19, 27])
            w = wt_ref[1, 3 * D // 2:2 * D, T * g:T * (g + 1)]
            rhs = _ubf(oT_ref[1, 64 * g:64 * g + 64, :])
            res = {}
            for rows in sets:
                lhs = jnp.concatenate([w[8 * v:8 * v + 8] for v in rows], axis=0)
                y = jnp.dot(_ubf(lhs), rhs, preferred_element_type=f32)
                for n, v in enumerate(rows):
                    res[v] = y[16 * n:16 * n + 16]
            return jnp.concatenate([res[v] for v in range(NR)], axis=0)

        it = qk(1, i, 0, left, late=True, extra=dma_tie())
        pv(0, i, 2)
        it = it[7:] + qk(1, i, 1, it[:7], 9, late=True)
        pv(0, i, 3, it[:3])
        it = it[14:] + qk(1, i, 2, it[3:14], 0, late=True)
        it = it[12:] + qk(1, i, 3, it[:12], 0, late=True)
        proj_o(0, i, it[:-5], 0)
        out_cp(r0, T, 0, 384).start()
        zd = dma_tie()
        pv(1, i, 0, it[-5:])
        for g in range(1, 4):
            pv(1, i, g)
        o = o_part(0) + o_part(1) + o_part(2) + o_part(3)
        oa = pltpu.bitcast(pltpu.bitcast(oa_ref[0, 0:8, :], u32) | zd, f32)
        ot = jnp.concatenate([oa, oa_ref[0, 8:64, :], o], axis=0).astype(bf16).T
        for a in range(0, T, 32):
            ob_v[r0 + a:r0 + a + 32, 384:896] = ot[a:a + 32]
            out_cp(r0 + a, 32, 384, 896).start()
        out_cp(0, S).wait()


@jax.jit
def pallas_concat_heads__sliding_block__sliding_block__prompt_kernel(A_x, A_wqkv, A_wo, B_x, B_wqkv, B_wo):
    anyspec = pl.BlockSpec(memory_space=pl.ANY)
    return pl.pallas_call(
        _kernel,
        grid=(NSTEP,),
        in_specs=[anyspec] * 6,
        out_specs=anyspec,
        out_shape=jax.ShapeDtypeStruct((1, S, 2 * D), bf16),
        scratch_shapes=[
            pltpu.VMEM((2, NT, D, T), bf16),
            pltpu.VMEM((2, D, 3 * D), bf16),
            pltpu.VMEM((2, D, D), bf16),
            pltpu.VMEM((S, 2 * D), bf16),
            pltpu.VMEM((2, 2 * D, 4 * T), u32),
            pltpu.VMEM((2, 4, S // 2, T), u32),
            pltpu.VMEM((2, NT + 1, 256, T), u32),
            pltpu.VMEM((4, 256, T), u32),
            pltpu.VMEM((4, 256, T), u32),
            pltpu.VMEM((2, 64, T), f32),
        ] + [pltpu.VMEM((MS + 1, 4, 8, 2 * T), f32)] * 4
        + [pltpu.VMEM((ZP + 1, 4, 16, 2 * T), bf16)] * 4
        + [
            pltpu.VMEM((4, 64, T), u32),
            pltpu.VMEM((32, T), u32),
            pltpu.SemaphoreType.DMA((8,)),
        ],
        compiler_params=pltpu.CompilerParams(
            dimension_semantics=("arbitrary",),
            vmem_limit_bytes=64 * 1024 * 1024),
        name="swa",
    )(jnp.swapaxes(A_x, 1, 2), A_wqkv, A_wo, jnp.swapaxes(B_x, 1, 2), B_wqkv, B_wo)
```

```python
import functools

import jax
import jax.numpy as jnp
from jax import lax
import jax.experimental.pallas as pl
import jax.experimental.pallas.tpu as pltpu

S, D, H, DH, WIN = 2048, 448, 16, 28, 256
T = 128
NT = S // T
U = 4
NLOOP = (NT - 4) // U
QSCALE = (DH ** -0.5) * 1.4426950408889634
NEG = -1e30
SB = 32
NR = D // 16
ZP = 12
MS = 16
TIE0 = 12
NF = 9
OTIE = 14

f32, bf16, u32 = jnp.float32, jnp.bfloat16, jnp.uint32


def _pk(x):
    return pltpu.bitcast(x.astype(bf16), u32)


def _ubf(x):
    return pltpu.bitcast(x, bf16)


def _kernel(xa_hbm, wqa_hbm, woa_hbm, xb_hbm, wqb_hbm, wob_hbm, o_hbm,
            x_v, wq_v, wo_v, ob_v, wt_ref, k_ref, vT_ref, qT_ref, q_ref, oT_ref, oa_ref,
            s0_ref, s1_ref, s2_ref, s3_ref, p0_ref, p1_ref, p2_ref, p3_ref,
            qm_ref, tmp_ref, sems):
    step = pl.program_id(0)
    s_refs = (s0_ref, s1_ref, s2_ref, s3_ref)
    p_refs = (p0_ref, p1_ref, p2_ref, p3_ref)

    def w_cp(name):
        src, dst, k = {
            "waq": (wqa_hbm.at[:, 0:256], wq_v.at[0, :, 0:256], 0),
            "waq2": (wqa_hbm.at[:, 256:512], wq_v.at[0, :, 256:512], 1),
            "wak": (wqa_hbm.at[:, 512:896], wq_v.at[0, :, 512:896], 2),
            "wav": (wqa_hbm.at[:, 896:1344], wq_v.at[0, :, 896:1344], 3),
            "wb": (wqb_hbm, wq_v.at[1], 4),
            "woa": (woa_hbm, wo_v.at[0], 5),
            "wob": (wob_hbm, wo_v.at[1], 5),
        }[name]
        return pltpu.make_async_copy(src, dst, sems.at[k])

    xgroups = {
        "xa0": (0, 0, 2, 7), "xa02": (0, 2, 3, 1), "xb0": (1, 0, 2, 4),
        "xb1": (1, 2, 2 + U, 0), "xa1": (0, 3, 3 + U, 0),
        "xb2": (1, 2 + U, NT, 6), "xa2": (0, 3 + U, NT, 6),
    }

    def start(*names):
        for name in names:
            if name in xgroups:
                br, t0, t1, k = xgroups[name]
                for t in range(t0, t1):
                    pltpu.make_async_copy((xa_hbm, xb_hbm)[br].at[0, :, t * T:(t + 1) * T],
                                          x_v.at[br, t], sems.at[k]).start()
            else:
                w_cp(name).start()

    def wait(*names):
        for name in names:
            if name in xgroups:
                br, t0, t1, k = xgroups[name]
                pltpu.make_async_copy(x_v.at[br, t0:t1], x_v.at[br, t0:t1], sems.at[k]).wait()
            else:
                w_cp(name).wait()

    def out_cp(row0, nrows, c0=0, c1=2 * D):
        return pltpu.make_async_copy(ob_v.at[row0:row0 + nrows, c0:c1],
                                     o_hbm.at[0, row0:row0 + nrows, c0:c1], sems.at[2])

    def init():
        start("waq", "xa0", "waq2", "xa02", "wak", "wav", "wb", "xb0", "woa", "wob")
        row = lax.broadcasted_iota(jnp.int32, (64, T), 0)
        col = lax.broadcasted_iota(jnp.int32, (64, T), 1)
        real = (jnp.logical_or((row & 31) < 14, (row & 31) >= 18),
                jnp.logical_or((col & 63) < 28, (col & 63) >= 36))
        code = ((row >> 4) + (col >> 5)) & 3
        for c in range(4):
            for f in range(2):
                qm_ref[f, c] = jnp.where(jnp.logical_and(real[f], code == c),
                                         jnp.uint32(0xFFFFFFFF), jnp.uint32(0))
            p_refs[c][ZP, 0] = jnp.zeros((16, 2 * T), bf16)
        vT_ref[1, 0, 192:256, :] = jnp.zeros((64, T), u32)
        ob_v[S:S + 16, 0:T] = jnp.zeros((16, T), bf16)
        oa_ref[0] = jnp.zeros((64, T), f32)

    zs = (step >> 10, step >> 11)
    zw, zr = zs

    mk = {}

    def make_masks():
        lane = lax.broadcasted_iota(jnp.int32, (SB, T), 1)
        mk["tri"] = lax.broadcasted_iota(jnp.int32, (SB, T), 0) <= (lane & (SB - 1))
        for n in (4, 1):
            lane = lax.broadcasted_iota(jnp.int32, (n, 8, 2 * T), 2)
            mk["odd", n] = (lane & SB) != 0
            mk["hi", n] = (lane & (2 * SB)) != 0
        key = lax.broadcasted_iota(jnp.int32, (1, 8, 2 * T), 1) + ((lane >> 7) << 4)
        for e in range(2):
            mk["tri", e] = key + 8 * e <= (lane & (SB - 1))

    zero2 = jnp.zeros((1, 8, 2 * T), bf16)
    zero8 = jnp.zeros((8, T), u32)

    def slack(z, r0):
        for r in (r0, r0 + 8):
            tmp_ref[r:r + 8, :] = z
            z = tmp_ref[r:r + 8, :]
        return z

    def ties(items, nrounds, t0, t1, extra=()):
        out = []
        done = 0
        for v in range(nrounds):
            zv = None
            if t0 <= v < t1:
                upto = (len(items) * (v - t0 + 1)) // (t1 - t0)
                if upto > done:
                    gs = sorted({it() for it in items[done:upto]})
                    done = upto
                    zv = slack(functools.reduce(jnp.bitwise_or, [
                        pltpu.bitcast(p_refs[g][ZP, 0, :, 0:T], u32) for g in gs]), 0)
            out.append(zv)
        for v, z in extra:
            out[v] = z if out[v] is None else out[v] | z
        if all(z is None for z in out):
            return None
        return jnp.concatenate([zero8 if z is None else z for z in out], axis=0)

    def pad_heads(a, fill=None):
        parts = []
        for p in range(a.shape[0] // 56):
            b = a[56 * p:56 * p + 56]
            mid = b[24:32]
            if fill is None:
                parts += [b[0:32], b[24:56]]
            else:
                m = lax.broadcasted_iota(jnp.int32, mid.shape, 0) < 4
                parts += [b[0:24], jnp.where(m, mid, fill), jnp.where(m, fill, mid), b[32:56]]
        return jnp.concatenate(parts, axis=0)

    def roll_heads(a, back):
        parts = []
        for h in range(a.shape[0] // 16):
            j = h % 4
            b = a[16 * h:16 * h + 16]
            parts.append(b if j == 0 else pltpu.roll(b, SB * j if back else T - SB * j, 1))
        return jnp.concatenate(parts, axis=0)

    def moff(i, n):
        return i * n if isinstance(i, int) else pl.multiple_of(i * n, n)

    def prep_w(br, c0, c1):
        w = jnp.concatenate([wq_v[br, :, c0:c1], jnp.zeros((64, c1 - c0), bf16)], axis=0)
        wt_ref[br, c0 // 2:c1 // 2, :] = pltpu.bitcast(w.T, u32)

    def prep_wo(br):
        w = pad_heads(wo_v[br].astype(f32), 0.0).astype(bf16)
        wt_ref[br, 3 * D // 2:2 * D, :] = pltpu.bitcast(w.T, u32)

    def project(br, part, rhs, items, t0, extra=()):
        zv = ties(items, NR, t0, NR, extra)
        w = wt_ref[br, part * (D // 2):(part + 1) * (D // 2), :]
        if zv is not None:
            w = w | jnp.concatenate([zv] * 4, axis=1)
        return jnp.dot(_ubf(w), rhs, preferred_element_type=f32)

    def xtile(br, i):
        return jnp.concatenate([x_v[br, i], jnp.zeros((64, T), bf16)], axis=0)

    def put_q(br, slot, y, hf=0):
        y = pad_heads(y * QSCALE)
        n = y.shape[0]
        if slot is None:
            q_ref[br, :, n * hf:n * (hf + 1)] = pltpu.bitcast(y.astype(bf16).T, u32)
        else:
            qT_ref[slot, n // 2 * hf:n // 2 * (hf + 1), :] = roll_heads(_pk(y), False)

    def proj_q(br, i, items=(), t0=TIE0, slot=None):
        put_q(br, slot, project(br, 0, xtile(br, i), items, t0))

    def proj_q_half(i, hf, slot, mid=()):
        y = jnp.dot(_ubf(wt_ref[0, 112 * hf:112 * hf + 112, :]), xtile(0, i),
                    preferred_element_type=f32)
        wait(*mid)
        put_q(0, slot, y, hf)

    def proj_k(br, i, items=(), t0=TIE0):
        kT = pad_heads(project(br, 1, xtile(br, i), items, t0))
        for gp in range(2):
            kt = pltpu.bitcast(kT[2 * T * gp:2 * T * (gp + 1)].astype(bf16).T, u32)
            for gg in range(2):
                k_ref[br, 2 * gp + gg, pl.ds(moff(i, 64), 64), :] = kt[:, T * gg:T * (gg + 1)]

    def proj_v(br, i, items=(), t0=TIE0, mid=(), extra=()):
        vT = project(br, 2, xtile(br, i), items, t0, extra)
        wait(*mid)
        vT_ref[br, i + 1] = _pk(pad_heads(vT, 1.0))

    def proj_o(br, i, items=(), t0=TIE0, slot=None, aslot=0, full=False, extra=()):
        o = project(br, 3, _ubf(oT_ref[br if slot is None else slot]), items, t0, extra)
        row0 = moff(i, T)
        if full:
            ob_v[pl.ds(row0, T), 0:D] = o.astype(bf16).T
        elif br == 0:
            ob_v[pl.ds(row0, T), 0:384] = o[0:384].astype(bf16).T
            oa_ref[aslot] = o[384:448]
        else:
            ob_v[pl.ds(row0, T), 384:896] = jnp.concatenate(
                [oa_ref[aslot], o], axis=0).astype(bf16).T

    def ntiles(i):
        return min(3, i + 1) if isinstance(i, int) else 3

    def qk(br, i, g, items=(), t0=1, t1=18, zero_fill=False, slot=None, col=0,
           late=False, extra=()):
        s_ref = s_refs[g]
        nt = ntiles(i)
        late = late or nt < 3
        zv = ties(items, 18, t0, t1, extra)
        if slot is None:
            q = q_ref[br, :, T * g:T * (g + 1)]
        else:
            q = qT_ref[slot, 64 * g:64 * g + 64, :]
        ms = [None] * 4
        for c in (range(4) if g % 2 == 0 else range(3, -1, -1)):
            n = min(WIN // 2, 64 * (nt - 1) + 16 * c)
            ks = k_ref[br, g, pl.ds(moff(i, 64) + (16 * c - n), n + 16), :]
            if n > 0:
                ks = jnp.concatenate([ks[n:], ks[:n]], axis=0)
            if zv is not None:
                ks = ks | (zv if nt == 3 else zv[:n + 16])
            if slot is None:
                w = jnp.concatenate([q[16 * c:16 * c + 16]] * 4, axis=0) & qm_ref[1, c]
                s = lax.dot_general(_ubf(ks), _ubf(w), (((1,), (1,)), ((), ())),
                                    preferred_element_type=f32)
            else:
                s = jnp.dot(_ubf(ks), _ubf(q & qm_ref[0, c]), preferred_element_type=f32)
            r0 = 2 * SB if nt == 3 else SB
            dg = jnp.where(mk["tri"], s[0:SB], s[SB:r0] if nt == 3 else NEG)
            r1 = s.shape[0] - SB * c

            def put_s(b0, rows):
                nb = rows.shape[0] // SB
                blk = rows.reshape(nb, 4, 8, T)
                blk = jnp.concatenate([blk[:, 0:2], blk[:, 2:4]], axis=3)
                s_ref[pl.ds(zw + 2 * b0, 2 * nb), c] = blk.reshape(2 * nb, 8, 2 * T)
            put_s(0, jnp.concatenate([s[r1:], dg], axis=0) if c > 0 else dg)
            if r1 > r0:
                put_s(8 - (r1 - r0) // SB, s[r0:r1])
            sm = jnp.concatenate([dg, s[r0:]], axis=0) if s.shape[0] > r0 else dg
            ms[c] = jnp.broadcast_to(jnp.max(sm, axis=0, keepdims=True), (8, T))
            if late:
                s_ref[zw + MS, c, :, 0:T] = ms[c]

        return sm_items(g, nt, None if late else jnp.stack(ms), zero_fill, col)

    def sm_items(g, nt=3, mall=None, zero_fill=False, col=0):
        s_ref, p_ref = s_refs[g], p_refs[g]

        def sel(m, a, b):
            if a is None and b is None:
                return None
            return lax.select(m, zero2 if a is None else a, zero2 if b is None else b)

        def put_p(b, e, x):
            if isinstance(x, list):
                x = [sel(mk["odd", 1], x[(j + 1) % 4], x[j]) for j in range(4)]
                x = jnp.concatenate(
                    [sel(mk["hi", 1], x[(j + 2) % 4], x[j]) for j in range(4)], axis=0)
            else:
                x = lax.select(mk["odd", 4], jnp.concatenate([x[1:], x[:1]], axis=0), x)
                x = lax.select(mk["hi", 4], jnp.concatenate([x[2:], x[:2]], axis=0), x)
            p_ref[zs[col] + b, :, 8 * e:8 * e + 8, :] = x

        def item(rho):
            b, e = rho // 2, rho % 2
            c0 = b if nt < 3 and rho < 8 else 0
            m = s_ref[zr + MS, c0:4, :, 0:T] if mall is None else mall
            x = jnp.exp2(s_ref[zr + rho, c0:4] - jnp.concatenate([m, m], axis=2)).astype(bf16)
            if rho < 8:
                x = [None] * c0 + [x[c:c + 1] for c in range(4 - c0)]
            if rho >= 8 or nt == 1:
                put_p(b, e, x)
            elif nt == 3:
                tri = mk["tri", e]
                put_p(b + 8, e, [None] * b + [sel(tri, x[b], None)] + x[b + 1:])
                put_p(b, e, x[:b] + [sel(tri, None, x[b])] + [None] * (3 - b))
            else:
                put_p(b + 8, e, x)
                if zero_fill:
                    p_ref[zs[col] + b, :, 8 * e:8 * e + 8, :] = jnp.zeros((4, 8, 2 * T), bf16)
            return g
        order = list(range(8, 16 if nt > 1 else 8)) + list(range(8))
        return [functools.partial(item, rho) for rho in order]

    def pv(br, i, g, slot=None, col=0):
        nt = ntiles(i)
        acc = [None] * 4
        for t in range(3 - nt, 3):
            vv = _ubf(vT_ref[br, i - 1 + t, 64 * g:64 * g + 64, :])
            bs = pl.ds(zs[1 - col] + (0 if nt == 1 else 4 * t), 4)
            for j in range(4):
                pj = jnp.concatenate([p_refs[g][bs, j, :, 0:T], p_refs[g][bs, j, :, T:2 * T]],
                                     axis=1).reshape(T, T)
                o = jnp.dot(vv[32 * j:32 * j + 32], pj, preferred_element_type=f32)
                acc[j] = o if acc[j] is None else acc[j] + o
        og = jnp.concatenate(
            [acc[j] * pl.reciprocal(acc[j][28:29] if j % 2 == 0 else acc[j][0:1], approx=False)
             for j in range(4)], axis=0)
        oT_ref[br if slot is None else slot, 64 * g:64 * g + 64, :] = roll_heads(_pk(og), True)

    def units(i0, n, cut):
        items = sm_items(0)
        for u in range(1, n + 1):
            i, br, g = i0 + u // 8, u // 4 % 2, u % 4
            pb, pg = (br, g - 1) if g > 0 else (1 - br, 3)
            pi = i if u % 8 > 0 else i - 1
            if pg == 2:
                proj_o(1 - pb, pi - 1 + pb, items[:NF])
            elif pg == 3:
                zo = pltpu.bitcast(ob_v[pl.ds(moff(zr, 16) + S, 16), 0:T], u32)
                proj_v(1 - pb, pi + pb, items[:NF], extra=[(OTIE, slack(zo, 16))])
            else:
                (proj_k, proj_q)[pg](1 - pb, pi + pb, items[:NF], 2 if u == 1 else TIE0)
            last = cut and u == n
            do_pv = functools.partial(pv, br, i, g - 2) if g > 1 else functools.partial(
                pv, 1 - br, i - 1 + br, g + 2)
            if last:
                do_pv()
            items = qk(br, i, g, items[NF:], late=last)
            if not last:
                do_pv()
        return items

    def first():
        make_masks()
        wait("waq")
        prep_w(0, 0, 256)
        start("xb1", "xa1", "xb2", "xa2")
        wait("xa0")
        proj_q_half(0, 0, 0)
        proj_q_half(1, 0, 1, mid=("waq2", "xa02"))
        prep_w(0, 256, 512)
        proj_q_half(2, 0, None)
        proj_q_half(0, 1, 0)
        proj_q_half(1, 1, 1, mid=("wak",))
        prep_w(0, 512, 896)
        proj_q_half(2, 1, None)
        proj_k(0, 0)
        proj_k(0, 1)
        it = sum([qk(0, 0, g, slot=0, col=1) for g in range(4)], [])
        proj_k(0, 2, it, 4)
        it0 = qk(0, 1, 0, slot=1)
        it1 = qk(0, 1, 1, slot=1)
        wait("wav")
        prep_w(0, 896, 1344)
        it2 = qk(0, 1, 2, it0[:8], 1, 10, slot=1)
        it3 = qk(0, 1, 3, it0[8:], 1, 10, slot=1)
        proj_v(0, 0, it1, 1)
        proj_v(0, 1, it2, 1, mid=("wb", "xb0"))
        prep_w(1, 384, 896)
        prep_w(1, 0, 384)
        prep_w(1, 896, 1344)
        for g in range(4):
            pv(0, 0, g, slot=2, col=1)
        for g in range(3):
            pv(0, 1, g, slot=4)
        proj_k(1, 0, it3, 11)
        proj_q(1, 0, slot=0)
        proj_k(1, 1)
        it = sum([qk(1, 0, g, slot=0, col=1) for g in range(4)], [])
        pv(0, 1, 3, slot=4)
        proj_q(1, 1, it, 2, slot=1)
        proj_v(1, 0)
        it = qk(1, 1, 0, slot=1)
        it = it + qk(1, 1, 1, slot=1)
        it = it[9:] + qk(1, 1, 2, it[:9], 1, 10, slot=1)
        it3 = qk(1, 1, 3, it[:12], 1, 10, zero_fill=True, slot=1)
        for g in range(4):
            pv(1, 0, g, slot=3, col=1)
        proj_v(1, 1, it[12:], 10)
        proj_v(0, 2, it3, 1)
        for g in range(3):
            pv(1, 1, g)
        qk(0, 2, 0, late=True)
        wait("woa", "wob", "xb1", "xa1")

    def steady(n, carry):
        make_masks()
        prep_wo(1)
        prep_wo(0)
        units(2 + n * U, 8 * U, True)

        @pl.when(n == 0)
        def _():
            out_cp(2 * T, (U - 1) * T).start()
            wait("xb2", "xa2")

        for k in range(1, NLOOP):
            pl.when(n == k)(out_cp((1 + k * U) * T, U * T).start)
        return carry

    def last():
        make_masks()
        i = NT - 1
        r0 = i * T
        it = units(i - 1, 11, False)
        proj_v(1, i, it[:NF])
        out_cp((NT - 3) * T, 2 * T).start()

        def dma_tie():
            ob_v[pl.ds(moff(zw, 16) + r0, 16), 512:640] = jnp.zeros((16, T), bf16)
            return pltpu.bitcast(ob_v[pl.ds(moff(zr, 16) + r0, 16), 512:640], u32)

        def o_part(g):
            sets = ([4, 5, 6, 7, 8, 9, 10], [12, 13, 14, 15, 16, 17, 18],
                    [20, 21, 22, 23, 24, 25, 26], [0, 1, 2, 3, 11, 19, 27])
            w = wt_ref[1, 3 * D // 2:2 * D, T * g:T * (g + 1)]
            rhs = _ubf(oT_ref[1, 64 * g:64 * g + 64, :])
            res = {}
            for rows in sets:
                lhs = jnp.concatenate([w[8 * v:8 * v + 8] for v in rows], axis=0)
                y = jnp.dot(_ubf(lhs), rhs, preferred_element_type=f32)
                for n, v in enumerate(rows):
                    res[v] = y[16 * n:16 * n + 16]
            return jnp.concatenate([res[v] for v in range(NR)], axis=0)

        it = qk(1, i, 0, it[NF:], late=True, extra=[(17, dma_tie())])
        pv(0, i, 2)
        proj_o(0, 0, it[:NF], slot=2, aslot=1)
        it = qk(1, i, 1, it[NF:], late=True)
        pv(0, i, 3)
        proj_o(1, 0, it[:NF], slot=3, aslot=1)
        out_cp(0, T).start()
        it = qk(1, i, 2, it[NF:], late=True)
        it = it[5:] + qk(1, i, 3, it[:5], 12, late=True, extra=[(17, dma_tie())])
        proj_o(0, 1, it[:15], 0, slot=4, full=True)
        out_cp(T, T).start()
        pv(1, i, 0)
        proj_o(0, i, it[15:], 0, extra=[(NR - 1, dma_tie())])
        out_cp(r0, T, 0, 384).start()
        zd = dma_tie()
        for g in range(1, 4):
            pv(1, i, g)
        o = o_part(0) + o_part(1) + o_part(2) + o_part(3)
        oa = pltpu.bitcast(pltpu.bitcast(oa_ref[0, 0:8, :], u32) | zd, f32)
        ot = jnp.concatenate([oa, oa_ref[0, 8:64, :], o], axis=0).astype(bf16).T
        for a in range(r0, S, 32):
            ob_v[a:a + 32, 384:896] = ot[a - r0:a - r0 + 32]
            out_cp(a, 32, 384, 896).start()
        out_cp(0, S).wait()

    pl.when(step == 0)(init)

    @pl.when(step == 1)
    def _():
        first()
        lax.fori_loop(0, NLOOP, steady, 0)
        last()


@jax.jit
def pallas_concat_heads__sliding_block__sliding_block__prompt_kernel(
        A_x, A_wqkv, A_wo, B_x, B_wqkv, B_wo):
    anyspec = pl.BlockSpec(memory_space=pl.ANY)
    return pl.pallas_call(
        _kernel,
        grid=(2,),
        in_specs=[anyspec] * 6,
        out_specs=anyspec,
        out_shape=jax.ShapeDtypeStruct((1, S, 2 * D), bf16),
        scratch_shapes=[
            pltpu.VMEM((2, NT, D, T), bf16),
            pltpu.VMEM((2, D, 3 * D), bf16),
            pltpu.VMEM((2, D, D), bf16),
            pltpu.VMEM((S + 64, 2 * D), bf16),
            pltpu.VMEM((2, 2 * D, 4 * T), u32),
            pltpu.VMEM((2, 4, S // 2, T), u32),
            pltpu.VMEM((2, NT + 1, 256, T), u32),
            pltpu.VMEM((2, 256, T), u32),
            pltpu.VMEM((2, 64, 4 * T), u32),
            pltpu.VMEM((5, 256, T), u32),
            pltpu.VMEM((2, 64, T), f32),
        ] + [pltpu.VMEM((MS + 1, 4, 8, 2 * T), f32)] * 4
        + [pltpu.VMEM((ZP + 1, 4, 16, 2 * T), bf16)] * 4
        + [
            pltpu.VMEM((2, 4, 64, T), u32),
            pltpu.VMEM((32, T), u32),
            pltpu.SemaphoreType.DMA((8,)),
        ],
        compiler_params=pltpu.CompilerParams(
            dimension_semantics=("arbitrary",),
            vmem_limit_bytes=64 * 1024 * 1024),
        name="swa",
    )(jnp.swapaxes(A_x, 1, 2), A_wqkv, A_wo, jnp.swapaxes(B_x, 1, 2), B_wqkv, B_wo)
```

```python
import functools

import jax
import jax.numpy as jnp
from jax import lax
import jax.experimental.pallas as pl
import jax.experimental.pallas.tpu as pltpu

S, D, H, DH, WIN = 2048, 448, 16, 28, 256
T = 128
NT = S // T
U = 4
NLOOP = (NT - 4) // U
QSCALE = (DH ** -0.5) * 1.4426950408889634
NEG = -1e30
SB = 32
NR = D // 16
ZP = 12
MS = 16
TIE0 = 12
NF = 9
OTIE = 14

f32, bf16, u32 = jnp.float32, jnp.bfloat16, jnp.uint32


def _pk(x):
    return pltpu.bitcast(x.astype(bf16), u32)


def _ubf(x):
    return pltpu.bitcast(x, bf16)


def _kernel(xa_hbm, wqa_hbm, woa_hbm, xb_hbm, wqb_hbm, wob_hbm, o_hbm,
            x_v, wq_v, wo_v, ob_v, wt_ref, k_ref, vT_ref, qT_ref, q_ref, oT_ref, oa_ref,
            s0_ref, s1_ref, s2_ref, s3_ref, p0_ref, p1_ref, p2_ref, p3_ref,
            qm_ref, tmp_ref, sems):
    step = pl.program_id(0)
    s_refs = (s0_ref, s1_ref, s2_ref, s3_ref)
    p_refs = (p0_ref, p1_ref, p2_ref, p3_ref)

    def w_cp(name):
        src, dst, k = {
            "waq": (wqa_hbm.at[:, 0:256], wq_v.at[0, :, 0:256], 0),
            "waq2": (wqa_hbm.at[:, 256:512], wq_v.at[0, :, 256:512], 1),
            "wak": (wqa_hbm.at[:, 512:896], wq_v.at[0, :, 512:896], 2),
            "wav": (wqa_hbm.at[:, 896:1344], wq_v.at[0, :, 896:1344], 3),
            "wb": (wqb_hbm, wq_v.at[1], 4),
            "woa": (woa_hbm, wo_v.at[0], 5),
            "wob": (wob_hbm, wo_v.at[1], 5),
        }[name]
        return pltpu.make_async_copy(src, dst, sems.at[k])

    xgroups = {
        "xa0": (0, 0, 2, 6), "xa02": (0, 2, 3, 1), "xb0": (1, 0, 2, 4),
        "xb1": (1, 2, 2 + U, 5), "xa1": (0, 3, 3 + U, 5),
        "xb2": (1, 2 + U, NT, 0), "xa2": (0, 3 + U, NT, 0),
    }

    def start(*names):
        for name in names:
            if name in xgroups:
                br, t0, t1, k = xgroups[name]
                for t in range(t0, t1):
                    pltpu.make_async_copy((xa_hbm, xb_hbm)[br].at[0, :, t * T:(t + 1) * T],
                                          x_v.at[br, t], sems.at[k]).start()
            else:
                w_cp(name).start()

    def wait(*names):
        for name in names:
            if name in xgroups:
                br, t0, t1, k = xgroups[name]
                pltpu.make_async_copy(x_v.at[br, t0:t1], x_v.at[br, t0:t1], sems.at[k]).wait()
            else:
                w_cp(name).wait()

    def out_cp(row0, nrows, c0=0, c1=2 * D):
        return pltpu.make_async_copy(ob_v.at[row0:row0 + nrows, c0:c1],
                                     o_hbm.at[0, row0:row0 + nrows, c0:c1], sems.at[2])

    def init():
        start("waq", "xa0", "waq2", "xa02", "wak", "wav", "wb", "xb0", "woa", "wob")
        row = lax.broadcasted_iota(jnp.int32, (64, T), 0)
        col = lax.broadcasted_iota(jnp.int32, (64, T), 1)
        real = (jnp.logical_or((row & 31) < 14, (row & 31) >= 18),
                jnp.logical_or((col & 63) < 28, (col & 63) >= 36))
        code = ((row >> 4) + (col >> 5)) & 3
        for c in range(4):
            for f in range(2):
                qm_ref[f, c] = jnp.where(jnp.logical_and(real[f], code == c),
                                         jnp.uint32(0xFFFFFFFF), jnp.uint32(0))
            p_refs[c][ZP, 0] = jnp.zeros((16, 2 * T), bf16)
        vT_ref[1, 0, 192:256, :] = jnp.zeros((64, T), u32)
        ob_v[S:S + 16, 0:T] = jnp.zeros((16, T), bf16)
        oa_ref[0] = jnp.zeros((64, T), f32)

    zs = (step >> 10, step >> 11)
    zw, zr = zs

    mk = {}

    def make_masks():
        lane = lax.broadcasted_iota(jnp.int32, (SB, T), 1)
        mk["tri"] = lax.broadcasted_iota(jnp.int32, (SB, T), 0) <= (lane & (SB - 1))
        for n in (4, 1):
            lane = lax.broadcasted_iota(jnp.int32, (n, 8, 2 * T), 2)
            mk["odd", n] = (lane & SB) != 0
            mk["hi", n] = (lane & (2 * SB)) != 0
        key = lax.broadcasted_iota(jnp.int32, (1, 8, 2 * T), 1) + ((lane >> 7) << 4)
        for e in range(2):
            mk["tri", e] = key + 8 * e <= (lane & (SB - 1))

    zero2 = jnp.zeros((1, 8, 2 * T), bf16)
    zero8 = jnp.zeros((8, T), u32)

    def slack(z, r0):
        for r in (r0, r0 + 8):
            tmp_ref[r:r + 8, :] = z
            z = tmp_ref[r:r + 8, :]
        return z

    def ties(items, nrounds, t0, t1, extra=()):
        out = []
        done = 0
        for v in range(nrounds):
            zv = None
            if t0 <= v < t1:
                upto = (len(items) * (v - t0 + 1)) // (t1 - t0)
                if upto > done:
                    gs = sorted({it() for it in items[done:upto]})
                    done = upto
                    zv = slack(functools.reduce(jnp.bitwise_or, [
                        pltpu.bitcast(p_refs[g][ZP, 0, :, 0:T], u32) for g in gs]), 0)
            out.append(zv)
        for v, z in extra:
            out[v] = z if out[v] is None else out[v] | z
        if all(z is None for z in out):
            return None
        return jnp.concatenate([zero8 if z is None else z for z in out], axis=0)

    def pad_heads(a, fill=None):
        parts = []
        for p in range(a.shape[0] // 56):
            b = a[56 * p:56 * p + 56]
            mid = b[24:32]
            if fill is None:
                parts += [b[0:32], b[24:56]]
            else:
                m = lax.broadcasted_iota(jnp.int32, mid.shape, 0) < 4
                parts += [b[0:24], jnp.where(m, mid, fill), jnp.where(m, fill, mid), b[32:56]]
        return jnp.concatenate(parts, axis=0)

    def roll_heads(a, back):
        parts = []
        for h in range(a.shape[0] // 16):
            j = h % 4
            b = a[16 * h:16 * h + 16]
            parts.append(b if j == 0 else pltpu.roll(b, SB * j if back else T - SB * j, 1))
        return jnp.concatenate(parts, axis=0)

    def moff(i, n):
        return i * n if isinstance(i, int) else pl.multiple_of(i * n, n)

    def prep_w(br, c0, c1):
        w = jnp.concatenate([wq_v[br, :, c0:c1], jnp.zeros((64, c1 - c0), bf16)], axis=0)
        wt_ref[br, c0 // 2:c1 // 2, :] = pltpu.bitcast(w.T, u32)

    def prep_wo(br):
        w = pad_heads(wo_v[br].astype(f32), 0.0).astype(bf16)
        wt_ref[br, 3 * D // 2:2 * D, :] = pltpu.bitcast(w.T, u32)

    def project(br, part, rhs, items, t0, extra=()):
        zv = ties(items, NR, t0, NR, extra)
        w = wt_ref[br, part * (D // 2):(part + 1) * (D // 2), :]
        if zv is not None:
            w = w | jnp.concatenate([zv] * 4, axis=1)
        return jnp.dot(_ubf(w), rhs, preferred_element_type=f32)

    def xtile(br, i):
        return jnp.concatenate([x_v[br, i], jnp.zeros((64, T), bf16)], axis=0)

    def put_q(br, slot, y, hf=0):
        y = pad_heads(y * QSCALE)
        n = y.shape[0]
        if slot is None:
            q_ref[br, :, n * hf:n * (hf + 1)] = pltpu.bitcast(y.astype(bf16).T, u32)
        else:
            qT_ref[slot, n // 2 * hf:n // 2 * (hf + 1), :] = roll_heads(_pk(y), False)

    def proj_q(br, i, items=(), t0=TIE0, slot=None):
        put_q(br, slot, project(br, 0, xtile(br, i), items, t0))

    def proj_q_half(i, hf, slot, mid=()):
        y = jnp.dot(_ubf(wt_ref[0, 112 * hf:112 * hf + 112, :]), xtile(0, i),
                    preferred_element_type=f32)
        wait(*mid)
        put_q(0, slot, y, hf)

    def proj_k(br, i, items=(), t0=TIE0):
        kT = pad_heads(project(br, 1, xtile(br, i), items, t0))
        for gp in range(2):
            kt = pltpu.bitcast(kT[2 * T * gp:2 * T * (gp + 1)].astype(bf16).T, u32)
            for gg in range(2):
                k_ref[br, 2 * gp + gg, pl.ds(moff(i, 64), 64), :] = kt[:, T * gg:T * (gg + 1)]

    def proj_v(br, i, items=(), t0=TIE0, mid=(), extra=()):
        vT = project(br, 2, xtile(br, i), items, t0, extra)
        wait(*mid)
        vT_ref[br, i + 1] = _pk(pad_heads(vT, 1.0))

    def proj_o(br, i, items=(), t0=TIE0, slot=None, aslot=0, full=False, extra=()):
        o = project(br, 3, _ubf(oT_ref[br if slot is None else slot]), items, t0, extra)
        row0 = moff(i, T)
        if full:
            ob_v[pl.ds(row0, T), 0:D] = o.astype(bf16).T
        elif br == 0:
            ob_v[pl.ds(row0, T), 0:384] = o[0:384].astype(bf16).T
            oa_ref[aslot] = o[384:448]
        else:
            ob_v[pl.ds(row0, T), 384:896] = jnp.concatenate(
                [oa_ref[aslot], o], axis=0).astype(bf16).T

    def ntiles(i):
        return min(3, i + 1) if isinstance(i, int) else 3

    def qk(br, i, g, items=(), t0=1, t1=18, zero_fill=False, slot=None, col=0,
           late=False, extra=()):
        s_ref = s_refs[g]
        nt = ntiles(i)
        late = late or nt < 3
        zv = ties(items, 18, t0, t1, extra)
        if slot is None:
            q = q_ref[br, :, T * g:T * (g + 1)]
        else:
            q = qT_ref[slot, 64 * g:64 * g + 64, :]
        ms = [None] * 4
        for c in (range(4) if g % 2 == 0 else range(3, -1, -1)):
            n = min(WIN // 2, 64 * (nt - 1) + 16 * c)
            ks = k_ref[br, g, pl.ds(moff(i, 64) + (16 * c - n), n + 16), :]
            if n > 0:
                ks = jnp.concatenate([ks[n:], ks[:n]], axis=0)
            if zv is not None:
                ks = ks | (zv if nt == 3 else zv[:n + 16])
            if slot is None:
                w = jnp.concatenate([q[16 * c:16 * c + 16]] * 4, axis=0) & qm_ref[1, c]
                s = lax.dot_general(_ubf(ks), _ubf(w), (((1,), (1,)), ((), ())),
                                    preferred_element_type=f32)
            else:
                s = jnp.dot(_ubf(ks), _ubf(q & qm_ref[0, c]), preferred_element_type=f32)
            r0 = 2 * SB if nt == 3 else SB
            dg = jnp.where(mk["tri"], s[0:SB], s[SB:r0] if nt == 3 else NEG)
            r1 = s.shape[0] - SB * c

            def put_s(b0, rows):
                nb = rows.shape[0] // SB
                blk = rows.reshape(nb, 4, 8, T)
                blk = jnp.concatenate([blk[:, 0:2], blk[:, 2:4]], axis=3)
                s_ref[pl.ds(zw + 2 * b0, 2 * nb), c] = blk.reshape(2 * nb, 8, 2 * T)
            put_s(0, jnp.concatenate([s[r1:], dg], axis=0) if c > 0 else dg)
            if r1 > r0:
                put_s(8 - (r1 - r0) // SB, s[r0:r1])
            sm = jnp.concatenate([dg, s[r0:]], axis=0) if s.shape[0] > r0 else dg
            ms[c] = jnp.broadcast_to(jnp.max(sm, axis=0, keepdims=True), (8, T))
            if late:
                s_ref[zw + MS, c, :, 0:T] = ms[c]

        return sm_items(g, nt, None if late else jnp.stack(ms), zero_fill, col)

    def sm_items(g, nt=3, mall=None, zero_fill=False, col=0):
        s_ref, p_ref = s_refs[g], p_refs[g]

        def sel(m, a, b):
            if a is None and b is None:
                return None
            return lax.select(m, zero2 if a is None else a, zero2 if b is None else b)

        def put_p(b, e, x):
            if isinstance(x, list):
                x = [sel(mk["odd", 1], x[(j + 1) % 4], x[j]) for j in range(4)]
                x = jnp.concatenate(
                    [sel(mk["hi", 1], x[(j + 2) % 4], x[j]) for j in range(4)], axis=0)
            else:
                x = lax.select(mk["odd", 4], jnp.concatenate([x[1:], x[:1]], axis=0), x)
                x = lax.select(mk["hi", 4], jnp.concatenate([x[2:], x[:2]], axis=0), x)
            p_ref[zs[col] + b, :, 8 * e:8 * e + 8, :] = x

        def item(rho):
            b, e = rho // 2, rho % 2
            c0 = b if nt < 3 and rho < 8 else 0
            m = s_ref[zr + MS, c0:4, :, 0:T] if mall is None else mall
            x = jnp.exp2(s_ref[zr + rho, c0:4] - jnp.concatenate([m, m], axis=2)).astype(bf16)
            if rho < 8:
                x = [None] * c0 + [x[c:c + 1] for c in range(4 - c0)]
            if rho >= 8 or nt == 1:
                put_p(b, e, x)
            elif nt == 3:
                tri = mk["tri", e]
                put_p(b + 8, e, [None] * b + [sel(tri, x[b], None)] + x[b + 1:])
                put_p(b, e, x[:b] + [sel(tri, None, x[b])] + [None] * (3 - b))
            else:
                put_p(b + 8, e, x)
                if zero_fill:
                    p_ref[zs[col] + b, :, 8 * e:8 * e + 8, :] = jnp.zeros((4, 8, 2 * T), bf16)
            return g
        order = list(range(8, 16 if nt > 1 else 8)) + list(range(8))
        return [functools.partial(item, rho) for rho in order]

    def pv(br, i, g, slot=None, col=0):
        nt = ntiles(i)
        acc = [None] * 4
        for t in range(3 - nt, 3):
            vv = _ubf(vT_ref[br, i - 1 + t, 64 * g:64 * g + 64, :])
            bs = pl.ds(zs[1 - col] + (0 if nt == 1 else 4 * t), 4)
            for j in range(4):
                pj = jnp.concatenate([p_refs[g][bs, j, :, 0:T], p_refs[g][bs, j, :, T:2 * T]],
                                     axis=1).reshape(T, T)
                o = jnp.dot(vv[32 * j:32 * j + 32], pj, preferred_element_type=f32)
                acc[j] = o if acc[j] is None else acc[j] + o
        og = jnp.concatenate(
            [acc[j] * pl.reciprocal(acc[j][28:29] if j % 2 == 0 else acc[j][0:1], approx=False)
             for j in range(4)], axis=0)
        oT_ref[br if slot is None else slot, 64 * g:64 * g + 64, :] = roll_heads(_pk(og), True)

    def units(i0, n, cut):
        items = sm_items(0)
        for u in range(1, n + 1):
            i, br, g = i0 + u // 8, u // 4 % 2, u % 4
            pb, pg = (br, g - 1) if g > 0 else (1 - br, 3)
            pi = i if u % 8 > 0 else i - 1
            if pg == 2:
                proj_o(1 - pb, pi - 1 + pb, items[:NF])
            elif pg == 3:
                zo = pltpu.bitcast(ob_v[pl.ds(moff(zr, 16) + S, 16), 0:T], u32)
                proj_v(1 - pb, pi + pb, items[:NF], extra=[(OTIE, slack(zo, 16))])
            else:
                (proj_k, proj_q)[pg](1 - pb, pi + pb, items[:NF], 2 if u == 1 else TIE0)
            last = cut and u == n
            do_pv = functools.partial(pv, br, i, g - 2) if g > 1 else functools.partial(
                pv, 1 - br, i - 1 + br, g + 2)
            if last:
                do_pv()
            items = qk(br, i, g, items[NF:], late=last)
            if not last:
                do_pv()
        return items

    def first():
        make_masks()
        wait("waq")
        prep_w(0, 0, 256)
        start("xb1", "xa1", "xb2", "xa2")
        wait("xa0")
        proj_q_half(0, 0, 0)
        proj_q_half(1, 0, 1, mid=("waq2", "xa02"))
        prep_w(0, 256, 512)
        proj_q_half(2, 0, None)
        proj_q_half(0, 1, 0)
        proj_q_half(1, 1, 1, mid=("wak",))
        prep_w(0, 512, 896)
        proj_q_half(2, 1, None)
        proj_k(0, 0)
        proj_k(0, 1)
        it = sum([qk(0, 0, g, slot=0, col=1) for g in range(4)], [])
        proj_k(0, 2, it, 4)
        it0 = qk(0, 1, 0, slot=1)
        it1 = qk(0, 1, 1, slot=1)
        wait("wav")
        prep_w(0, 896, 1344)
        it2 = qk(0, 1, 2, it0[:8], 1, 10, slot=1)
        it3 = qk(0, 1, 3, it0[8:], 1, 10, slot=1)
        proj_v(0, 0, it1, 1)
        proj_v(0, 1, it2, 1, mid=("wb", "xb0"))
        prep_w(1, 384, 896)
        prep_w(1, 0, 384)
        prep_w(1, 896, 1344)
        for g in range(4):
            pv(0, 0, g, slot=2, col=1)
        for g in range(3):
            pv(0, 1, g, slot=4)
        proj_k(1, 0, it3, 11)
        proj_q(1, 0, slot=0)
        proj_k(1, 1)
        it = sum([qk(1, 0, g, slot=0, col=1) for g in range(4)], [])
        pv(0, 1, 3, slot=4)
        proj_q(1, 1, it, 2, slot=1)
        proj_v(1, 0)
        it = qk(1, 1, 0, slot=1)
        it = it + qk(1, 1, 1, slot=1)
        it = it[9:] + qk(1, 1, 2, it[:9], 1, 10, slot=1)
        it3 = qk(1, 1, 3, it[:12], 1, 10, zero_fill=True, slot=1)
        for g in range(4):
            pv(1, 0, g, slot=3, col=1)
        proj_v(1, 1, it[12:], 10)
        proj_v(0, 2, it3, 1)
        for g in range(3):
            pv(1, 1, g)
        qk(0, 2, 0, late=True)
        wait("woa", "wob", "xb1", "xa1")

    def steady(n, carry):
        make_masks()
        prep_wo(1)
        prep_wo(0)
        units(2 + n * U, 8 * U, True)

        @pl.when(n == 0)
        def _():
            out_cp(2 * T, (U - 1) * T).start()
            wait("xb2", "xa2")

        for k in range(1, NLOOP):
            pl.when(n == k)(out_cp((1 + k * U) * T, U * T).start)
        return carry

    def last():
        make_masks()
        i = NT - 1
        r0 = i * T
        it = units(i - 1, 11, False)
        proj_v(1, i, it[:NF])
        out_cp((NT - 3) * T, 2 * T).start()

        def dma_tie():
            ob_v[pl.ds(moff(zw, 16) + r0, 16), 512:640] = jnp.zeros((16, T), bf16)
            return pltpu.bitcast(ob_v[pl.ds(moff(zr, 16) + r0, 16), 512:640], u32)

        def o_part(g):
            sets = ([4, 5, 6, 7, 8, 9, 10], [12, 13, 14, 15, 16, 17, 18],
                    [20, 21, 22, 23, 24, 25, 26], [0, 1, 2, 3, 11, 19, 27])
            w = wt_ref[1, 3 * D // 2:2 * D, T * g:T * (g + 1)]
            rhs = _ubf(oT_ref[1, 64 * g:64 * g + 64, :])
            res = {}
            for rows in sets:
                lhs = jnp.concatenate([w[8 * v:8 * v + 8] for v in rows], axis=0)
                y = jnp.dot(_ubf(lhs), rhs, preferred_element_type=f32)
                for n, v in enumerate(rows):
                    res[v] = y[16 * n:16 * n + 16]
            return jnp.concatenate([res[v] for v in range(NR)], axis=0)

        it = qk(1, i, 0, it[NF:], late=True, extra=[(17, dma_tie())])
        pv(0, i, 2)
        proj_o(0, 0, it[:NF], slot=2, aslot=1)
        it = qk(1, i, 1, it[NF:], late=True)
        pv(0, i, 3)
        proj_o(1, 0, it[:NF], slot=3, aslot=1)
        out_cp(0, T).start()
        it = qk(1, i, 2, it[NF:], late=True)
        it = it[5:] + qk(1, i, 3, it[:5], 12, late=True, extra=[(17, dma_tie())])
        proj_o(0, 1, it[:15], 0, slot=4, full=True)
        out_cp(T, T).start()
        pv(1, i, 0)
        proj_o(0, i, it[15:], 0, extra=[(NR - 1, dma_tie())])
        out_cp(r0, T, 0, 384).start()
        zd = dma_tie()
        for g in range(1, 4):
            pv(1, i, g)
        o = o_part(0) + o_part(1) + o_part(2) + o_part(3)
        oa = pltpu.bitcast(pltpu.bitcast(oa_ref[0, 0:8, :], u32) | zd, f32)
        ot = jnp.concatenate([oa, oa_ref[0, 8:64, :], o], axis=0).astype(bf16).T
        for a in range(r0, S, 32):
            ob_v[a:a + 32, 384:896] = ot[a - r0:a - r0 + 32]
            out_cp(a, 32, 384, 896).start()
        out_cp(0, S).wait()

    pl.when(step == 0)(init)

    @pl.when(step == 1)
    def _():
        first()
        lax.fori_loop(0, NLOOP, steady, 0)
        last()


@jax.jit
def pallas_concat_heads__sliding_block__sliding_block__prompt_kernel(
        A_x, A_wqkv, A_wo, B_x, B_wqkv, B_wo):
    anyspec = pl.BlockSpec(memory_space=pl.ANY)
    return pl.pallas_call(
        _kernel,
        grid=(2,),
        in_specs=[anyspec] * 6,
        out_specs=anyspec,
        out_shape=jax.ShapeDtypeStruct((1, S, 2 * D), bf16),
        scratch_shapes=[
            pltpu.VMEM((2, NT, D, T), bf16),
            pltpu.VMEM((2, D, 3 * D), bf16),
            pltpu.VMEM((2, D, D), bf16),
            pltpu.VMEM((S + 64, 2 * D), bf16),
            pltpu.VMEM((2, 2 * D, 4 * T), u32),
            pltpu.VMEM((2, 4, S // 2, T), u32),
            pltpu.VMEM((2, NT + 1, 256, T), u32),
            pltpu.VMEM((2, 256, T), u32),
            pltpu.VMEM((2, 64, 4 * T), u32),
            pltpu.VMEM((5, 256, T), u32),
            pltpu.VMEM((2, 64, T), f32),
        ] + [pltpu.VMEM((MS + 1, 4, 8, 2 * T), f32)] * 4
        + [pltpu.VMEM((ZP + 1, 4, 16, 2 * T), bf16)] * 4
        + [
            pltpu.VMEM((2, 4, 64, T), u32),
            pltpu.VMEM((32, T), u32),
            pltpu.SemaphoreType.DMA((7,)),
        ],
        compiler_params=pltpu.CompilerParams(
            dimension_semantics=("arbitrary",),
            vmem_limit_bytes=64 * 1024 * 1024),
        name="swa",
    )(jnp.swapaxes(A_x, 1, 2), A_wqkv, A_wo, jnp.swapaxes(B_x, 1, 2), B_wqkv, B_wo)
```

```python
import functools

import jax
import jax.numpy as jnp
from jax import lax
import jax.experimental.pallas as pl
import jax.experimental.pallas.tpu as pltpu

S, D, H, DH, WIN = 2048, 448, 16, 28, 256
T = 128
NT = S // T
U = 4
NLOOP = (NT - 4) // U
QSCALE = (DH ** -0.5) * 1.4426950408889634
NEG = -1e30
SB = 32
NR = D // 16
ZP = 12
MS = 16
TIE0 = 12
NF = 9
OTIE = 14

f32, bf16, u32 = jnp.float32, jnp.bfloat16, jnp.uint32


def _pk(x):
    return pltpu.bitcast(x.astype(bf16), u32)


def _ubf(x):
    return pltpu.bitcast(x, bf16)


def _kernel(xa_hbm, wqa_hbm, woa_hbm, xb_hbm, wqb_hbm, wob_hbm, o_hbm,
            x_v, wq_v, wo_v, ob_v, wt_ref, k_ref, vT_ref, qT_ref, q_ref, oT_ref, oa_ref,
            s0_ref, s1_ref, s2_ref, s3_ref, p0_ref, p1_ref, p2_ref, p3_ref,
            qm_ref, tmp_ref, sems):
    step = pl.program_id(0)
    s_refs = (s0_ref, s1_ref, s2_ref, s3_ref)
    p_refs = (p0_ref, p1_ref, p2_ref, p3_ref)

    def w_cp(name):
        src, dst, k = {
            "waq": (wqa_hbm.at[:, 0:256], wq_v.at[0, :, 0:256], 0),
            "waq2": (wqa_hbm.at[:, 256:512], wq_v.at[0, :, 256:512], 1),
            "wak": (wqa_hbm.at[:, 512:896], wq_v.at[0, :, 512:896], 2),
            "wav": (wqa_hbm.at[:, 896:1344], wq_v.at[0, :, 896:1344], 3),
            "wb": (wqb_hbm, wq_v.at[1], 4),
            "woa": (woa_hbm, wo_v.at[0], 5),
            "wob": (wob_hbm, wo_v.at[1], 5),
        }[name]
        return pltpu.make_async_copy(src, dst, sems.at[k])

    xgroups = {
        "xa0": (0, 0, 2, 6), "xa02": (0, 2, 3, 1), "xb0": (1, 0, 2, 4),
        "xb1": (1, 2, 2 + U, 5), "xa1": (0, 3, 3 + U, 5),
        "xb2": (1, 2 + U, NT, 0), "xa2": (0, 3 + U, NT, 0),
    }

    def start(*names):
        for name in names:
            if name in xgroups:
                br, t0, t1, k = xgroups[name]
                for t in range(t0, t1):
                    pltpu.make_async_copy((xa_hbm, xb_hbm)[br].at[0, :, t * T:(t + 1) * T],
                                          x_v.at[br, t], sems.at[k]).start()
            else:
                w_cp(name).start()

    def wait(*names):
        for name in names:
            if name in xgroups:
                br, t0, t1, k = xgroups[name]
                pltpu.make_async_copy(x_v.at[br, t0:t1], x_v.at[br, t0:t1], sems.at[k]).wait()
            else:
                w_cp(name).wait()

    def out_cp(row0, nrows, c0=0, c1=2 * D):
        return pltpu.make_async_copy(ob_v.at[row0:row0 + nrows, c0:c1],
                                     o_hbm.at[0, row0:row0 + nrows, c0:c1], sems.at[2])

    def init():
        start("waq", "xa0", "waq2", "xa02", "wak", "wav", "wb", "xb0", "woa", "wob")
        row = lax.broadcasted_iota(jnp.int32, (64, T), 0)
        col = lax.broadcasted_iota(jnp.int32, (64, T), 1)
        real = (jnp.logical_or((row & 31) < 14, (row & 31) >= 18),
                jnp.logical_or((col & 63) < 28, (col & 63) >= 36))
        code = ((row >> 4) + (col >> 5)) & 3
        for c in range(4):
            for f in range(2):
                qm_ref[f, c] = jnp.where(jnp.logical_and(real[f], code == c),
                                         jnp.uint32(0xFFFFFFFF), jnp.uint32(0))
            p_refs[c][ZP, 0] = jnp.zeros((16, 2 * T), bf16)
        vT_ref[1, 0, 192:256, :] = jnp.zeros((64, T), u32)
        ob_v[S:S + 16, 0:T] = jnp.zeros((16, T), bf16)
        oa_ref[0] = jnp.zeros((64, T), f32)

    zs = (step >> 10, step >> 11)
    zw, zr = zs

    mk = {}

    def make_masks():
        lane = lax.broadcasted_iota(jnp.int32, (SB, T), 1)
        mk["tri"] = lax.broadcasted_iota(jnp.int32, (SB, T), 0) <= (lane & (SB - 1))
        for n in (4, 1):
            lane = lax.broadcasted_iota(jnp.int32, (n, 8, 2 * T), 2)
            mk["odd", n] = (lane & SB) != 0
            mk["hi", n] = (lane & (2 * SB)) != 0
        key = lax.broadcasted_iota(jnp.int32, (1, 8, 2 * T), 1) + ((lane >> 7) << 4)
        for e in range(2):
            mk["tri", e] = key + 8 * e <= (lane & (SB - 1))

    zero2 = jnp.zeros((1, 8, 2 * T), bf16)
    zero8 = jnp.zeros((8, T), u32)

    def slack(z, r0):
        for r in (r0, r0 + 8):
            tmp_ref[r:r + 8, :] = z
            z = tmp_ref[r:r + 8, :]
        return z

    def ties(items, nrounds, t0, t1, extra=()):
        out = []
        done = 0
        for v in range(nrounds):
            zv = None
            if t0 <= v < t1:
                upto = (len(items) * (v - t0 + 1)) // (t1 - t0)
                if upto > done:
                    gs = sorted({it() for it in items[done:upto]})
                    done = upto
                    zv = slack(functools.reduce(jnp.bitwise_or, [
                        pltpu.bitcast(p_refs[g][ZP, 0, :, 0:T], u32) for g in gs]), 0)
            out.append(zv)
        for v, z in extra:
            out[v] = z if out[v] is None else out[v] | z
        if all(z is None for z in out):
            return None
        return jnp.concatenate([zero8 if z is None else z for z in out], axis=0)

    def pad_heads(a, fill=None):
        parts = []
        for p in range(a.shape[0] // 56):
            b = a[56 * p:56 * p + 56]
            mid = b[24:32]
            if fill is None:
                parts += [b[0:32], b[24:56]]
            else:
                m = lax.broadcasted_iota(jnp.int32, mid.shape, 0) < 4
                parts += [b[0:24], jnp.where(m, mid, fill), jnp.where(m, fill, mid), b[32:56]]
        return jnp.concatenate(parts, axis=0)

    def roll_heads(a, back):
        parts = []
        for h in range(a.shape[0] // 16):
            j = h % 4
            b = a[16 * h:16 * h + 16]
            parts.append(b if j == 0 else pltpu.roll(b, SB * j if back else T - SB * j, 1))
        return jnp.concatenate(parts, axis=0)

    def moff(i, n):
        return i * n if isinstance(i, int) else pl.multiple_of(i * n, n)

    def prep_w(br, c0, c1):
        w = jnp.concatenate([wq_v[br, :, c0:c1], jnp.zeros((64, c1 - c0), bf16)], axis=0)
        wt_ref[br, c0 // 2:c1 // 2, :] = pltpu.bitcast(w.T, u32)

    def prep_wo(br):
        w = pad_heads(wo_v[br].astype(f32), 0.0).astype(bf16)
        wt_ref[br, 3 * D // 2:2 * D, :] = pltpu.bitcast(w.T, u32)

    def project(br, part, rhs, items, t0, extra=()):
        zv = ties(items, NR, t0, NR, extra)
        w = wt_ref[br, part * (D // 2):(part + 1) * (D // 2), :]
        if zv is not None:
            w = w | jnp.concatenate([zv] * 4, axis=1)
        return jnp.dot(_ubf(w), rhs, preferred_element_type=f32)

    def xtile(br, i):
        return jnp.concatenate([x_v[br, i], jnp.zeros((64, T), bf16)], axis=0)

    def put_q(br, slot, y, hf=0):
        y = pad_heads(y * QSCALE)
        n = y.shape[0]
        if slot is None:
            q_ref[br, :, n * hf:n * (hf + 1)] = pltpu.bitcast(y.astype(bf16).T, u32)
        else:
            qT_ref[slot, n // 2 * hf:n // 2 * (hf + 1), :] = roll_heads(_pk(y), False)

    def proj_q(br, i, items=(), t0=TIE0, slot=None):
        put_q(br, slot, project(br, 0, xtile(br, i), items, t0))

    def proj_q_half(i, hf, slot, mid=()):
        y = jnp.dot(_ubf(wt_ref[0, 112 * hf:112 * hf + 112, :]), xtile(0, i),
                    preferred_element_type=f32)
        wait(*mid)
        put_q(0, slot, y, hf)

    def proj_k(br, i, items=(), t0=TIE0):
        kT = pad_heads(project(br, 1, xtile(br, i), items, t0))
        for gp in range(2):
            kt = pltpu.bitcast(kT[2 * T * gp:2 * T * (gp + 1)].astype(bf16).T, u32)
            for gg in range(2):
                k_ref[br, 2 * gp + gg, pl.ds(moff(i, 64), 64), :] = kt[:, T * gg:T * (gg + 1)]

    def proj_v(br, i, items=(), t0=TIE0, mid=(), extra=()):
        vT = project(br, 2, xtile(br, i), items, t0, extra)
        wait(*mid)
        vT_ref[br, i + 1] = _pk(pad_heads(vT, 1.0))

    def proj_o(br, i, items=(), t0=TIE0, slot=None, aslot=0, extra=()):
        o = project(br, 3, _ubf(oT_ref[br if slot is None else slot]), items, t0, extra)
        row0 = moff(i, T)
        if br == 0:
            ob_v[pl.ds(row0, T), 0:384] = o[0:384].astype(bf16).T
            oa_ref[aslot] = o[384:448]
        else:
            ob_v[pl.ds(row0, T), 384:896] = jnp.concatenate(
                [oa_ref[aslot], o], axis=0).astype(bf16).T

    def ntiles(i):
        return min(3, i + 1) if isinstance(i, int) else 3

    def qk(br, i, g, items=(), t0=1, t1=18, zero_fill=False, slot=None, col=0,
           late=False, extra=()):
        s_ref = s_refs[g]
        nt = ntiles(i)
        late = late or nt < 3
        zv = ties(items, 18, t0, t1, extra)
        if slot is None:
            q = q_ref[br, :, T * g:T * (g + 1)]
        else:
            q = qT_ref[slot, 64 * g:64 * g + 64, :]
        ms = [None] * 4
        for c in (range(4) if g % 2 == 0 else range(3, -1, -1)):
            n = min(WIN // 2, 64 * (nt - 1) + 16 * c)
            ks = k_ref[br, g, pl.ds(moff(i, 64) + (16 * c - n), n + 16), :]
            if n > 0:
                ks = jnp.concatenate([ks[n:], ks[:n]], axis=0)
            if zv is not None:
                ks = ks | (zv if nt == 3 else zv[:n + 16])
            if slot is None:
                w = jnp.concatenate([q[16 * c:16 * c + 16]] * 4, axis=0) & qm_ref[1, c]
                s = lax.dot_general(_ubf(ks), _ubf(w), (((1,), (1,)), ((), ())),
                                    preferred_element_type=f32)
            else:
                s = jnp.dot(_ubf(ks), _ubf(q & qm_ref[0, c]), preferred_element_type=f32)
            r0 = 2 * SB if nt == 3 else SB
            dg = jnp.where(mk["tri"], s[0:SB], s[SB:r0] if nt == 3 else NEG)
            r1 = s.shape[0] - SB * c

            def put_s(b0, rows):
                nb = rows.shape[0] // SB
                blk = rows.reshape(nb, 4, 8, T)
                blk = jnp.concatenate([blk[:, 0:2], blk[:, 2:4]], axis=3)
                s_ref[pl.ds(zw + 2 * b0, 2 * nb), c] = blk.reshape(2 * nb, 8, 2 * T)
            put_s(0, jnp.concatenate([s[r1:], dg], axis=0) if c > 0 else dg)
            if r1 > r0:
                put_s(8 - (r1 - r0) // SB, s[r0:r1])
            sm = jnp.concatenate([dg, s[r0:]], axis=0) if s.shape[0] > r0 else dg
            ms[c] = jnp.broadcast_to(jnp.max(sm, axis=0, keepdims=True), (8, T))
            if late:
                s_ref[zw + MS, c, :, 0:T] = ms[c]

        return sm_items(g, nt, None if late else jnp.stack(ms), zero_fill, col)

    def sm_items(g, nt=3, mall=None, zero_fill=False, col=0):
        s_ref, p_ref = s_refs[g], p_refs[g]

        def sel(m, a, b):
            if a is None and b is None:
                return None
            return lax.select(m, zero2 if a is None else a, zero2 if b is None else b)

        def put_p(b, e, x):
            if isinstance(x, list):
                x = [sel(mk["odd", 1], x[(j + 1) % 4], x[j]) for j in range(4)]
                x = jnp.concatenate(
                    [sel(mk["hi", 1], x[(j + 2) % 4], x[j]) for j in range(4)], axis=0)
            else:
                x = lax.select(mk["odd", 4], jnp.concatenate([x[1:], x[:1]], axis=0), x)
                x = lax.select(mk["hi", 4], jnp.concatenate([x[2:], x[:2]], axis=0), x)
            p_ref[zs[col] + b, :, 8 * e:8 * e + 8, :] = x

        def item(rho):
            b, e = rho // 2, rho % 2
            c0 = b if nt < 3 and rho < 8 else 0
            m = s_ref[zr + MS, c0:4, :, 0:T] if mall is None else mall
            x = jnp.exp2(s_ref[zr + rho, c0:4] - jnp.concatenate([m, m], axis=2)).astype(bf16)
            if rho < 8:
                x = [None] * c0 + [x[c:c + 1] for c in range(4 - c0)]
            if rho >= 8 or nt == 1:
                put_p(b, e, x)
            elif nt == 3:
                tri = mk["tri", e]
                put_p(b + 8, e, [None] * b + [sel(tri, x[b], None)] + x[b + 1:])
                put_p(b, e, x[:b] + [sel(tri, None, x[b])] + [None] * (3 - b))
            else:
                put_p(b + 8, e, x)
                if zero_fill:
                    p_ref[zs[col] + b, :, 8 * e:8 * e + 8, :] = jnp.zeros((4, 8, 2 * T), bf16)
            return g
        order = list(range(8, 16 if nt > 1 else 8)) + list(range(8))
        return [functools.partial(item, rho) for rho in order]

    def pv(br, i, g, slot=None, col=0):
        nt = ntiles(i)
        acc = [None] * 4
        for t in range(3 - nt, 3):
            vv = _ubf(vT_ref[br, i - 1 + t, 64 * g:64 * g + 64, :])
            bs = pl.ds(zs[1 - col] + (0 if nt == 1 else 4 * t), 4)
            for j in range(4):
                pj = jnp.concatenate([p_refs[g][bs, j, :, 0:T], p_refs[g][bs, j, :, T:2 * T]],
                                     axis=1).reshape(T, T)
                o = jnp.dot(vv[32 * j:32 * j + 32], pj, preferred_element_type=f32)
                acc[j] = o if acc[j] is None else acc[j] + o
        og = jnp.concatenate(
            [acc[j] * pl.reciprocal(acc[j][28:29] if j % 2 == 0 else acc[j][0:1], approx=False)
             for j in range(4)], axis=0)
        oT_ref[br if slot is None else slot, 64 * g:64 * g + 64, :] = roll_heads(_pk(og), True)

    def units(i0, n, cut):
        items = sm_items(0)
        for u in range(1, n + 1):
            i, br, g = i0 + u // 8, u // 4 % 2, u % 4
            pb, pg = (br, g - 1) if g > 0 else (1 - br, 3)
            pi = i if u % 8 > 0 else i - 1
            if pg == 2:
                proj_o(1 - pb, pi - 1 + pb, items[:NF])
            elif pg == 3:
                zo = pltpu.bitcast(ob_v[pl.ds(moff(zr, 16) + S, 16), 0:T], u32)
                proj_v(1 - pb, pi + pb, items[:NF], extra=[(OTIE, slack(zo, 16))])
            else:
                (proj_k, proj_q)[pg](1 - pb, pi + pb, items[:NF], 2 if u == 1 else TIE0)
            last = cut and u == n
            do_pv = functools.partial(pv, br, i, g - 2) if g > 1 else functools.partial(
                pv, 1 - br, i - 1 + br, g + 2)
            if last:
                do_pv()
            items = qk(br, i, g, items[NF:], late=last)
            if not last:
                do_pv()
        return items

    def first():
        make_masks()
        wait("waq")
        prep_w(0, 0, 256)
        start("xb1", "xa1", "xb2", "xa2")
        wait("xa0")
        proj_q_half(0, 0, 0)
        proj_q_half(1, 0, 1, mid=("waq2", "xa02"))
        prep_w(0, 256, 512)
        proj_q_half(2, 0, None)
        proj_q_half(0, 1, 0)
        proj_q_half(1, 1, 1, mid=("wak",))
        prep_w(0, 512, 896)
        proj_q_half(2, 1, None)
        proj_k(0, 0)
        proj_k(0, 1)
        it = sum([qk(0, 0, g, slot=0, col=1) for g in range(4)], [])
        proj_k(0, 2, it, 4)
        it0 = qk(0, 1, 0, slot=1)
        it1 = qk(0, 1, 1, slot=1)
        wait("wav")
        prep_w(0, 896, 1344)
        it2 = qk(0, 1, 2, it0[:8], 1, 10, slot=1)
        it3 = qk(0, 1, 3, it0[8:], 1, 10, slot=1)
        proj_v(0, 0, it1, 1)
        proj_v(0, 1, it2, 1, mid=("wb", "xb0"))
        prep_w(1, 384, 896)
        prep_w(1, 0, 384)
        prep_w(1, 896, 1344)
        for g in range(4):
            pv(0, 0, g, slot=2, col=1)
        for g in range(3):
            pv(0, 1, g, slot=4)
        proj_k(1, 0, it3, 11)
        proj_q(1, 0, slot=0)
        proj_k(1, 1)
        it = sum([qk(1, 0, g, slot=0, col=1) for g in range(4)], [])
        pv(0, 1, 3, slot=4)
        proj_q(1, 1, it, 2, slot=1)
        proj_v(1, 0)
        it = qk(1, 1, 0, slot=1)
        it = it + qk(1, 1, 1, slot=1)
        it = it[9:] + qk(1, 1, 2, it[:9], 1, 10, slot=1)
        it3 = qk(1, 1, 3, it[:12], 1, 10, zero_fill=True, slot=1)
        for g in range(4):
            pv(1, 0, g, slot=3, col=1)
        proj_v(1, 1, it[12:], 10)
        proj_v(0, 2, it3, 1)
        for g in range(3):
            pv(1, 1, g)
        qk(0, 2, 0, late=True)
        wait("woa", "wob", "xb1", "xa1")

    def steady(n, carry):
        make_masks()
        prep_wo(1)
        prep_wo(0)
        units(2 + n * U, 8 * U, True)

        @pl.when(n == 0)
        def _():
            out_cp(2 * T, (U - 1) * T).start()
            wait("xb2", "xa2")

        for k in range(1, NLOOP):
            pl.when(n == k)(out_cp((1 + k * U) * T, U * T).start)
        return carry

    def last():
        make_masks()
        i = NT - 1
        r0 = i * T
        it = units(i - 1, 11, False)
        proj_v(1, i, it[:NF])
        out_cp((NT - 3) * T, 2 * T).start()

        def dma_tie():
            ob_v[pl.ds(moff(zw, 16) + S, 16), 0:T] = jnp.zeros((16, T), bf16)
            return pltpu.bitcast(ob_v[pl.ds(moff(zr, 16) + S, 16), 0:T], u32)

        o1 = pltpu.bitcast(_ubf(oT_ref[4]).T, u32)
        out_cp(T, T, 512, 896).start()

        it = qk(1, i, 0, it[NF:], late=True, extra=[(17, dma_tie())])
        pv(0, i, 2)
        it = it[7:] + qk(1, i, 1, it[:7], 9, late=True)
        pv(0, i, 3)
        proj_o(0, 0, it[:12], 0, slot=2, aslot=1)
        it = it[19:] + qk(1, i, 2, it[12:19], 0, late=True)
        it = it[10:] + qk(1, i, 3, it[:10], 0, late=True)
        proj_o(1, 0, it, 0, slot=3, aslot=1)
        out_cp(0, T).start()
        for g in range(4):
            pv(1, i, g)
        proj_o(0, i, extra=[(8, dma_tie())])
        out_cp(r0, T, 0, 384).start()
        o = project(1, 3, _ubf(oT_ref[1]), (), 0, [(NR - 1, dma_tie())])
        ot = jnp.concatenate([oa_ref[0], o], axis=0).astype(bf16).T
        for a in range(0, T, 32):
            ob_v[r0 + a:r0 + a + 32, 384:896] = ot[a:a + 32]
            out_cp(r0 + a, 32, 384, 896).start()
        zd = dma_tie()
        wo = pad_heads(wo_v[0].astype(f32), 0.0).astype(bf16)
        for c0 in range(0, D, T):
            c1 = min(c0 + T, D)
            lhs = o1
            if c1 == D:
                lhs = jnp.concatenate(
                    [o1[0:56], o1[56:64] | jnp.concatenate([zd] * 4, axis=1)], axis=0)
            y = jnp.dot(_ubf(lhs), wo[:, c0:c1], preferred_element_type=f32).astype(bf16)
            for a, b in ((0, T),) if c1 < D else ((0, 64), (64, 96), (96, T)):
                ob_v[T + a:T + b, c0:c1] = y[a:b]
                out_cp(T + a, b - a, c0, c0 + T).start()
        out_cp(0, S).wait()

    pl.when(step == 0)(init)

    @pl.when(step == 1)
    def _():
        first()
        lax.fori_loop(0, NLOOP, steady, 0)
        last()


@jax.jit
def pallas_concat_heads__sliding_block__sliding_block__prompt_kernel(
        A_x, A_wqkv, A_wo, B_x, B_wqkv, B_wo):
    anyspec = pl.BlockSpec(memory_space=pl.ANY)
    return pl.pallas_call(
        _kernel,
        grid=(2,),
        in_specs=[anyspec] * 6,
        out_specs=anyspec,
        out_shape=jax.ShapeDtypeStruct((1, S, 2 * D), bf16),
        scratch_shapes=[
            pltpu.VMEM((2, NT, D, T), bf16),
            pltpu.VMEM((2, D, 3 * D), bf16),
            pltpu.VMEM((2, D, D), bf16),
            pltpu.VMEM((S + 64, 2 * D), bf16),
            pltpu.VMEM((2, 2 * D, 4 * T), u32),
            pltpu.VMEM((2, 4, S // 2, T), u32),
            pltpu.VMEM((2, NT + 1, 256, T), u32),
            pltpu.VMEM((2, 256, T), u32),
            pltpu.VMEM((2, 64, 4 * T), u32),
            pltpu.VMEM((5, 256, T), u32),
            pltpu.VMEM((2, 64, T), f32),
        ] + [pltpu.VMEM((MS + 1, 4, 8, 2 * T), f32)] * 4
        + [pltpu.VMEM((ZP + 1, 4, 16, 2 * T), bf16)] * 4
        + [
            pltpu.VMEM((2, 4, 64, T), u32),
            pltpu.VMEM((32, T), u32),
            pltpu.SemaphoreType.DMA((7,)),
        ],
        compiler_params=pltpu.CompilerParams(
            dimension_semantics=("arbitrary",),
            vmem_limit_bytes=64 * 1024 * 1024),
        name="swa",
    )(jnp.swapaxes(A_x, 1, 2), A_wqkv, A_wo, jnp.swapaxes(B_x, 1, 2), B_wqkv, B_wo)
```

```python
import functools

import jax
import jax.numpy as jnp
from jax import lax
import jax.experimental.pallas as pl
import jax.experimental.pallas.tpu as pltpu

S, D, H, DH, WIN = 2048, 448, 16, 28, 256
T = 128
NT = S // T
U = 4
NLOOP = (NT - 4) // U
QSCALE = (DH ** -0.5) * 1.4426950408889634
NEG = -1e30
SB = 32
NR = D // 16
ZP = 12
MS = 16
TIE0 = 12
NF = 9
OTIE = 14

f32, bf16, u32 = jnp.float32, jnp.bfloat16, jnp.uint32


def _pk(x):
    return pltpu.bitcast(x.astype(bf16), u32)


def _ubf(x):
    return pltpu.bitcast(x, bf16)


def _kernel(xa_hbm, wqa_hbm, woa_hbm, xb_hbm, wqb_hbm, wob_hbm, o_hbm,
            x_v, wq_v, wo_v, ob_v, wt_ref, k_ref, vT_ref, qT_ref, q_ref, oT_ref, oa_ref,
            s0_ref, s1_ref, s2_ref, s3_ref, p0_ref, p1_ref, p2_ref, p3_ref,
            qm_ref, tmp_ref, sems):
    step = pl.program_id(0)
    s_refs = (s0_ref, s1_ref, s2_ref, s3_ref)
    p_refs = (p0_ref, p1_ref, p2_ref, p3_ref)

    def w_cp(name):
        src, dst, k = {
            "waq": (wqa_hbm.at[:, 0:256], wq_v.at[0, :, 0:256], 0),
            "waq2": (wqa_hbm.at[:, 256:512], wq_v.at[0, :, 256:512], 1),
            "wak": (wqa_hbm.at[:, 512:896], wq_v.at[0, :, 512:896], 2),
            "wav": (wqa_hbm.at[:, 896:1344], wq_v.at[0, :, 896:1344], 3),
            "wb": (wqb_hbm, wq_v.at[1], 4),
            "woa": (woa_hbm, wo_v.at[0], 5),
            "wob": (wob_hbm, wo_v.at[1], 5),
        }[name]
        return pltpu.make_async_copy(src, dst, sems.at[k])

    xgroups = {
        "xa0": (0, 0, 2, 6), "xa02": (0, 2, 3, 1), "xb0": (1, 0, 2, 4),
        "xb1": (1, 2, 2 + U, 5), "xa1": (0, 3, 3 + U, 5),
        "xb2": (1, 2 + U, NT, 0), "xa2": (0, 3 + U, NT, 0),
    }

    def start(*names):
        for name in names:
            if name in xgroups:
                br, t0, t1, k = xgroups[name]
                for t in range(t0, t1):
                    pltpu.make_async_copy((xa_hbm, xb_hbm)[br].at[0, :, t * T:(t + 1) * T],
                                          x_v.at[br, t], sems.at[k]).start()
            else:
                w_cp(name).start()

    def wait(*names):
        for name in names:
            if name in xgroups:
                br, t0, t1, k = xgroups[name]
                pltpu.make_async_copy(x_v.at[br, t0:t1], x_v.at[br, t0:t1], sems.at[k]).wait()
            else:
                w_cp(name).wait()

    def out_cp(row0, nrows, c0=0, c1=2 * D):
        return pltpu.make_async_copy(ob_v.at[row0:row0 + nrows, c0:c1],
                                     o_hbm.at[0, row0:row0 + nrows, c0:c1], sems.at[2])

    def init():
        start("waq", "xa0", "waq2", "xa02", "wak", "wav", "wb", "xb0", "woa", "wob")
        row = lax.broadcasted_iota(jnp.int32, (64, T), 0)
        col = lax.broadcasted_iota(jnp.int32, (64, T), 1)
        real = (jnp.logical_or((row & 31) < 14, (row & 31) >= 18),
                jnp.logical_or((col & 63) < 28, (col & 63) >= 36))
        code = ((row >> 4) + (col >> 5)) & 3
        for c in range(4):
            for f in range(2):
                qm_ref[f, c] = jnp.where(jnp.logical_and(real[f], code == c),
                                         jnp.uint32(0xFFFFFFFF), jnp.uint32(0))
            p_refs[c][ZP, 0] = jnp.zeros((16, 2 * T), bf16)
        vT_ref[1, 0, 192:256, :] = jnp.zeros((64, T), u32)
        ob_v[S:S + 16, 0:T] = jnp.zeros((16, T), bf16)
        oa_ref[0] = jnp.zeros((64, T), f32)

    zs = (step >> 10, step >> 11)
    zw, zr = zs

    mk = {}

    def make_masks():
        lane = lax.broadcasted_iota(jnp.int32, (SB, T), 1)
        mk["tri"] = lax.broadcasted_iota(jnp.int32, (SB, T), 0) <= (lane & (SB - 1))
        for n in (4, 1):
            lane = lax.broadcasted_iota(jnp.int32, (n, 8, 2 * T), 2)
            mk["odd", n] = (lane & SB) != 0
            mk["hi", n] = (lane & (2 * SB)) != 0
        key = lax.broadcasted_iota(jnp.int32, (1, 8, 2 * T), 1) + ((lane >> 7) << 4)
        for e in range(2):
            mk["tri", e] = key + 8 * e <= (lane & (SB - 1))

    zero2 = jnp.zeros((1, 8, 2 * T), bf16)
    zero8 = jnp.zeros((8, T), u32)

    def slack(z, r0):
        for r in (r0, r0 + 8):
            tmp_ref[r:r + 8, :] = z
            z = tmp_ref[r:r + 8, :]
        return z

    def ties(items, nrounds, t0, t1, extra=()):
        out = []
        done = 0
        for v in range(nrounds):
            zv = None
            if t0 <= v < t1:
                upto = (len(items) * (v - t0 + 1)) // (t1 - t0)
                if upto > done:
                    gs = sorted({it() for it in items[done:upto]})
                    done = upto
                    zv = slack(functools.reduce(jnp.bitwise_or, [
                        pltpu.bitcast(p_refs[g][ZP, 0, :, 0:T], u32) for g in gs]), 0)
            out.append(zv)
        for v, z in extra:
            out[v] = z if out[v] is None else out[v] | z
        if all(z is None for z in out):
            return None
        return jnp.concatenate([zero8 if z is None else z for z in out], axis=0)

    def pad_heads(a, fill=None):
        parts = []
        for p in range(a.shape[0] // 56):
            b = a[56 * p:56 * p + 56]
            mid = b[24:32]
            if fill is None:
                parts += [b[0:32], b[24:56]]
            else:
                m = lax.broadcasted_iota(jnp.int32, mid.shape, 0) < 4
                parts += [b[0:24], jnp.where(m, mid, fill), jnp.where(m, fill, mid), b[32:56]]
        return jnp.concatenate(parts, axis=0)

    def roll_heads(a, back):
        parts = []
        for h in range(a.shape[0] // 16):
            j = h % 4
            b = a[16 * h:16 * h + 16]
            parts.append(b if j == 0 else pltpu.roll(b, SB * j if back else T - SB * j, 1))
        return jnp.concatenate(parts, axis=0)

    def moff(i, n):
        return i * n if isinstance(i, int) else pl.multiple_of(i * n, n)

    def prep_w(br, c0, c1):
        w = jnp.concatenate([wq_v[br, :, c0:c1], jnp.zeros((64, c1 - c0), bf16)], axis=0)
        wt_ref[br, c0 // 2:c1 // 2, :] = pltpu.bitcast(w.T, u32)

    def prep_wo(br):
        w = pad_heads(wo_v[br].astype(f32), 0.0).astype(bf16)
        wt_ref[br, 3 * D // 2:2 * D, :] = pltpu.bitcast(w.T, u32)

    def project(br, part, rhs, items, t0, extra=()):
        zv = ties(items, NR, t0, NR, extra)
        w = wt_ref[br, part * (D // 2):(part + 1) * (D // 2), :]
        if zv is not None:
            w = w | jnp.concatenate([zv] * 4, axis=1)
        return jnp.dot(_ubf(w), rhs, preferred_element_type=f32)

    def xtile(br, i):
        return jnp.concatenate([x_v[br, i], jnp.zeros((64, T), bf16)], axis=0)

    def put_q(br, slot, y, hf=0):
        y = pad_heads(y * QSCALE)
        n = y.shape[0]
        if slot is None:
            q_ref[br, :, n * hf:n * (hf + 1)] = pltpu.bitcast(y.astype(bf16).T, u32)
        else:
            qT_ref[slot, n // 2 * hf:n // 2 * (hf + 1), :] = roll_heads(_pk(y), False)

    def proj_q(br, i, items=(), t0=TIE0, slot=None):
        put_q(br, slot, project(br, 0, xtile(br, i), items, t0))

    def proj_q_half(i, hf, slot, mid=()):
        y = jnp.dot(_ubf(wt_ref[0, 112 * hf:112 * hf + 112, :]), xtile(0, i),
                    preferred_element_type=f32)
        wait(*mid)
        put_q(0, slot, y, hf)

    def proj_k(br, i, items=(), t0=TIE0):
        kT = pad_heads(project(br, 1, xtile(br, i), items, t0))
        for gp in range(2):
            kt = pltpu.bitcast(kT[2 * T * gp:2 * T * (gp + 1)].astype(bf16).T, u32)
            for gg in range(2):
                k_ref[br, 2 * gp + gg, pl.ds(moff(i, 64), 64), :] = kt[:, T * gg:T * (gg + 1)]

    def proj_v(br, i, items=(), t0=TIE0, mid=(), extra=()):
        vT = project(br, 2, xtile(br, i), items, t0, extra)
        wait(*mid)
        vT_ref[br, i + 1] = _pk(pad_heads(vT, 1.0))

    def proj_o(br, i, items=(), t0=TIE0, slot=None, aslot=0, extra=()):
        o = project(br, 3, _ubf(oT_ref[br if slot is None else slot]), items, t0, extra)
        row0 = moff(i, T)
        if br == 0:
            ob_v[pl.ds(row0, T), 0:384] = o[0:384].astype(bf16).T
            oa_ref[aslot] = o[384:448]
        else:
            ob_v[pl.ds(row0, T), 384:896] = jnp.concatenate(
                [oa_ref[aslot], o], axis=0).astype(bf16).T

    def ntiles(i):
        return min(3, i + 1) if isinstance(i, int) else 3

    def qk(br, i, g, items=(), t0=1, t1=18, zero_fill=False, slot=None, col=0,
           late=False, extra=()):
        s_ref = s_refs[g]
        nt = ntiles(i)
        late = late or nt < 3
        zv = ties(items, 18, t0, t1, extra)
        if slot is None:
            q = q_ref[br, :, T * g:T * (g + 1)]
        else:
            q = qT_ref[slot, 64 * g:64 * g + 64, :]
        ms = [None] * 4
        for c in (range(4) if g % 2 == 0 else range(3, -1, -1)):
            n = min(WIN // 2, 64 * (nt - 1) + 16 * c)
            ks = k_ref[br, g, pl.ds(moff(i, 64) + (16 * c - n), n + 16), :]
            if n > 0:
                ks = jnp.concatenate([ks[n:], ks[:n]], axis=0)
            if zv is not None:
                ks = ks | (zv if nt == 3 else zv[:n + 16])
            if slot is None:
                w = jnp.concatenate([q[16 * c:16 * c + 16]] * 4, axis=0) & qm_ref[1, c]
                s = lax.dot_general(_ubf(ks), _ubf(w), (((1,), (1,)), ((), ())),
                                    preferred_element_type=f32)
            else:
                s = jnp.dot(_ubf(ks), _ubf(q & qm_ref[0, c]), preferred_element_type=f32)
            r0 = 2 * SB if nt == 3 else SB
            dg = jnp.where(mk["tri"], s[0:SB], s[SB:r0] if nt == 3 else NEG)
            r1 = s.shape[0] - SB * c

            def put_s(b0, rows):
                nb = rows.shape[0] // SB
                blk = rows.reshape(nb, 4, 8, T)
                blk = jnp.concatenate([blk[:, 0:2], blk[:, 2:4]], axis=3)
                s_ref[pl.ds(zw + 2 * b0, 2 * nb), c] = blk.reshape(2 * nb, 8, 2 * T)
            put_s(0, jnp.concatenate([s[r1:], dg], axis=0) if c > 0 else dg)
            if r1 > r0:
                put_s(8 - (r1 - r0) // SB, s[r0:r1])
            sm = jnp.concatenate([dg, s[r0:]], axis=0) if s.shape[0] > r0 else dg
            ms[c] = jnp.broadcast_to(jnp.max(sm, axis=0, keepdims=True), (8, T))
            if late:
                s_ref[zw + MS, c, :, 0:T] = ms[c]

        mall = None if late else jnp.concatenate(ms, axis=0).reshape(4, 8, T)
        return sm_items(g, nt, mall, zero_fill, col)

    def sm_items(g, nt=3, mall=None, zero_fill=False, col=0):
        s_ref, p_ref = s_refs[g], p_refs[g]

        def sel(m, a, b):
            if a is None and b is None:
                return None
            return lax.select(m, zero2 if a is None else a, zero2 if b is None else b)

        def put_p(b, e, x):
            if isinstance(x, list):
                x = [sel(mk["odd", 1], x[(j + 1) % 4], x[j]) for j in range(4)]
                x = jnp.concatenate(
                    [sel(mk["hi", 1], x[(j + 2) % 4], x[j]) for j in range(4)], axis=0)
            else:
                x = lax.select(mk["odd", 4], jnp.concatenate([x[1:], x[:1]], axis=0), x)
                x = lax.select(mk["hi", 4], jnp.concatenate([x[2:], x[:2]], axis=0), x)
            p_ref[zs[col] + b, :, 8 * e:8 * e + 8, :] = x

        def item(rho):
            b, e = rho // 2, rho % 2
            c0 = b if nt < 3 and rho < 8 else 0
            m = s_ref[zr + MS, c0:4, :, 0:T] if mall is None else mall
            x = jnp.exp2(s_ref[zr + rho, c0:4] - jnp.concatenate([m, m], axis=2)).astype(bf16)
            if rho < 8:
                x = [None] * c0 + [x[c:c + 1] for c in range(4 - c0)]
            if rho >= 8 or nt == 1:
                put_p(b, e, x)
            elif nt == 3:
                tri = mk["tri", e]
                put_p(b + 8, e, [None] * b + [sel(tri, x[b], None)] + x[b + 1:])
                put_p(b, e, x[:b] + [sel(tri, None, x[b])] + [None] * (3 - b))
            else:
                put_p(b + 8, e, x)
                if zero_fill:
                    p_ref[zs[col] + b, :, 8 * e:8 * e + 8, :] = jnp.zeros((4, 8, 2 * T), bf16)
            return g
        order = list(range(8, 16 if nt > 1 else 8)) + list(range(8))
        return [functools.partial(item, rho) for rho in order]

    def pv(br, i, g, slot=None, col=0):
        nt = ntiles(i)
        acc = [None] * 4
        for t in range(3 - nt, 3):
            vv = _ubf(vT_ref[br, i - 1 + t, 64 * g:64 * g + 64, :])
            bs = pl.ds(zs[1 - col] + (0 if nt == 1 else 4 * t), 4)
            for j in range(4):
                pj = jnp.concatenate([p_refs[g][bs, j, :, 0:T], p_refs[g][bs, j, :, T:2 * T]],
                                     axis=1).reshape(T, T)
                o = jnp.dot(vv[32 * j:32 * j + 32], pj, preferred_element_type=f32)
                acc[j] = o if acc[j] is None else acc[j] + o
        og = jnp.concatenate(
            [acc[j] * pl.reciprocal(acc[j][28:29] if j % 2 == 0 else acc[j][0:1], approx=False)
             for j in range(4)], axis=0)
        oT_ref[br if slot is None else slot, 64 * g:64 * g + 64, :] = roll_heads(_pk(og), True)

    def units(i0, n, cut):
        items = sm_items(0)
        for u in range(1, n + 1):
            i, br, g = i0 + u // 8, u // 4 % 2, u % 4
            pb, pg = (br, g - 1) if g > 0 else (1 - br, 3)
            pi = i if u % 8 > 0 else i - 1
            if pg == 2:
                proj_o(1 - pb, pi - 1 + pb, items[:NF])
            elif pg == 3:
                zo = pltpu.bitcast(ob_v[pl.ds(moff(zr, 16) + S, 16), 0:T], u32)
                proj_v(1 - pb, pi + pb, items[:NF], extra=[(OTIE, slack(zo, 16))])
            else:
                (proj_k, proj_q)[pg](1 - pb, pi + pb, items[:NF], 2 if u == 1 else TIE0)
            last = cut and u == n
            do_pv = functools.partial(pv, br, i, g - 2) if g > 1 else functools.partial(
                pv, 1 - br, i - 1 + br, g + 2)
            if last:
                do_pv()
            items = qk(br, i, g, items[NF:], late=last)
            if not last:
                do_pv()
        return items

    def first():
        make_masks()
        wait("waq")
        prep_w(0, 0, 256)
        start("xb1", "xa1", "xb2", "xa2")
        wait("xa0")
        proj_q_half(0, 0, 0)
        proj_q_half(1, 0, 1, mid=("waq2", "xa02"))
        prep_w(0, 256, 512)
        proj_q_half(2, 0, None)
        proj_q_half(0, 1, 0)
        proj_q_half(1, 1, 1, mid=("wak",))
        prep_w(0, 512, 896)
        proj_q_half(2, 1, None)
        proj_k(0, 0)
        proj_k(0, 1)
        it = sum([qk(0, 0, g, slot=0, col=1) for g in range(4)], [])
        proj_k(0, 2, it, 4)
        it0 = qk(0, 1, 0, slot=1)
        it1 = qk(0, 1, 1, slot=1)
        wait("wav")
        prep_w(0, 896, 1344)
        it2 = qk(0, 1, 2, it0[:8], 1, 10, slot=1)
        it3 = qk(0, 1, 3, it0[8:], 1, 10, slot=1)
        proj_v(0, 0, it1, 1)
        proj_v(0, 1, it2, 1, mid=("wb", "xb0"))
        prep_w(1, 384, 896)
        prep_w(1, 0, 384)
        prep_w(1, 896, 1344)
        for g in range(4):
            pv(0, 0, g, slot=2, col=1)
        for g in range(3):
            pv(0, 1, g, slot=4)
        proj_k(1, 0, it3, 11)
        proj_q(1, 0, slot=0)
        proj_k(1, 1)
        it = sum([qk(1, 0, g, slot=0, col=1) for g in range(4)], [])
        pv(0, 1, 3, slot=4)
        proj_q(1, 1, it, 2, slot=1)
        proj_v(1, 0)
        it = qk(1, 1, 0, slot=1)
        it = it + qk(1, 1, 1, slot=1)
        it = it[9:] + qk(1, 1, 2, it[:9], 1, 10, slot=1)
        it3 = qk(1, 1, 3, it[:12], 1, 10, zero_fill=True, slot=1)
        for g in range(4):
            pv(1, 0, g, slot=3, col=1)
        proj_v(1, 1, it[12:], 10)
        proj_v(0, 2, it3, 1)
        for g in range(3):
            pv(1, 1, g)
        qk(0, 2, 0, late=True)
        wait("woa", "wob", "xb1", "xa1")

    def steady(n, carry):
        make_masks()
        prep_wo(1)
        prep_wo(0)
        units(2 + n * U, 8 * U, True)

        @pl.when(n == 0)
        def _():
            out_cp(2 * T, (U - 1) * T).start()
            wait("xb2", "xa2")

        for k in range(1, NLOOP):
            pl.when(n == k)(out_cp((1 + k * U) * T, U * T).start)
        return carry

    def last():
        make_masks()
        i = NT - 1
        r0 = i * T
        it = units(i - 1, 11, False)
        proj_v(1, i, it[:NF])
        out_cp((NT - 3) * T, 2 * T).start()

        def dma_tie():
            ob_v[pl.ds(moff(zw, 16) + S, 16), 0:T] = jnp.zeros((16, T), bf16)
            return pltpu.bitcast(ob_v[pl.ds(moff(zr, 16) + S, 16), 0:T], u32)

        q_ref[0] = pltpu.bitcast(_ubf(oT_ref[4]).T, u32)
        out_cp(T, T, 512, 896).start()

        it = qk(1, i, 0, it[NF:], late=True, extra=[(17, dma_tie())])
        pv(0, i, 2)
        it = it[7:] + qk(1, i, 1, it[:7], 9, late=True)
        pv(0, i, 3)
        proj_o(0, 0, it[:12], 0, slot=2, aslot=1)
        it = it[19:] + qk(1, i, 2, it[12:19], 0, late=True)
        it = it[10:] + qk(1, i, 3, it[:10], 0, late=True)
        proj_o(1, 0, it, 0, slot=3, aslot=1)
        out_cp(0, T).start()
        for g in range(4):
            pv(1, i, g)
        proj_o(0, i, extra=[(8, dma_tie())])
        out_cp(r0, T, 0, 384).start()
        o = project(1, 3, _ubf(oT_ref[1]), (), 0, [(NR - 1, dma_tie())])
        ot = jnp.concatenate([oa_ref[0], o], axis=0).astype(bf16).T
        for a in range(0, T, 32):
            ob_v[r0 + a:r0 + a + 32, 384:896] = ot[a:a + 32]
            out_cp(r0 + a, 32, 384, 896).start()
        zd = dma_tie()
        wo = pad_heads(wo_v[0].astype(f32), 0.0).astype(bf16)
        for c0 in range(0, D, T):
            c1 = min(c0 + T, D)
            lhs = q_ref[0]
            if c1 == D:
                lhs = jnp.concatenate(
                    [lhs[0:56], lhs[56:64] | jnp.concatenate([zd] * 4, axis=1)], axis=0)
            y = jnp.dot(_ubf(lhs), wo[:, c0:c1], preferred_element_type=f32).astype(bf16)
            for a, b in ((0, T),) if c1 < D else ((0, 64), (64, 96), (96, T)):
                ob_v[T + a:T + b, c0:c1] = y[a:b]
                out_cp(T + a, b - a, c0, c0 + T).start()
        out_cp(0, S).wait()

    pl.when(step == 0)(init)

    @pl.when(step == 1)
    def _():
        first()
        lax.fori_loop(0, NLOOP, steady, 0)
        last()


@jax.jit
def pallas_concat_heads__sliding_block__sliding_block__prompt_kernel(
        A_x, A_wqkv, A_wo, B_x, B_wqkv, B_wo):
    anyspec = pl.BlockSpec(memory_space=pl.ANY)
    return pl.pallas_call(
        _kernel,
        grid=(2,),
        in_specs=[anyspec] * 6,
        out_specs=anyspec,
        out_shape=jax.ShapeDtypeStruct((1, S, 2 * D), bf16),
        scratch_shapes=[
            pltpu.VMEM((2, NT, D, T), bf16),
            pltpu.VMEM((2, D, 3 * D), bf16),
            pltpu.VMEM((2, D, D), bf16),
            pltpu.VMEM((S + 64, 2 * D), bf16),
            pltpu.VMEM((2, 2 * D, 4 * T), u32),
            pltpu.VMEM((2, 4, S // 2, T), u32),
            pltpu.VMEM((2, NT + 1, 256, T), u32),
            pltpu.VMEM((2, 256, T), u32),
            pltpu.VMEM((2, 64, 4 * T), u32),
            pltpu.VMEM((5, 256, T), u32),
            pltpu.VMEM((2, 64, T), f32),
        ] + [pltpu.VMEM((MS + 1, 4, 8, 2 * T), f32)] * 4
        + [pltpu.VMEM((ZP + 1, 4, 16, 2 * T), bf16)] * 4
        + [
            pltpu.VMEM((2, 4, 64, T), u32),
            pltpu.VMEM((32, T), u32),
            pltpu.SemaphoreType.DMA((7,)),
        ],
        compiler_params=pltpu.CompilerParams(
            dimension_semantics=("arbitrary",),
            vmem_limit_bytes=64 * 1024 * 1024),
        name="swa",
    )(jnp.swapaxes(A_x, 1, 2), A_wqkv, A_wo, jnp.swapaxes(B_x, 1, 2), B_wqkv, B_wo)
```

```python
import functools

import jax
import jax.numpy as jnp
from jax import lax
import jax.experimental.pallas as pl
import jax.experimental.pallas.tpu as pltpu

S, D, H, DH, WIN = 2048, 448, 16, 28, 256
T = 128
NT = S // T
U = 4
NLOOP = (NT - 4) // U
QSCALE = (DH ** -0.5) * 1.4426950408889634
NEG = -1e30
SB = 32
NR = D // 16
ZP = 12
MS = 16
TIE0 = 12
NF = 9
OTIE = 14

f32, bf16, u32 = jnp.float32, jnp.bfloat16, jnp.uint32


def _pk(x):
    return pltpu.bitcast(x.astype(bf16), u32)


def _ubf(x):
    return pltpu.bitcast(x, bf16)


def _kernel(xa_hbm, wqa_hbm, woa_hbm, xb_hbm, wqb_hbm, wob_hbm, o_hbm,
            x_v, wq_v, wo_v, ob_v, wt_ref, k_ref, vT_ref, qT_ref, q_ref, oT_ref, oa_ref,
            s0_ref, s1_ref, s2_ref, s3_ref, p0_ref, p1_ref, p2_ref, p3_ref,
            qm_ref, tmp_ref, sems):
    step = pl.program_id(0)
    s_refs = (s0_ref, s1_ref, s2_ref, s3_ref)
    p_refs = (p0_ref, p1_ref, p2_ref, p3_ref)

    def w_cp(name):
        src, dst, k = {
            "waq": (wqa_hbm.at[:, 0:256], wq_v.at[0, :, 0:256], 0),
            "waq2": (wqa_hbm.at[:, 256:512], wq_v.at[0, :, 256:512], 1),
            "wak": (wqa_hbm.at[:, 512:896], wq_v.at[0, :, 512:896], 2),
            "wav": (wqa_hbm.at[:, 896:1344], wq_v.at[0, :, 896:1344], 3),
            "wb": (wqb_hbm, wq_v.at[1], 4),
            "woa": (woa_hbm, wo_v.at[0], 5),
            "wob": (wob_hbm, wo_v.at[1], 5),
        }[name]
        return pltpu.make_async_copy(src, dst, sems.at[k])

    xgroups = {
        "xa0": (0, 0, 2, 6), "xa02": (0, 2, 3, 1), "xb0": (1, 0, 2, 4),
        "xb1": (1, 2, 2 + U, 5), "xa1": (0, 3, 3 + U, 5),
        "xb2": (1, 2 + U, NT, 0), "xa2": (0, 3 + U, NT, 0),
    }

    def copies(names):
        for name in names:
            if name in xgroups:
                br, t0, t1, k = xgroups[name]
                for t in range(t0, t1):
                    yield pltpu.make_async_copy(
                        (xa_hbm, xb_hbm)[br].at[0, :, t * T:(t + 1) * T], x_v.at[br, t],
                        sems.at[k])
            else:
                yield w_cp(name)

    def start(*names):
        for cp in copies(names):
            cp.start()

    def wait(*names):
        for cp in copies(names):
            cp.wait()

    def out_cp(row0, nrows, c0=0, c1=2 * D):
        return pltpu.make_async_copy(ob_v.at[row0:row0 + nrows, c0:c1],
                                     o_hbm.at[0, row0:row0 + nrows, c0:c1], sems.at[2])

    def init():
        start("waq", "xa0", "waq2", "xa02", "wak", "wav", "wb", "xb0", "woa", "wob")
        row = lax.broadcasted_iota(jnp.int32, (64, T), 0)
        col = lax.broadcasted_iota(jnp.int32, (64, T), 1)
        real = (jnp.logical_or((row & 31) < 14, (row & 31) >= 18),
                jnp.logical_or((col & 63) < 28, (col & 63) >= 36))
        code = ((row >> 4) + (col >> 5)) & 3
        for c in range(4):
            for f in range(2):
                qm_ref[f, c] = jnp.where(jnp.logical_and(real[f], code == c),
                                         jnp.uint32(0xFFFFFFFF), jnp.uint32(0))
            p_refs[c][ZP, 0] = jnp.zeros((16, 2 * T), bf16)
        vT_ref[1, 0, 192:256, :] = jnp.zeros((64, T), u32)
        ob_v[S:S + 16, 0:T] = jnp.zeros((16, T), bf16)
        oa_ref[0] = jnp.zeros((64, T), f32)

    zs = (step >> 10, step >> 11)
    zw, zr = zs

    mk = {}

    def make_masks():
        lane = lax.broadcasted_iota(jnp.int32, (SB, T), 1)
        mk["tri"] = lax.broadcasted_iota(jnp.int32, (SB, T), 0) <= (lane & (SB - 1))
        for n in (4, 1):
            lane = lax.broadcasted_iota(jnp.int32, (n, 8, 2 * T), 2)
            mk["odd", n] = (lane & SB) != 0
            mk["hi", n] = (lane & (2 * SB)) != 0
        key = lax.broadcasted_iota(jnp.int32, (1, 8, 2 * T), 1) + ((lane >> 7) << 4)
        for e in range(2):
            mk["tri", e] = key + 8 * e <= (lane & (SB - 1))

    zero2 = jnp.zeros((1, 8, 2 * T), bf16)
    zero8 = jnp.zeros((8, T), u32)

    def slack(z, r0):
        for r in (r0, r0 + 8):
            tmp_ref[r:r + 8, :] = z
            z = tmp_ref[r:r + 8, :]
        return z

    def ties(items, nrounds, t0, t1, extra=()):
        out = []
        done = 0
        for v in range(nrounds):
            zv = None
            if t0 <= v < t1:
                upto = (len(items) * (v - t0 + 1)) // (t1 - t0)
                if upto > done:
                    gs = sorted({it() for it in items[done:upto]})
                    done = upto
                    zv = slack(functools.reduce(jnp.bitwise_or, [
                        pltpu.bitcast(p_refs[g][ZP, 0, :, 0:T], u32) for g in gs]), 0)
            out.append(zv)
        for v, z in extra:
            out[v] = z if out[v] is None else out[v] | z
        if all(z is None for z in out):
            return None
        return jnp.concatenate([zero8 if z is None else z for z in out], axis=0)

    def pad_heads(a, fill=None):
        parts = []
        for p in range(a.shape[0] // 56):
            b = a[56 * p:56 * p + 56]
            mid = b[24:32]
            if fill is None:
                parts += [b[0:32], b[24:56]]
            else:
                m = lax.broadcasted_iota(jnp.int32, mid.shape, 0) < 4
                parts += [b[0:24], jnp.where(m, mid, fill), jnp.where(m, fill, mid), b[32:56]]
        return jnp.concatenate(parts, axis=0)

    def roll_heads(a, back):
        parts = []
        for h in range(a.shape[0] // 16):
            j = h % 4
            b = a[16 * h:16 * h + 16]
            parts.append(b if j == 0 else pltpu.roll(b, SB * j if back else T - SB * j, 1))
        return jnp.concatenate(parts, axis=0)

    def moff(i, n):
        return i * n if isinstance(i, int) else pl.multiple_of(i * n, n)

    def prep_w(br, c0, c1):
        w = jnp.concatenate([wq_v[br, :, c0:c1], jnp.zeros((64, c1 - c0), bf16)], axis=0)
        wt_ref[br, c0 // 2:c1 // 2, :] = pltpu.bitcast(w.T, u32)

    def prep_wo(br):
        w = pad_heads(wo_v[br].astype(f32), 0.0).astype(bf16)
        wt_ref[br, 3 * D // 2:2 * D, :] = pltpu.bitcast(w.T, u32)

    def project(br, part, rhs, items, t0, extra=()):
        zv = ties(items, NR, t0, NR, extra)
        w = wt_ref[br, part * (D // 2):(part + 1) * (D // 2), :]
        if zv is not None:
            w = w | jnp.concatenate([zv] * 4, axis=1)
        return jnp.dot(_ubf(w), rhs, preferred_element_type=f32)

    def xtile(br, i):
        return jnp.concatenate([x_v[br, i], jnp.zeros((64, T), bf16)], axis=0)

    def put_q(br, slot, y, hf=0):
        y = pad_heads(y * QSCALE)
        n = y.shape[0]
        if slot is None:
            q_ref[br, :, n * hf:n * (hf + 1)] = pltpu.bitcast(y.astype(bf16).T, u32)
        else:
            qT_ref[slot, n // 2 * hf:n // 2 * (hf + 1), :] = roll_heads(_pk(y), False)

    def proj_q(br, i, items=(), t0=TIE0, slot=None):
        put_q(br, slot, project(br, 0, xtile(br, i), items, t0))

    def proj_q_half(i, hf, slot, mid=()):
        y = jnp.dot(_ubf(wt_ref[0, 112 * hf:112 * hf + 112, :]), xtile(0, i),
                    preferred_element_type=f32)
        wait(*mid)
        put_q(0, slot, y, hf)

    def proj_k(br, i, items=(), t0=TIE0):
        kT = pad_heads(project(br, 1, xtile(br, i), items, t0))
        for gp in range(2):
            kt = pltpu.bitcast(kT[2 * T * gp:2 * T * (gp + 1)].astype(bf16).T, u32)
            for gg in range(2):
                k_ref[br, 2 * gp + gg, pl.ds(moff(i, 64), 64), :] = kt[:, T * gg:T * (gg + 1)]

    def proj_v(br, i, items=(), t0=TIE0, mid=(), extra=()):
        vT = project(br, 2, xtile(br, i), items, t0, extra)
        wait(*mid)
        vT_ref[br, i + 1] = _pk(pad_heads(vT, 1.0))

    def proj_o(br, i, items=(), t0=TIE0, slot=None, aslot=0, extra=()):
        o = project(br, 3, _ubf(oT_ref[br if slot is None else slot]), items, t0, extra)
        row0 = moff(i, T)
        if br == 0:
            ob_v[pl.ds(row0, T), 0:384] = o[0:384].astype(bf16).T
            oa_ref[aslot] = o[384:448]
        else:
            ob_v[pl.ds(row0, T), 384:896] = jnp.concatenate(
                [oa_ref[aslot], o], axis=0).astype(bf16).T

    def ntiles(i):
        return min(3, i + 1) if isinstance(i, int) else 3

    def qk(br, i, g, items=(), t0=1, t1=18, zero_fill=False, slot=None, col=0,
           late=False, extra=()):
        s_ref = s_refs[g]
        nt = ntiles(i)
        late = late or nt < 3
        zv = ties(items, 18, t0, t1, extra)
        if slot is None:
            q = q_ref[br, :, T * g:T * (g + 1)]
        else:
            q = qT_ref[slot, 64 * g:64 * g + 64, :]
        ms = [None] * 4
        for c in (range(4) if g % 2 == 0 else range(3, -1, -1)):
            n = min(WIN // 2, 64 * (nt - 1) + 16 * c)
            ks = k_ref[br, g, pl.ds(moff(i, 64) + (16 * c - n), n + 16), :]
            if n > 0:
                ks = jnp.concatenate([ks[n:], ks[:n]], axis=0)
            if zv is not None:
                ks = ks | (zv if nt == 3 else zv[:n + 16])
            if slot is None:
                w = jnp.concatenate([q[16 * c:16 * c + 16]] * 4, axis=0) & qm_ref[1, c]
                s = lax.dot_general(_ubf(ks), _ubf(w), (((1,), (1,)), ((), ())),
                                    preferred_element_type=f32)
            else:
                s = jnp.dot(_ubf(ks), _ubf(q & qm_ref[0, c]), preferred_element_type=f32)
            r0 = 2 * SB if nt == 3 else SB
            dg = jnp.where(mk["tri"], s[0:SB], s[SB:r0] if nt == 3 else NEG)
            r1 = s.shape[0] - SB * c

            def put_s(b0, rows):
                nb = rows.shape[0] // SB
                blk = rows.reshape(nb, 4, 8, T)
                blk = jnp.concatenate([blk[:, 0:2], blk[:, 2:4]], axis=3)
                s_ref[pl.ds(zw + 2 * b0, 2 * nb), c] = blk.reshape(2 * nb, 8, 2 * T)
            put_s(0, jnp.concatenate([s[r1:], dg], axis=0) if c > 0 else dg)
            if r1 > r0:
                put_s(8 - (r1 - r0) // SB, s[r0:r1])
            sm = jnp.concatenate([dg, s[r0:]], axis=0) if s.shape[0] > r0 else dg
            ms[c] = jnp.broadcast_to(jnp.max(sm, axis=0, keepdims=True), (8, T))
            if late:
                s_ref[zw + MS, c, :, 0:T] = ms[c]

        mall = None if late else jnp.concatenate(ms, axis=0).reshape(4, 8, T)
        return sm_items(g, nt, mall, zero_fill, col)

    def sm_items(g, nt=3, mall=None, zero_fill=False, col=0):
        s_ref, p_ref = s_refs[g], p_refs[g]

        def sel(m, a, b):
            if a is None and b is None:
                return None
            return lax.select(m, zero2 if a is None else a, zero2 if b is None else b)

        def put_p(b, e, x):
            if isinstance(x, list):
                x = [sel(mk["odd", 1], x[(j + 1) % 4], x[j]) for j in range(4)]
                x = jnp.concatenate(
                    [sel(mk["hi", 1], x[(j + 2) % 4], x[j]) for j in range(4)], axis=0)
            else:
                x = lax.select(mk["odd", 4], jnp.concatenate([x[1:], x[:1]], axis=0), x)
                x = lax.select(mk["hi", 4], jnp.concatenate([x[2:], x[:2]], axis=0), x)
            p_ref[zs[col] + b, :, 8 * e:8 * e + 8, :] = x

        def item(rho):
            b, e = rho // 2, rho % 2
            c0 = b if nt < 3 and rho < 8 else 0
            m = s_ref[zr + MS, c0:4, :, 0:T] if mall is None else mall
            x = jnp.exp2(s_ref[zr + rho, c0:4] - jnp.concatenate([m, m], axis=2)).astype(bf16)
            if rho < 8:
                x = [None] * c0 + [x[c:c + 1] for c in range(4 - c0)]
            if rho >= 8 or nt == 1:
                put_p(b, e, x)
            elif nt == 3:
                tri = mk["tri", e]
                put_p(b + 8, e, [None] * b + [sel(tri, x[b], None)] + x[b + 1:])
                put_p(b, e, x[:b] + [sel(tri, None, x[b])] + [None] * (3 - b))
            else:
                put_p(b + 8, e, x)
                if zero_fill:
                    p_ref[zs[col] + b, :, 8 * e:8 * e + 8, :] = jnp.zeros((4, 8, 2 * T), bf16)
            return g
        order = list(range(8, 16 if nt > 1 else 8)) + list(range(8))
        return [functools.partial(item, rho) for rho in order]

    def pv(br, i, g, slot=None, col=0):
        nt = ntiles(i)
        acc = [None] * 4
        for t in range(3 - nt, 3):
            vv = _ubf(vT_ref[br, i - 1 + t, 64 * g:64 * g + 64, :])
            bs = pl.ds(zs[1 - col] + (0 if nt == 1 else 4 * t), 4)
            for j in range(4):
                pj = jnp.concatenate([p_refs[g][bs, j, :, 0:T], p_refs[g][bs, j, :, T:2 * T]],
                                     axis=1).reshape(T, T)
                o = jnp.dot(vv[32 * j:32 * j + 32], pj, preferred_element_type=f32)
                acc[j] = o if acc[j] is None else acc[j] + o
        og = jnp.concatenate(
            [acc[j] * pl.reciprocal(acc[j][28:29] if j % 2 == 0 else acc[j][0:1], approx=False)
             for j in range(4)], axis=0)
        oT_ref[br if slot is None else slot, 64 * g:64 * g + 64, :] = roll_heads(_pk(og), True)

    def units(i0, n, cut):
        items = sm_items(0)
        for u in range(1, n + 1):
            i, br, g = i0 + u // 8, u // 4 % 2, u % 4
            pb, pg = (br, g - 1) if g > 0 else (1 - br, 3)
            pi = i if u % 8 > 0 else i - 1
            if pg == 2:
                proj_o(1 - pb, pi - 1 + pb, items[:NF])
            elif pg == 3:
                zo = pltpu.bitcast(ob_v[pl.ds(moff(zr, 16) + S, 16), 0:T], u32)
                proj_v(1 - pb, pi + pb, items[:NF], extra=[(OTIE, slack(zo, 16))])
            else:
                (proj_k, proj_q)[pg](1 - pb, pi + pb, items[:NF], 2 if u == 1 else TIE0)
            last = cut and u == n
            do_pv = functools.partial(pv, br, i, g - 2) if g > 1 else functools.partial(
                pv, 1 - br, i - 1 + br, g + 2)
            if last:
                do_pv()
            items = qk(br, i, g, items[NF:], late=last)
            if not last:
                do_pv()
        return items

    def first():
        make_masks()
        wait("waq")
        prep_w(0, 0, 256)
        start("xb1", "xa1", "xb2", "xa2")
        wait("xa0")
        proj_q_half(0, 0, 0)
        proj_q_half(1, 0, 1, mid=("waq2", "xa02"))
        prep_w(0, 256, 512)
        proj_q_half(2, 0, None)
        proj_q_half(0, 1, 0)
        proj_q_half(1, 1, 1, mid=("wak",))
        prep_w(0, 512, 896)
        proj_q_half(2, 1, None)
        proj_k(0, 0)
        proj_k(0, 1)
        it = sum([qk(0, 0, g, slot=0, col=1) for g in range(4)], [])
        proj_k(0, 2, it, 4)
        it0 = qk(0, 1, 0, slot=1)
        it1 = qk(0, 1, 1, slot=1)
        wait("wav")
        prep_w(0, 896, 1344)
        it2 = qk(0, 1, 2, it0[:8], 1, 10, slot=1)
        it3 = qk(0, 1, 3, it0[8:], 1, 10, slot=1)
        proj_v(0, 0, it1, 1)
        proj_v(0, 1, it2, 1, mid=("wb", "xb0"))
        prep_w(1, 384, 896)
        prep_w(1, 0, 384)
        prep_w(1, 896, 1344)
        for g in range(4):
            pv(0, 0, g, slot=2, col=1)
        for g in range(3):
            pv(0, 1, g, slot=4)
        proj_k(1, 0, it3, 11)
        proj_q(1, 0, slot=0)
        proj_k(1, 1)
        it = sum([qk(1, 0, g, slot=0, col=1) for g in range(4)], [])
        pv(0, 1, 3, slot=4)
        proj_q(1, 1, it, 2, slot=1)
        proj_v(1, 0)
        it = qk(1, 1, 0, slot=1)
        it = it + qk(1, 1, 1, slot=1)
        it = it[9:] + qk(1, 1, 2, it[:9], 1, 10, slot=1)
        it3 = qk(1, 1, 3, it[:12], 1, 10, zero_fill=True, slot=1)
        for g in range(4):
            pv(1, 0, g, slot=3, col=1)
        proj_v(1, 1, it[12:], 10)
        proj_v(0, 2, it3, 1)
        for g in range(3):
            pv(1, 1, g)
        qk(0, 2, 0, late=True)
        wait("woa", "wob", "xb1", "xa1")

    def steady(n, carry):
        make_masks()
        prep_wo(1)
        prep_wo(0)
        units(2 + n * U, 8 * U, True)

        @pl.when(n == 0)
        def _():
            out_cp(2 * T, (U - 1) * T).start()
            wait("xb2", "xa2")

        for k in range(1, NLOOP):
            pl.when(n == k)(out_cp((1 + k * U) * T, U * T).start)
        return carry

    def last():
        make_masks()
        i = NT - 1
        r0 = i * T
        it = units(i - 1, 11, False)
        proj_v(1, i, it[:NF])
        out_cp((NT - 3) * T, 2 * T).start()

        def dma_tie():
            ob_v[pl.ds(moff(zw, 16) + S, 16), 0:T] = jnp.zeros((16, T), bf16)
            return pltpu.bitcast(ob_v[pl.ds(moff(zr, 16) + S, 16), 0:T], u32)

        q_ref[0] = pltpu.bitcast(_ubf(oT_ref[4]).T, u32)
        out_cp(T, T, 512, 896).start()

        it = qk(1, i, 0, it[NF:], late=True, extra=[(17, dma_tie())])
        pv(0, i, 2)
        it = it[7:] + qk(1, i, 1, it[:7], 9, late=True)
        pv(0, i, 3)
        proj_o(0, 0, it[:12], 0, slot=2, aslot=1)
        it = it[19:] + qk(1, i, 2, it[12:19], 0, late=True)
        it = it[10:] + qk(1, i, 3, it[:10], 0, late=True)
        proj_o(1, 0, it, 0, slot=3, aslot=1)
        out_cp(0, T).start()
        for g in range(4):
            pv(1, i, g)
        proj_o(0, i, extra=[(8, dma_tie())])
        out_cp(r0, T, 0, 384).start()
        o = project(1, 3, _ubf(oT_ref[1]), (), 0, [(NR - 1, dma_tie())])
        ot = jnp.concatenate([oa_ref[0], o], axis=0).astype(bf16).T
        for a in range(0, T, 32):
            ob_v[r0 + a:r0 + a + 32, 384:896] = ot[a:a + 32]
            out_cp(r0 + a, 32, 384, 896).start()
        zd = dma_tie()
        wo = pad_heads(wo_v[0].astype(f32), 0.0).astype(bf16)
        for c0 in range(0, D, T):
            c1 = min(c0 + T, D)
            lhs = q_ref[0]
            if c1 == D:
                lhs = jnp.concatenate(
                    [lhs[0:56], lhs[56:64] | jnp.concatenate([zd] * 4, axis=1)], axis=0)
            y = jnp.dot(_ubf(lhs), wo[:, c0:c1], preferred_element_type=f32).astype(bf16)
            for a, b in ((0, T),) if c1 < D else ((0, 64), (64, 96), (96, T)):
                ob_v[T + a:T + b, c0:c1] = y[a:b]
                out_cp(T + a, b - a, c0, c0 + T).start()
        out_cp(0, S).wait()

    pl.when(step == 0)(init)

    @pl.when(step == 1)
    def _():
        first()
        lax.fori_loop(0, NLOOP, steady, 0)
        last()


@jax.jit
def pallas_concat_heads__sliding_block__sliding_block__prompt_kernel(
        A_x, A_wqkv, A_wo, B_x, B_wqkv, B_wo):
    anyspec = pl.BlockSpec(memory_space=pl.ANY)
    return pl.pallas_call(
        _kernel,
        grid=(2,),
        in_specs=[anyspec] * 6,
        out_specs=anyspec,
        out_shape=jax.ShapeDtypeStruct((1, S, 2 * D), bf16),
        scratch_shapes=[
            pltpu.VMEM((2, NT, D, T), bf16),
            pltpu.VMEM((2, D, 3 * D), bf16),
            pltpu.VMEM((2, D, D), bf16),
            pltpu.VMEM((S + 64, 2 * D), bf16),
            pltpu.VMEM((2, 2 * D, 4 * T), u32),
            pltpu.VMEM((2, 4, S // 2, T), u32),
            pltpu.VMEM((2, NT + 1, 256, T), u32),
            pltpu.VMEM((2, 256, T), u32),
            pltpu.VMEM((2, 64, 4 * T), u32),
            pltpu.VMEM((5, 256, T), u32),
            pltpu.VMEM((2, 64, T), f32),
        ] + [pltpu.VMEM((MS + 1, 4, 8, 2 * T), f32)] * 4
        + [pltpu.VMEM((ZP + 1, 4, 16, 2 * T), bf16)] * 4
        + [
            pltpu.VMEM((2, 4, 64, T), u32),
            pltpu.VMEM((32, T), u32),
            pltpu.SemaphoreType.DMA((7,)),
        ],
        compiler_params=pltpu.CompilerParams(
            dimension_semantics=("arbitrary",),
            vmem_limit_bytes=64 * 1024 * 1024),
        name="swa",
    )(jnp.swapaxes(A_x, 1, 2), A_wqkv, A_wo, jnp.swapaxes(B_x, 1, 2), B_wqkv, B_wo)
```
